```python
import jax
import jax.numpy as jnp

def _softmax(x, axis=-1):
    return jax.nn.softmax(x, axis=axis)

def _gelu(x):
    return jax.nn.gelu(x, approximate=True)

def _silu(x):
    return jax.nn.silu(x)

def _sigmoid(x):
    return jax.nn.sigmoid(x)

def _layernorm(x, axis=-1, eps=1e-05):
    m = jnp.mean(x, axis=axis, keepdims=True)
    v = jnp.var(x, axis=axis, keepdims=True)
    return (x - m) / jnp.sqrt(v + eps)

def _scatter_add(tgt, idx, src, axis=0):
    return tgt.at[idx].add(src)

def _segment_sum(src, seg, n):
    return jax.ops.segment_sum(src, seg, n)

class _Rng:

    def __init__(self, key):
        self._k = key

    def _next(self):
        self._k, sub = jax.random.split(self._k)
        return sub

    def normal(self, shape):
        return jax.random.normal(self._next(), shape, dtype=jnp.bfloat16)

    def randint(self, lo, hi, shape):
        return jax.random.randint(self._next(), shape, lo, hi, dtype=jnp.int32)

    def uniform(self, shape, lo=0.0, hi=1.0):
        return jax.random.uniform(self._next(), shape, jnp.bfloat16, lo, hi)

    def permutation(self, n):
        return jax.random.permutation(self._next(), n)
kernel_name = 'sequential_preLN__sliding_local_dilated__mixer_gmlp__prompt'

def setup_inputs():
    _rng = _Rng(jax.random.key(int.from_bytes(__import__("os").urandom(4), "little")))
    _w = lambda a: (lambda t: t.astype(jnp.bfloat16) if jnp.issubdtype(t.dtype, jnp.floating) else t)(jnp.asarray(a))

    def _A_setup():
        B, S, D = (1, 2048, 1024)
        return {'x': _w((lambda *s: _rng.normal(s) * 0.05)(B, S, D)), 'wqkv': _w((lambda *s: _rng.normal(s) * 0.05)(D, 3 * D)), 'wo': _w((lambda *s: _rng.normal(s) * 0.05)(D, D))}
    _A_in = _A_setup()

    def _B_setup():
        B, S, D, F = (1, 2048, 1024, 3584)
        Fh = F // 2
        return {'x': _w((lambda *s: _rng.normal(s) * 0.05)(B, S, D)), 'w_in': _w((lambda *s: _rng.normal(s) * 0.05)(D, 2 * Fh)), 'w_sp': _w(0.01 * (lambda *s: _rng.normal(s) * 0.05)(S, S)), 'b_sp': _w(1.0 + 0.01 * (lambda *s: _rng.normal(s) * 0.05)(S)), 'w_out': _w((lambda *s: _rng.normal(s) * 0.05)(Fh, D))}
    _B_in = _B_setup()
    return {'A_x': _A_in['x'], 'A_wqkv': _A_in['wqkv'], 'A_wo': _A_in['wo'], 'B_x': _B_in['x'], 'B_w_in': _B_in['w_in'], 'B_w_sp': _B_in['w_sp'], 'B_b_sp': _B_in['b_sp'], 'B_w_out': _B_in['w_out']}

def reference(A_x, A_wqkv, A_wo, B_x, B_w_in, B_w_sp, B_b_sp, B_w_out):

    def _A_ref(x, wqkv, wo):
        B, S, D = x.shape
        H = 32
        Dh = D // H
        W, dil = (8, 2)
        qkv = (lambda x, *d: x.transpose(*d))((x @ wqkv).reshape(B, S, 3, H, Dh), 2, 0, 3, 1, 4)
        q, k, v = (qkv[0], qkv[1], qkv[2])
        scale = Dh ** (-0.5)
        pos = jnp.arange(S)
        off = jnp.arange(W) * dil
        idx = pos[:, None] - off[None, :]
        mask = idx >= 0
        idx_c = jnp.where(mask, idx, 0).reshape(-1)
        kg = k[:, :, idx_c, :].reshape(B, H, S, W, Dh)
        vg = v[:, :, idx_c, :].reshape(B, H, S, W, Dh)
        logits = jnp.einsum('bhsd,bhswd->bhsw', q, kg) * scale
        logits = jnp.where(mask[None, None, :, :], logits, -1000000000.0)
        attn = _softmax(logits, axis=-1)
        o = jnp.einsum('bhsw,bhswd->bhsd', attn, vg)
        return (lambda x, *d: x.transpose(*d))(o, 0, 2, 1, 3).reshape(B, S, D) @ wo

    def _B_ref(x, w_in, w_sp, b_sp, w_out):
        B, S, D = x.shape
        F = w_in.shape[-1]
        Fh = F // 2
        z = _gelu(jnp.einsum('bsd,df->bsf', x, w_in))
        z1 = z[..., :Fh].copy()
        z2 = _layernorm(z[..., Fh:], axis=-1)
        g = jnp.einsum('ts,bsf->btf', w_sp, z2) + b_sp[None, :, None]
        return jnp.einsum('bsf,fd->bsd', z1 * g, w_out)
    x = A_x
    h = x + _A_ref(_layernorm(x, axis=-1), A_wqkv, A_wo)
    h2 = h + _B_ref(_layernorm(h, axis=-1), B_w_in, B_w_sp, B_b_sp, B_w_out)
    return h2
```

```python
import functools
import jax
import jax.numpy as jnp
from jax import lax
import jax.experimental.pallas as pl
import jax.experimental.pallas.tpu as pltpu

S, D, FH = 2048, 1024, 1792
H, DH, W, DIL = 32, 32, 8, 2
PAD = 16
EPS = 1e-5
F32, BF16 = jnp.float32, jnp.bfloat16


def _ln(x):
    m = jnp.mean(x, axis=-1, keepdims=True)
    xc = x - m
    v = jnp.mean(xc * xc, axis=-1, keepdims=True)
    return xc * lax.rsqrt(v + EPS)


def _gelu(x):
    c = 0.7978845608028654
    u = x * (c + (c * 0.044715) * (x * x))
    hx = 0.5 * x
    return hx + hx * jnp.tanh(u)


def _swap_chunks(chunks):
    shape = chunks[0].shape
    grp = (lax.broadcasted_iota(jnp.int32, shape, 1) >> 1) & 7
    r = [c if i == 0 else pltpu.roll(c, 2 * i, 1) for i, c in enumerate(chunks)]
    out = []
    for j in range(8):
        t = r[0]
        for i in range(1, 8):
            t = jnp.where(grp == (i + j) % 8, r[i], t)
        out.append(t if j == 0 else pltpu.roll(t, 128 - 2 * j, 1))
    return out


def _dot(a, b):
    return jnp.dot(a, b, preferred_element_type=F32)


def build(TM=256, TM2=256):
    NB = S // TM
    NB2 = S // TM2

    def kernel(x_hbm, wqkv_hbm, wo_hbm, win_hbm, wsp_hbm, b_ref, wout_hbm, out_hbm,
               x_v, wqkv_v, wo_v, win_v, wsp_v, wout_v, q_s, k_s, v_s, o_s, h_v, hn_v, z2_v, out_v,
               sems, osem):
        cps = [
            pltpu.make_async_copy(x_hbm, x_v, sems.at[0]),
            pltpu.make_async_copy(wqkv_hbm, wqkv_v, sems.at[1]),
            pltpu.make_async_copy(wo_hbm, wo_v, sems.at[2]),
            pltpu.make_async_copy(win_hbm, win_v, sems.at[3]),
            pltpu.make_async_copy(wsp_hbm, wsp_v, sems.at[4]),
            pltpu.make_async_copy(wout_hbm, wout_v, sems.at[5]),
        ]
        for c in cps:
            c.start()
        cps[0].wait()
        cps[1].wait()

        def perm(r, _):
            rows = pl.ds(pl.multiple_of(r * 64, 64), 64)
            for t in range(3):
                ch = [pltpu.bitcast(wqkv_v[rows, t * D + c * 128:t * D + (c + 1) * 128], jnp.int32) for c in range(8)]
                ch = _swap_chunks(ch)
                for c in range(8):
                    wqkv_v[rows, t * D + c * 128:t * D + (c + 1) * 128] = pltpu.bitcast(ch[c], BF16)
            return 0
        lax.fori_loop(0, D // 64, perm, 0)
        cps[2].wait()
        cps[3].wait()

        k_s[:, 0:PAD, :] = jnp.zeros((8, PAD, 128), F32)
        v_s[:, 0:PAD, :] = jnp.zeros((8, PAD, 128), F32)

        def p1(i, _):
            rows = pl.ds(pl.multiple_of(i * TM, TM), TM)
            x = x_v[rows, :].astype(F32)
            xn = _ln(x).astype(BF16)
            qkv = _dot(xn, wqkv_v[...])
            for c in range(8):
                q_s[c] = qkv[:, c * 128:(c + 1) * 128] * (DH ** -0.5)
                k_s[c, PAD:, :] = qkv[:, D + c * 128:D + (c + 1) * 128]
                v_s[c, PAD:, :] = qkv[:, 2 * D + c * 128:2 * D + (c + 1) * 128]
            RB = 32
            lane = lax.broadcasted_iota(jnp.int32, (RB, 128), 1)
            row = lax.broadcasted_iota(jnp.int32, (RB, 128), 0)
            b0 = (lane & 1) == 0
            b4 = (lane & 16) == 0
            for r0 in range(0, TM, RB):
                q = [q_s[c, r0:r0 + RB, :] for c in range(8)]
                lg = []
                for w in range(W):
                    o = PAD + r0 - DIL * w
                    p = q[0] * k_s[0, o:o + RB, :]
                    for c in range(1, 8):
                        p = p + q[c] * k_s[c, o:o + RB, :]
                    p = p + jnp.where(b4, pltpu.roll(p, 128 - 16, 1), pltpu.roll(p, 16, 1))
                    p = p + jnp.where(b0, pltpu.roll(p, 128 - 1, 1), pltpu.roll(p, 1, 1))
                    if r0 < DIL * w:
                        p = jnp.where(row + (i * TM + r0) >= DIL * w, p, -1e9)
                    lg.append(p)
                m = functools.reduce(jnp.maximum, lg)
                e = [jnp.exp(p - m) for p in lg]
                inv = 1.0 / functools.reduce(jnp.add, e)
                a = [t * inv for t in e]
                oc = []
                for c in range(8):
                    acc = a[0] * v_s[c, PAD + r0:PAD + r0 + RB, :]
                    for w in range(1, W):
                        o = PAD + r0 - DIL * w
                        acc = acc + a[w] * v_s[c, o:o + RB, :]
                    oc.append(pltpu.bitcast(acc.astype(BF16), jnp.int32))
                oc = _swap_chunks(oc)
                for c in range(8):
                    o_s[r0:r0 + RB, c * 128:(c + 1) * 128] = pltpu.bitcast(oc[c], BF16)
            k_s[:, 0:PAD, :] = k_s[:, TM:TM + PAD, :]
            v_s[:, 0:PAD, :] = v_s[:, TM:TM + PAD, :]
            h = x + _dot(o_s[...], wo_v[...])
            h_v[rows, :] = h
            hn = _ln(h).astype(BF16)
            hn_v[rows, :] = hn
            z = _gelu(_dot(hn, win_v[:, FH:]))
            z2_v[rows, :] = _ln(z).astype(BF16)
            return 0
        lax.fori_loop(0, NB, p1, 0)
        cps[4].wait()
        cps[5].wait()

        def p2(i, _):
            rows = pl.ds(pl.multiple_of(i * TM2, TM2), TM2)
            z1 = _gelu(_dot(hn_v[rows, :], win_v[:, :FH]))
            g = _dot(wsp_v[rows, :], z2_v[...]) + b_ref[rows, :]
            y = (z1 * g).astype(BF16)
            out_v[rows, :] = (h_v[rows, :] + _dot(y, wout_v[...])).astype(BF16)
            pltpu.make_async_copy(out_v.at[rows, :], out_hbm.at[rows, :], osem).start()
            return 0
        lax.fori_loop(0, NB2, p2, 0)
        pltpu.make_async_copy(out_v, out_hbm, osem).wait()

    def fn(A_x, A_wqkv, A_wo, B_x, B_w_in, B_w_sp, B_b_sp, B_w_out):
        del B_x
        hbm = pl.BlockSpec(memory_space=pl.ANY)
        out = pl.pallas_call(
            kernel,
            out_shape=jax.ShapeDtypeStruct((S, D), BF16),
            in_specs=[hbm, hbm, hbm, hbm, hbm, pl.BlockSpec(memory_space=pltpu.VMEM), hbm],
            out_specs=hbm,
            scratch_shapes=[
                pltpu.VMEM((S, D), BF16), pltpu.VMEM((D, 3 * D), BF16), pltpu.VMEM((D, D), BF16),
                pltpu.VMEM((D, 2 * FH), BF16), pltpu.VMEM((S, S), BF16), pltpu.VMEM((FH, D), BF16),
                pltpu.VMEM((8, TM, 128), F32), pltpu.VMEM((8, TM + PAD, 128), F32), pltpu.VMEM((8, TM + PAD, 128), F32),
                pltpu.VMEM((TM, D), BF16), pltpu.VMEM((S, D), F32), pltpu.VMEM((S, D), BF16),
                pltpu.VMEM((S, FH), BF16), pltpu.VMEM((S, D), BF16),
                pltpu.SemaphoreType.DMA((6,)), pltpu.SemaphoreType.DMA(()),
            ],
            compiler_params=pltpu.CompilerParams(vmem_limit_bytes=110 * 1024 * 1024),
        )(A_x.reshape(S, D), A_wqkv, A_wo, B_w_in, B_w_sp, B_b_sp.reshape(S, 1), B_w_out)
        return out.reshape(1, S, D)
    return fn


@jax.jit
def pallas_sequential_preLN__sliding_local_dilated__mixer_gmlp__prompt_kernel(A_x, A_wqkv, A_wo, B_x, B_w_in, B_w_sp, B_b_sp, B_w_out):
    return build()(A_x, A_wqkv, A_wo, B_x, B_w_in, B_w_sp, B_b_sp, B_w_out)
```

```python
import functools
import math

import jax
import jax.numpy as jnp
from jax import lax
import jax.experimental.pallas as pl
import jax.experimental.pallas.tpu as pltpu

S, D, FH = 2048, 1024, 1792
H, DH, W, DIL = 32, 32, 8, 2
EPS = 1e-5
F32, BF16, I32 = jnp.float32, jnp.bfloat16, jnp.int32
T = 128
TM = 2 * T
NB = S // TM
PAD = 16


def _gelu(x):
    c = math.sqrt(2.0 / math.pi)
    u = x * (c + (c * 0.044715) * (x * x))
    hx = 0.5 * x
    return hx + hx * jnp.tanh(u)


def _skew(parts, axis, unit):
    return [c if i == 0 else pltpu.roll(c, unit * i, axis) for i, c in enumerate(parts)]


def _unskew(parts, axis, unit):
    n = parts[0].shape[axis]
    grp = (lax.broadcasted_iota(I32, parts[0].shape, axis) // unit) & 7
    out = []
    for j in range(8):
        t = parts[0]
        for i in range(1, 8):
            t = jnp.where(grp == (i + j) % 8, parts[i], t)
        out.append(t if j == 0 else pltpu.roll(t, n - unit * j, axis))
    return out


def _lhs7(a11, a12, a21, a22):
    return [a11 + a22, a21 + a22, a11, a22, a11 + a12, a21 - a11, a12 - a22]


def _rhs7(b11, b12, b21, b22):
    return [b11 + b22, b11, b12 - b22, b21 - b11, b22, b11 + b12, b21 + b22]


def _sum(xs):
    return functools.reduce(jnp.add, xs)


def _overlap(main, *sides):
    total, t, ev = sum(c for c, _ in main), 0.0, []
    for c, f in main:
        ev.append((t / total, 1, c, f))
        t += c
    for side, lo, hi, *due in sides:
        ev += [(when, 0, 0.0, f) for when, f in due]
        total, t = sum(c for c, _ in side), 0.0
        for c, f in side:
            ev.append((lo + (hi - lo) * t / total, 0, 0.0, f))
            t += c
    ev.sort(key=lambda e: e[:2])
    return [(e[2], e[3]) for e in ev]


def _stagger(stages):
    n, out = len(stages[0]), []
    for k in range(n + len(stages) - 1):
        now = [st[k - s] for s, st in enumerate(stages) if 0 <= k - s < n]
        now = [((j + 0.5) / len(g), s, t) for s, g in enumerate(now) for j, t in enumerate(g)]
        out += [t for _, _, t in sorted(now, key=lambda e: e[:2])]
    return out


def _tile(c):
    return slice(c * T, (c + 1) * T)


def _ds(start, n, align=8):
    return pl.ds(start if isinstance(start, int) else pl.multiple_of(start, align), n)


class _Operand:
    def __init__(self, ref, base, rows, nt):
        self.ref, self.base, self.rows, self.nt = ref, base, rows, nt

    @staticmethod
    def size(rows, nt):
        return (7 * nt + 1) // 2 * rows // 2

    def at(self, j, r, c, n):
        g = j * self.nt + c
        return _ds(self.base + g // 2 * self.rows // 2 + r // 2, n // 2), _tile(g % 2)

    def put(self, r, c, mats):
        for j, t in enumerate(mats):
            self.ref[self.at(j, r, c, t.shape[0])] = pltpu.bitcast(t.astype(BF16), I32)

    def col(self, j, c):
        return pltpu.bitcast(self.ref[self.at(j, 0, c, self.rows)], BF16)

    def full(self, j, zeros=()):
        cols = [self.ref[self.at(j, 0, c, self.rows)] for c in range(self.nt)]
        for z in zeros:
            cols[-1] = jnp.concatenate([cols[-1][:-8], cols[-1][-8:] | z], 0)
        return jnp.concatenate([pltpu.bitcast(c, BF16) for c in cols], 1)


_STATIC = dict(wq=(D // 2, 4), wk=(D // 2, 4), wv=(D // 2, 4), wo=(D // 2, 4), w1=(D // 2, 7), w2=(D // 2, 7),
               wout=(FH // 2, 4), xa=(T, 4), xb=(T, 4), oa=(T, 4), sa=(T, 8), ya=(T, 7))
_HA = _Operand.size(T, 4)


def build(RA=8, RB=64, RS=32, RL=16, RW=32, scopes=False, only=None, f1=0.38, f2=0.84, f3=0.268, rel=0, nq=2, fz=0.3, fx=0.8, fy=0.96, macc=0, flags=None):
    def kernel(x_hbm, wqkv_hbm, wo_hbm, win_hbm, wsp_hbm, b_hbm, wout_hbm, out_hbm,
               x_v, wqkv_v, wo_v, win_v, wsp_v, wout_v, ops_v, ha_v, z2_v,
               qk0, v0, qk1, v1, h_v, gz_v, z1_v, stat_v, acc_v, bias_v, b_v, sems, osem, *stage_v):
        out_v = x_v
        op, top = {}, 0
        for name, (r, nt) in _STATIC.items():
            op[name] = _Operand(ops_v, top, r, nt)
            top += _Operand.size(r, nt)
        z2_op = _Operand(z2_v, 0, S // 2, 7)

        def ha(i):
            return _Operand(ha_v, (i % 2) * _HA, T, 4)

        zero, zero2 = lax.fori_loop(0, 2, lambda _, c: (c[1] ^ 1, c[0] ^ 1), (0, 0))

        class Acc:
            def __init__(self):
                self.v = {}

            def __setitem__(self, k, v):
                n = 'tk'.index(k)
                if n < macc:
                    acc_v[_ds(zero * 8 + n * T, T), :] = v
                else:
                    self.v[k] = v

            def __getitem__(self, k):
                n = 'tk'.index(k)
                return acc_v[_ds(zero2 * 8 + n * T, T), :] if n < macc else self.v[k]

        copies, last, paced, ready = {}, [None], {}, {}

        def pace(ref):
            if last[0] is None or paced.get(id(ref)) is last[0]:
                return
            paced[id(ref)] = last[0]
            n = 8 if ref.dtype == F32 else 16
            ref[_ds(zero * n + (ref.shape[0] - n), n, n), 0:T] = last[0][rel:rel + n].astype(ref.dtype)

        pending = []
        for ref in (ops_v, z2_v):
            ref[_ds(ref.shape[0] - 8, 8), 0:T] = jnp.zeros((8, T), I32)

        def due(ref, when):
            return when, lambda: pending.append(ref[_ds(zero * 8 + (ref.shape[0] - 8), 8), 0:T])

        def start(key, src, dst):
            copies[key] = pltpu.make_async_copy(src, dst, sems.at[len(copies)])
            copies[key].start()

        def unit(lhs, rhs, u, emit, reverse=False):
            s = Acc()

            def step(n, r):
                def run():
                    last[0] = m = jnp.dot(lhs.full(r, pending), rhs.col(r, u), preferred_element_type=F32)
                    pending.clear()
                    mid = (0, 1) if reverse else (1, 0)
                    diag = (1, 1) if reverse else (0, 0)
                    if n == 0:
                        s['t'] = m
                    elif n == 1:
                        s['t'], s['k'] = s['t'] + m, m
                    elif n == 2:
                        emit(*mid, m + s['k'])
                        s['k'] = m
                    elif n == 3:
                        s['t'], s['k'] = s['t'] + m, m - s['k']
                    elif n == 4:
                        emit(*diag, s['t'] - m)
                        s['t'] = m
                    elif n == 5:
                        emit(*mid[::-1], m + s['t'])
                        s['k'] = s['k'] + m
                    else:
                        emit(1 - diag[0], 1 - diag[1], s['k'] + m)
                return run
            order = (6, 3, 1, 0, 4, 2, 5)[::-1 if reverse else 1]
            return [(rhs.rows // 4, step(n, r)) for n, r in enumerate(order)]

        def ln_combos(src, load, nt, dst, row0, combos, stat):
            def mean(r):
                def run():
                    pace(src)
                    m = jnp.sum(_sum([load(r, c, RS) for c in range(nt)]), axis=-1, keepdims=True) * (1.0 / (nt * T))
                    stat_v[_ds(stat + r, RS), :] = jnp.broadcast_to(m, (RS, T))
                return (nt * RS / 64, run)

            def rstd(r):
                def run():
                    pace(src)
                    m = stat_v[_ds(stat + r, RS), :]
                    v = [load(r, c, RS) - m for c in range(nt)]
                    var = jnp.sum(_sum([t * t for t in v]), axis=-1, keepdims=True) * (1.0 / (nt * T))
                    stat_v[_ds(stat + TM + r, RS), :] = jnp.broadcast_to(lax.rsqrt(var + EPS), (RS, T))
                return (3 * nt * RS / 64, run)

            def norm(r0, cs):
                def run():
                    pace(src)
                    st = [(stat_v[_ds(stat + r, RL), :], stat_v[_ds(stat + TM + r, RL), :]) for r in (r0, T + r0)]
                    for c in cs:
                        dst.put(row0 + r0, c, combos(*[(load(r, cc, RL) - m) * inv
                                                       for r, (m, inv) in zip((r0, T + r0), st)
                                                       for cc in (c, nt // 2 + c)]))
                return (17 * len(cs) * RL / 64, run)
            gs = range(0, T, RS)
            parts = [range(c, min(c + 4, nt // 2)) for c in range(0, nt // 2, 4)]
            return _stagger([[[mean(g), mean(T + g)] for g in gs], [[rstd(g), rstd(T + g)] for g in gs],
                             [[norm(r, cs) for r in range(g, g + RS, RL) for cs in parts] for g in gs]])

        def w_prep(w_ref, c0, dst):
            kh, nh = dst.rows, dst.nt

            def task(r0, c):
                def run():
                    pace(w_ref)
                    dst.put(r0, c, _rhs7(*[w_ref[r:r + RW, c0 + cc * T:c0 + (cc + 1) * T].astype(F32)
                                           for r in (r0, kh + r0) for cc in (c, nh + c)]))
                return (3.5 * RW / 16, run)
            return [task(r0, c) for c in range(nh) for r0 in range(0, kh, RW)]

        def qkv_prep(t, lo=0, hi=D // 2):
            val = {}

            def skew(r):
                def run():
                    pace(wqkv_v)
                    val[r] = _skew([pltpu.bitcast(wqkv_v[r:r + 16, _tile(8 * t + c)], I32) for c in range(8)], 1, 2)
                return (2, run)

            def unskew(r):
                def run():
                    val[r] = _unskew(val[r], 1, 2)
                return (7, run)

            def store(r0):
                def run():
                    hv = [[pltpu.bitcast(p, BF16).astype(F32) for p in val[r]] for r in (r0, D // 2 + r0)]
                    for c in range(4):
                        op['w' + 'qkv'[t]].put(r0, c, _rhs7(hv[0][c], hv[0][4 + c], hv[1][c], hv[1][4 + c]))
                return (12, run)
            rs = [a + r for r in range(lo, hi, 16) for a in (0, D // 2)]
            return _stagger([[[skew(r)] for r in rs], [[unskew(r)] for r in rs],
                             [[store(r - D // 2)] if r >= D // 2 else [] for r in rs]])

        def wo_prep():
            def task(g, c):
                def run():
                    pace(wo_v)
                    hv = [[pltpu.bitcast(p, BF16).astype(F32) for p in _unskew(_skew(
                        [pltpu.bitcast(wo_v[i * T + g:i * T + g + 16, _tile(cc)], I32) for i in range(8)], 0, 1), 0, 1)]
                        for cc in (c, 4 + c)]
                    for j in range(4):
                        op['wo'].put(j * T + g, c, _rhs7(hv[0][j], hv[1][j], hv[0][4 + j], hv[1][4 + j]))
                return (32, run)
            return [task(g, c) for c in range(4) for g in range(0, T, 16)]

        def ln_x(i, dst):
            return ln_combos(x_v, lambda r, c, n: x_v[_ds(i * TM + r, n, 16), _tile(c)].astype(F32), 8,
                             dst, 0, _lhs7, 0)

        def ln_h(i):
            return ln_combos(h_v, lambda r, c, n: h_v[_ds(c * S + i * TM + r, n), :], 8, ha(i), 0, _lhs7, 2 * TM)

        def ln_z(i):
            return ln_combos(gz_v, lambda r, c, n: gz_v[_ds(c * TM + r, n), :], 14, z2_op, i * T, _rhs7, 4 * TM)

        def sp_prep(i):
            def task(r0, b):
                def run():
                    pace(wsp_v)
                    op['sa'].put(r0, b, _lhs7(*[wsp_v[_ds(i * TM + r, 32, 16), _tile(2 * b + cc)].astype(F32)
                                                for r in (r0, T + r0) for cc in (0, 1)]))
                return (7, run)
            return [task(r0, b) for b in range(NB) for r0 in range(0, T, 32)]

        def row(c, r):
            return c * (TM + PAD) + PAD + r

        def qkv(i, lhs, bufs, which):
            tasks = []
            for t in which:
                for u in range(4):
                    def emit(a, b, v, t=t, u=u):
                        ref, c = bufs[t // 2], t % 2 * 8 + 4 * b + u
                        ref[_ds(row(c, a * T), T), :] = v
                        ready[id(ref)] = t > 0 and (u, a, b) == (3, 1, 1)
                        if t and a == 0 and isinstance(i, int) and i == 0:
                            ref[_ds(row(c, -PAD), PAD), :] = jnp.broadcast_to(v[0:1], (PAD, T))
                    tasks += unit(lhs, op['w' + 'qkv'[t]], u, emit)
            return tasks

        def history(src, dst):
            for t in (1, 2):
                for c in range(t % 2 * 8, t % 2 * 8 + 8):
                    dst[t // 2][_ds(row(c, -PAD), PAD), :] = src[t // 2][_ds(row(c, TM - PAD), PAD), :]

        def slot(stage, w, r):
            return stage_v[2 * stage + r // RB % 2], (w * 2 + r // T) * RB + r % RB

        def groups(f):
            return [[f(a + r) for a in (0, T) for r in range(g, g + RB, RA)] for g in range(0, T, RB)]

        def att(bufs, first=False):
            scale = DH ** -0.5
            qk, v = bufs

            def grab(stage, r):
                pace(slot(stage, 0, r)[0])
                return [ref[_ds(o, RA), :] for ref, o in (slot(stage, w, r) for w in range(W))]

            def scores(r):
                def run():
                    assert ready[id(qk)]
                    pace(qk)
                    q = [qk[_ds(row(c, r), RA), :] for c in range(8)]
                    for w in range(W):
                        ref, o = slot(0, w, r)
                        ref[_ds(o, RA), :] = _sum([q[c] * qk[_ds(row(8 + c, r - DIL * w), RA), :] for c in range(8)])
                return (15 * RA / 8, run)

            def fold(r):
                def run():
                    lane = lax.broadcasted_iota(I32, (RA, T), 1)
                    b0, b4 = (lane & 1) == 0, (lane & 16) == 0
                    ps = grab(0, r)
                    for bit, low in ((16, b4), (1, b0)):
                        ps = [p + jnp.where(low, pltpu.roll(p, T - bit, 1), pltpu.roll(p, bit, 1)) for p in ps]
                    for w, p in enumerate(ps):
                        if first and r < DIL * w:
                            p = jnp.where(lax.broadcasted_iota(I32, (RA, T), 0) + r >= DIL * w, p, -1e9 / scale)
                        ref, o = slot(1, w, r)
                        ref[_ds(o, RA), :] = p
                return (8 * RA / 8, run)

            def softmax(r):
                def run():
                    lg = grab(1, r)
                    m = functools.reduce(jnp.maximum, lg)
                    e = [jnp.exp2((p - m) * (scale * math.log2(math.e))) for p in lg]
                    inv = 1.0 / _sum(e)
                    for w in range(W):
                        ref, o = slot(2, w, r)
                        ref[_ds(o, RA), :] = e[w] * inv
                return (7 * RA / 8, run)

            def mix(r):
                def run():
                    pace(v)
                    assert ready[id(v)]
                    p = grab(2, r)
                    for c in range(8):
                        ref, o = slot(3, c, r)
                        ref[_ds(o, RA), :] = _sum([p[w] * v[_ds(row(c, r - DIL * w), RA), :] for w in range(W)])
                return (15 * RA / 8, run)

            def combo(r, cs):
                def run():
                    pace(slot(3, 0, r)[0])
                    for c in cs:
                        op['oa'].put(r, c, _lhs7(*[ref[_ds(o, 16), :] for ref, o in (
                            slot(3, cc, a + r) for a in (0, T) for cc in (c, 4 + c))]))
                return (2 * len(cs), run)
            return _stagger([groups(f) for f in (scores, fold, softmax, mix)] + [
                [[combo(r, range(4)) for r in range(g, g + RB, 16)] for g in range(0, T, RB)]])

        def proj(i):
            tasks = []
            for u in range(4):
                def emit(a, b, v, u=u):
                    c, r = 4 * b + u, i * TM + a * T
                    h_v[_ds(c * S + r, T), :] = x_v[_ds(r, T, 16), _tile(c)].astype(F32) + v
                tasks += unit(op['oa'], op['wo'], u, emit)
            return tasks

        def z2(i):
            tasks = []
            for u in range(7):
                def emit(a, b, v, u=u):
                    gz_v[_ds((7 * b + u) * TM + a * T, T), :] = _gelu(v)
                tasks += unit(ha(i), op['w2'], u, emit)
            return tasks

        def z1(i):
            tasks = []
            for u in range(7):
                def emit(a, b, v, u=u):
                    z1_v[_ds((u * S + i * TM + a * T) // 2, T // 2), _tile(b)] = pltpu.bitcast(
                        _gelu(v).astype(BF16), I32)
                tasks += unit(ha(i), op['w1'], u, emit)
            return tasks

        def bias_prep():
            def task(k):
                def run():
                    bias_v[_ds(k * T, T), :] = jnp.broadcast_to(b_v[...].astype(F32)[k:k + 1, :], (T, T)).T
                return (4, run)
            return [task(k) for k in range(S // T)]

        def gate(i):
            tasks = []
            for u in range(7):
                y = {}

                def emit(a, b, v, u=u, y=y):
                    z = z1_v[_ds((u * S + i * TM + a * T) // 2, T // 2), _tile(b)]
                    y[a, b] = pltpu.bitcast(z, BF16).astype(F32) * (v + bias_v[_ds(i * TM + a * T, T), :])
                    if len(y) == 4:
                        op['ya'].put(0, u, _lhs7(y[0, 0], y[0, 1], y[1, 0], y[1, 1]))
                tasks += unit(op['sa'], z2_op, u, emit)
            return tasks

        def down(i):
            tasks = []
            for u in range(4):
                def emit(a, b, v, u=u):
                    c, r = 4 * b + u, i * TM + a * T
                    out_v[_ds(r, T, 16), _tile(c)] = (h_v[_ds(c * S + r, T), :] + v).astype(BF16)
                tasks += unit(op['ya'], op['wout'], u, emit, reverse=True)
            return tasks

        def go(name, tasks):
            if scopes:
                with jax.named_scope(name):
                    for _, f in tasks:
                        f()
            else:
                for _, f in tasks:
                    f()

        def wait(*keys):
            for k in keys:
                copies[k].wait()

        first, cur = (qk1, v1), (qk0, v0)

        def mixer_step(i, _):
            last[0] = None
            history(cur, cur)
            go('p1', _overlap(
                qkv(i, op['xa'], cur, (0, 1, 2)) + z2(i - 1) + z1(i - 2) + proj(i),
                (ln_z(i - 2) + ln_h(i - 1), 0.0, f1, due(z2_v, fz)), (att(cur), f3, f2),
                (ln_x(jnp.minimum(i + 1, NB - 1), op['xa']), fx, fy, due(ops_v, 0.99))))
            last[0] = None

        def gate_step(i, _):
            last[0] = None
            go('p2', _overlap(gate(i) + down(i), (sp_prep(jnp.minimum(i + 1, NB - 1)), 0.67, 0.95)))
            rows = _ds(i * TM, TM, 16)
            pltpu.make_async_copy(out_v.at[rows], out_hbm.at[rows], osem).start()
            last[0] = None

        if only:
            lax.fori_loop(2, NB, mixer_step if only == 1 else gate_step, None)
            dyn = _ds(zero * 16, 16)
            out_v[0:16, 0:T] = (h_v[dyn, :] + (z2_v[dyn, 0:T] + z1_v[dyn, 0:T] + ops_v[dyn, 0:T]).astype(F32)).astype(BF16)
            pltpu.make_async_copy(out_v.at[0:S], out_hbm, osem).start()
            pltpu.make_async_copy(out_v.at[0:S], out_hbm, osem).wait()
            return

        start('x0', x_hbm.at[0:TM], x_v.at[0:TM])
        QC = D // 2 // nq
        for k in range(nq):
            for a in (0, D // 2):
                start(('q', k, a), wqkv_hbm.at[a + k * QC:a + (k + 1) * QC, 0:D],
                      wqkv_v.at[a + k * QC:a + (k + 1) * QC, 0:D])
        for t in (1, 2):
            start(t, wqkv_hbm.at[:, t * D:(t + 1) * D], wqkv_v.at[0:D, t * D:(t + 1) * D])
        start('x1', x_hbm.at[TM:2 * TM], x_v.at[TM:2 * TM])
        start('wo', wo_hbm, wo_v.at[0:D])
        start('w2', win_hbm.at[:, FH:], win_v.at[0:D, FH:])
        start('x', x_hbm.at[2 * TM:], x_v.at[2 * TM:S])
        start('w1', win_hbm.at[:, :FH], win_v.at[0:D, :FH])
        start('b', b_hbm, b_v)

        wait('x0')
        go('lnx', ln_x(0, op['xa']))
        for k in range(nq):
            wait(('q', k, 0), ('q', k, D // 2))
            go('wq', qkv_prep(0, k * QC, (k + 1) * QC))
        wait(1)
        go('q0', _overlap(qkv(0, op['xa'], first, (0,)), (qkv_prep(1), 0.0, 0.9)))
        wait(2, 'x1')
        go('k0', _overlap(qkv(0, op['xa'], first, (1,)), (qkv_prep(2), 0.0, 0.9)))
        wait('wo')
        main = qkv(0, op['xa'], first, (2,)) + [(0, lambda: history(first, cur))] + qkv(1, op['xb'], cur, (0, 1))
        go('s1', _overlap(main, (ln_x(1, op['xb']), 0.0, 0.28), (att(first, True), 0.1, 0.93),
                          (wo_prep(), 0.3, 0.93)))
        wait('w2', 'x', 'w1', 'b')
        start('wsp', wsp_hbm, wsp_v.at[0:S])
        start('wout', wout_hbm, wout_v.at[0:FH])
        go('s2', _overlap(proj(0) + qkv(1, op['xb'], cur, (2,)) + z2(0) + proj(1),
                          (w_prep(win_v, FH, op['w2']), 0.0, 0.5), (ln_h(0), 0.22, 0.39), (att(cur), 0.15, 0.75),
                          (ln_x(2, op['xa']), 0.7, 0.95), (w_prep(win_v, 0, op['w1']), 0.55, 0.96, due(ops_v, 0.985))))
        lax.fori_loop(2, NB, mixer_step, None)
        wait('wsp', 'wout')
        go('t', _overlap(z1(NB - 2) + z2(NB - 1) + z1(NB - 1),
                         (ln_h(NB - 1) + ln_z(NB - 2), 0.0, 0.32, due(z2_v, 0.36)),
                         (w_prep(wout_v, 0, op['wout']) + sp_prep(0) + bias_prep(), 0.33, 0.7, due(ops_v, 0.75)),
                         (ln_z(NB - 1), 0.68, 0.95, due(z2_v, 0.985))))
        lax.fori_loop(0, NB, gate_step, None)
        pltpu.make_async_copy(out_v.at[0:S], out_hbm, osem).wait()

    def fn(A_x, A_wqkv, A_wo, B_x, B_w_in, B_w_sp, B_b_sp, B_w_out):
        del B_x
        hbm = pl.BlockSpec(memory_space=pl.ANY)
        vm = pltpu.VMEM
        out = pl.pallas_call(
            kernel,
            out_shape=jax.ShapeDtypeStruct((S, D), BF16),
            in_specs=[hbm, hbm, hbm, hbm, hbm, hbm, hbm],
            out_specs=hbm,
            scratch_shapes=[
                vm((S + PAD, D), BF16), vm((D + PAD, 3 * D), BF16), vm((D + PAD, D), BF16),
                vm((D + PAD, 2 * FH), BF16), vm((S + PAD, S), BF16), vm((FH + PAD, D), BF16),
                vm((sum(_Operand.size(*s) for s in _STATIC.values()) + 8, 2 * T), I32),
                vm((2 * _HA, 2 * T), I32), vm((_Operand.size(S // 2, 7) + 8, 2 * T), I32),
                *[vm((n * (TM + PAD) + PAD, T), F32) for n in (16, 8, 16, 8)],
                vm((8 * S + PAD, T), F32), vm((14 * TM + PAD, T), F32), vm((7 * S // 2, 2 * T), I32),
                vm((6 * TM, T), F32), vm((2 * T, T), F32), vm((S, T), F32), vm((S // T, T), BF16),
                pltpu.SemaphoreType.DMA((24,)), pltpu.SemaphoreType.DMA(()),
                *[vm((16 * RB + 8, T), F32)] * 8,
            ],
            compiler_params=pltpu.CompilerParams(vmem_limit_bytes=124 * 1024 * 1024,
                                                 flags=({flags: True} if flags else None)),
        )(A_x.reshape(S, D), A_wqkv, A_wo, B_w_in, B_w_sp, B_b_sp.reshape(S // T, T), B_w_out)
        return out.reshape(1, S, D)
    return fn


@jax.jit
def pallas_sequential_preLN__sliding_local_dilated__mixer_gmlp__prompt_kernel(
        A_x, A_wqkv, A_wo, B_x, B_w_in, B_w_sp, B_b_sp, B_w_out):
    return build()(A_x, A_wqkv, A_wo, B_x, B_w_in, B_w_sp, B_b_sp, B_w_out)
```

```python
import functools
import math

import numpy as np
import jax
import jax.numpy as jnp
from jax import lax
import jax.experimental.pallas as pl
import jax.experimental.pallas.tpu as pltpu

S, D, FH = 2048, 1024, 1792
H, DH, W, DIL = 32, 32, 8, 2
EPS = 1e-5
F32, BF16, I32 = jnp.float32, jnp.bfloat16, jnp.int32
T = 128
Q = 64
TM = 2 * T
NB = S // TM
PAD = 16


def _gelu(x):
    c = math.sqrt(2.0 / math.pi)
    u = x * (c + (c * 0.044715) * (x * x))
    hx = 0.5 * x
    return hx + hx * jnp.tanh(u)


def _skew(parts, axis, unit):
    return [c if i == 0 else pltpu.roll(c, unit * i, axis) for i, c in enumerate(parts)]


def _unskew(parts, axis, unit):
    n = parts[0].shape[axis]
    idx = lax.broadcasted_iota(I32, parts[0].shape, axis)
    x = [parts[-j % 8] for j in range(8)]
    for b in (1, 2, 4):
        on = (idx & (b * unit)) != 0
        x = [jnp.where(on, x[(j - b) % 8], x[j]) for j in range(8)]
    return [t if j == 0 else pltpu.roll(t, n - unit * j, axis) for j, t in enumerate(x)]


_LHS = (((1, 0, 0), (1, 1, 1)), ((1, 1, 0), (1, 1, 1)), ((1, 0, 0),), ((1, 1, 1),),
        ((1, 0, 0), (1, 0, 1)), ((1, 1, 0), (-1, 0, 0)), ((1, 0, 1), (-1, 1, 1)))
_RHS = (((1, 0, 0), (1, 1, 1)), ((1, 0, 0),), ((1, 0, 1), (-1, 1, 1)), ((1, 1, 0), (-1, 0, 0)),
        ((1, 1, 1),), ((1, 0, 0), (1, 0, 1)), ((1, 1, 0), (1, 1, 1)))


def _combine(terms, get):
    v = get(*terms[0][1:])
    for sign, a, b in terms[1:]:
        v = (lax.add if sign > 0 else lax.sub)(v, get(a, b))
    return v


def _seven(table, quad):
    return [_combine(terms, lambda a, b: quad[2 * a + b]) for terms in table]


def _sum(xs):
    return functools.reduce(lax.add, xs)


def _overlap(main, *sides):
    total, t, ev = sum(c for c, _ in main), 0.0, []
    for c, f in main:
        ev.append((t / total, 1, c, f))
        t += c
    for side, lo, hi, *due in sides:
        ev += [(when, 0, 0.0, f) for when, f in due]
        total, t = sum(c for c, _ in side), 0.0
        for c, f in side:
            ev.append((lo + (hi - lo) * t / total, 0, 0.0, f))
            t += c
    ev.sort(key=lambda e: e[:2])
    return [(e[2], e[3]) for e in ev]


def _stagger(stages):
    n, out = len(stages[0]), []
    for k in range(n + len(stages) - 1):
        now = [st[k - s] for s, st in enumerate(stages) if 0 <= k - s < n]
        now = [((j + 0.5) / len(g), s, t) for s, g in enumerate(now) for j, t in enumerate(g)]
        out += [t for _, _, t in sorted(now, key=lambda e: e[:2])]
    return out


def _tile(c):
    return slice(c * T, (c + 1) * T)


def _ds(start, n, align=8):
    if isinstance(start, int):
        return pl.ds(lax.add(np.int32(start), np.int32(0)), n)
    return pl.ds(pl.multiple_of(start, align), n)


class _Operand:
    def __init__(self, ref, base, levels, rows, nt):
        self.ref, self.base, self.levels, self.rows, self.nt = ref, base, levels, rows, nt

    @staticmethod
    def size(levels, rows, nt):
        return (7 ** levels * nt + 1) // 2 * rows // 2

    def at(self, j, r, c, n):
        g = j * self.nt + c
        return _ds(self.base + g // 2 * self.rows // 2 + r // 2, n // 2), _tile(g % 2)

    def put(self, r, c, mats, first=0):
        for j, t in enumerate(mats):
            self.ref[self.at(first + j, r, c, t.shape[0])] = pltpu.bitcast(lax.convert_element_type(t, BF16), I32)

    def col(self, j, c):
        return pltpu.bitcast(self.ref[self.at(j, 0, c, self.rows)], BF16)

    def full(self, j, zeros=()):
        cols = [self.ref[self.at(j, 0, c, self.rows)] for c in range(self.nt)]
        for z in zeros:
            cols[-1] = jnp.concatenate([cols[-1][:-8], cols[-1][-8:] | z], 0)
        return jnp.concatenate([pltpu.bitcast(c, BF16) for c in cols], 1)


_EARLY = dict(wq=(1, D // 2, 4), wk=(1, D // 2, 4), wv=(1, D // 2, 4), wo=(1, D // 2, 4),
              xa=(1, T, 4), xb=(1, T, 4), oa=(1, T, 4))
_LATE = dict(wd2=(2, 3 * T, 2), wd1=(1, T, 4), sa2=(2, Q, 4), sa1=(1, T, 8))
_BOTH = dict(win=(2, D // 4, 7), ha=(2, Q, 2), ya2=(2, Q, 3), ya1=(1, T, 1))
_Z2 = dict(z22=(2, S // 4, 3), z21=(1, S // 2, 1))


def _rows(*tables):
    return max(sum(_Operand.size(*s) for s in t.values()) for t in tables)


def build(RA=8, RB=64, RS=32, scopes=False, only=None, f1=0.4, f2=0.83, f3=0.287, fz=0.32, fx=0.8, fy=0.96,
          m1=0, m2=0, nq=2, flags=None):
    macc = (m1, m2)

    def kernel(x_hbm, wqkv_hbm, wo_hbm, win_hbm, wsp_hbm, b_hbm, wout_hbm, out_hbm,
               x_v, raw_a, raw_b, ops_v, z2_v, qk0, v0, qk1, v1, h_v, gz_v, z1_v, stat_v, acc1_v, acc2_v,
               bias_v, b_v, sems, osem, *small):
        out_v, stage_v, tmp_v = x_v, small[:8], small[8:]
        op = {}
        for ref, top, table in ((ops_v, 0, _EARLY), (ops_v, 0, _LATE), (ops_v, _rows(_EARLY, _LATE), _BOTH),
                                (z2_v, 0, _Z2)):
            for name, shape in table.items():
                op[name] = _Operand(ref, top, *shape)
                top += _Operand.size(*shape)

        zero, zero2 = lax.fori_loop(0, 2, lambda _, c: (c[1] ^ 1, c[0] ^ 1), (0, 0))
        copies, last, paced, ready, pending, turn = {}, [None], {}, {}, [], [0]

        def pace(ref):
            if last[0] is None or paced.get(id(ref)) is last[0]:
                return
            paced[id(ref)] = last[0]
            n = 8 if ref.dtype == F32 else 16
            ref[_ds(zero * n + (ref.shape[0] - n), n, n), 0:T] = last[0][0:n].astype(ref.dtype)

        for ref in (ops_v, z2_v):
            ref[_ds(ref.shape[0] - 8, 8), 0:T] = jnp.zeros((8, T), I32)

        def due(ref, when):
            return when, lambda: pending.append(ref[_ds(zero * 8 + (ref.shape[0] - 8), 8), 0:T])

        def start(key, src, dst):
            copies[key] = pltpu.make_async_copy(src, dst, sems.at[len(copies)])
            copies[key].start()

        class Partial:
            def __init__(self, level, base, rows):
                self.level, self.base, self.rows, self.v = level, base, rows, {}

            def __setitem__(self, n, v):
                if n < macc[self.level - 1]:
                    (acc1_v, acc2_v)[self.level - 1][_ds(zero * 8 + self.base + n * self.rows, self.rows), :] = v
                else:
                    self.v[n] = v

            def __getitem__(self, n):
                if n < macc[self.level - 1]:
                    return (acc1_v, acc2_v)[self.level - 1][_ds(zero2 * 8 + self.base + n * self.rows, self.rows), :]
                return self.v[n]

        def unit(lhs, rhs, u, emit, level=None, first=0):
            level = lhs.levels if level is None else level
            if level == 0:
                def run():
                    last[0] = jnp.dot(lhs.full(first, pending), rhs.col(first, u), preferred_element_type=F32)
                    pending.clear()
                    emit(0, 0, last[0])
                return [(rhs.rows * lhs.rows / (4 * T), run)]
            h = 2 ** (level - 1)
            state = {(i, j): Partial(level, (i * h + j) * 2 * lhs.rows, lhs.rows) for i in range(h) for j in range(h)}

            def step(n):
                def take(i, j, m):
                    s = state[i, j]
                    if n == 0:
                        s[0] = m
                    elif n == 1:
                        s[0], s[1] = s[0] + m, m
                    elif n == 2:
                        emit(h + i, j, m + s[1])
                        s[1] = m
                    elif n == 3:
                        s[0], s[1] = s[0] + m, m - s[1]
                    elif n == 4:
                        emit(i, j, s[0] - m)
                        s[0] = m
                    elif n == 5:
                        emit(i, h + j, m + s[0])
                        s[1] = s[1] + m
                    else:
                        emit(h + i, h + j, s[1] + m)
                return take
            return [t for n, r in enumerate((6, 3, 1, 0, 4, 2, 5))
                    for t in unit(lhs, rhs, u, step(n), level - 1, first * 7 + r)]

        def expand2(table, ref, get, dst, r, c):
            def task(r1):
                def run():
                    pace(ref)
                    quad = [_combine(table[r1], lambda a, b: get(2 * a + i, 2 * b + j)) for i in (0, 1) for j in (0, 1)]
                    dst.put(r, c, _seven(table, quad), 7 * r1)
                return (3, run)
            return [task(r1) for r1 in (6, 3, 1, 0, 4, 2, 5)]

        def staged2(table, src, make, cost, dst, jobs, pair):
            fill, use = [], []
            for n, job in enumerate(jobs):
                ref = tmp_v[2 * pair + n % 2]

                def task(a, job=job, ref=ref):
                    def run():
                        pace(src)
                        for b, t in enumerate(make(job, a)):
                            ref[_ds((4 * a + b) * 16, 16), :] = t
                    return (cost, run)
                fill.append([task(a) for a in range(4)])
                use.append(expand2(table, ref, lambda a, b, ref=ref: ref[_ds((4 * a + b) * 16, 16), :], dst, *job[:2]))
            return _stagger([fill, use])

        def ln_stats(src, load, nt, stat):
            def mean(r):
                def run():
                    pace(src)
                    m = jnp.sum(_sum([load(r, c, RS) for c in range(nt)]), axis=-1, keepdims=True) * (1.0 / (nt * T))
                    stat_v[_ds(stat + r, RS), :] = jnp.broadcast_to(m, (RS, T))
                return (nt * RS / 64, run)

            def rstd(r):
                def run():
                    pace(src)
                    m = stat_v[_ds(stat + r, RS), :]
                    v = [load(r, c, RS) - m for c in range(nt)]
                    var = jnp.sum(_sum([t * t for t in v]), axis=-1, keepdims=True) * (1.0 / (nt * T))
                    stat_v[_ds(stat + TM + r, RS), :] = jnp.broadcast_to(lax.rsqrt(var + EPS), (RS, T))
                return (3 * nt * RS / 64, run)

            def norm(r, cs):
                m, inv = stat_v[_ds(stat + r, 16), :], stat_v[_ds(stat + TM + r, 16), :]
                return [(load(r, c, 16) - m) * inv for c in cs]
            return _stagger([[[f(g)] for g in range(0, TM, RS)] for f in (mean, rstd)]), norm

        def ln_x(i, dst):
            stats, norm = ln_stats(x_v, lambda r, c, n: x_v[_ds(i * TM + r, n, 16), _tile(c)].astype(F32), 8, 0)

            def task(r, c):
                def run():
                    pace(x_v)
                    dst.put(r, c, _seven(_LHS, norm(r, (c, 4 + c)) + norm(T + r, (c, 4 + c))))
                return (5, run)
            return stats + [task(r, c) for r in range(0, T, 16) for c in range(4)]

        def ln_h(i):
            stats, norm = ln_stats(h_v, lambda r, c, n: h_v[_ds(c * S + i * TM + r, n), :], 8, 2 * TM)
            return stats + staged2(_LHS, h_v, lambda job, a: norm(a * Q + job[0], range(job[1], 8, 2)), 2, op['ha'],
                                   [(r, c) for c in range(2) for r in range(0, Q, 16)], 0)

        def ln_z(i):
            stats, norm = ln_stats(gz_v, lambda r, c, n: gz_v[_ds(c * TM + r, n), :], 14, 4 * TM)

            def task(r):
                def run():
                    pace(gz_v)
                    op['z21'].put(i * T + r, 0, _seven(_RHS, norm(r, (12, 13)) + norm(T + r, (12, 13))))
                return (4, run)
            return stats + [task(r) for r in range(0, T, 16)] + staged2(
                _RHS, gz_v, lambda job, a: norm(a * Q + job[2], range(job[1], 12, 3)), 2, op['z22'],
                [(i * Q + r, c, r) for c in range(3) for r in range(0, Q, 16)], 0)

        def raw_tile(ref, r, c):
            return ref[_ds(r, 16, 16), _tile(c)]

        def win_prep(units):
            return staged2(_RHS, raw_b, lambda job, a: [
                raw_tile(raw_b, a * (D // 4) + job[0], 7 * b + job[1]).astype(F32) for b in range(4)],
                1.5, op['win'], [(r, u) for u in units for r in range(0, D // 4, 16)], 1)

        def wd_prep():
            def get(k, r, c):
                return raw_tile(raw_b, k % 7 * T + r, k // 7 * 8 + c).astype(F32)

            def task(r, c):
                def run():
                    pace(raw_b)
                    op['wd1'].put(r, c, _seven(_RHS, [get(k, r, cc) for k in (12, 13) for cc in (c, 4 + c)]))
                return (3.5, run)
            return [task(r, c) for c in range(4) for r in range(0, T, 16)] + staged2(
                _RHS, raw_b, lambda job, a: [get(3 * a + job[0] // T, job[0] % T, 2 * b + job[1]) for b in range(4)],
                1.5, op['wd2'], [(r, u) for u in range(2) for r in range(0, 3 * T, 16)], 1)

        def sp_prep1(i):
            def task(r, b):
                def run():
                    pace(raw_a)
                    op['sa1'].put(r, b, _seven(_LHS, [raw_tile(raw_a, i * TM + a + r, 2 * b + cc).astype(F32)
                                                      for a in (0, T) for cc in (0, 1)]))
                return (3.5, run)
            return [task(r, b) for b in range(NB) for r in range(0, T, 16)]

        def sp_prep2(i):
            def make(job, a):
                low = lax.broadcasted_iota(I32, (8, T), 1) < Q
                out = []
                for cc in (0, 1):
                    u, v = (pltpu.bitcast(raw_tile(raw_a, i * TM + a * Q + job[0], 4 * job[1] + 2 * k + cc), I32)
                            for k in (0, 1))
                    out += [jnp.where(low, u, pltpu.roll(v, Q, 1)), jnp.where(low, pltpu.roll(u, Q, 1), v)]
                return [pltpu.bitcast(t, BF16).astype(F32) for t in out]
            return staged2(_LHS, raw_a, make, 2, op['sa2'], [(r, c) for c in range(4) for r in range(0, Q, 16)], 1)

        def qkv_prep(t, lo=0, hi=D // 2):
            val = {}

            def skew(r):
                def run():
                    pace(raw_a)
                    val[r] = _skew([pltpu.bitcast(raw_tile(raw_a, t // 2 * D + r, t % 2 * 8 + c), I32)
                                    for c in range(8)], 1, 2)
                return (2, run)

            def unskew(r):
                def run():
                    val[r] = _unskew(val[r], 1, 2)
                return (4, run)

            def store(r0):
                def run():
                    hv = [[pltpu.bitcast(p, BF16).astype(F32) for p in val[r]] for r in (r0, D // 2 + r0)]
                    for c in range(4):
                        op['w' + 'qkv'[t]].put(r0, c, _seven(_RHS, [hv[0][c], hv[0][4 + c], hv[1][c], hv[1][4 + c]]))
                return (12, run)
            rs = [a + r for r in range(lo, hi, 16) for a in (0, D // 2)]
            return _stagger([[[skew(r)] for r in rs], [[unskew(r)] for r in rs],
                             [[store(r - D // 2)] if r >= D // 2 else [] for r in rs]])

        def wo_prep():
            def task(g, c):
                def run():
                    pace(raw_a)
                    hv = [[pltpu.bitcast(p, BF16).astype(F32) for p in _unskew(_skew(
                        [pltpu.bitcast(raw_tile(raw_a, D + i * T + g, 8 + cc), I32) for i in range(8)], 0, 1), 0, 1)]
                        for cc in (c, 4 + c)]
                    for j in range(4):
                        op['wo'].put(j * T + g, c, _seven(_RHS, [hv[0][j], hv[1][j], hv[0][4 + j], hv[1][4 + j]]))
                return (22, run)
            return [task(g, c) for c in range(4) for g in range(0, T, 16)]

        def row(c, r):
            return c * (TM + PAD) + PAD + r

        def qkv(i, lhs, bufs, which):
            tasks = []
            for t in which:
                for u in range(4):
                    def emit(a, b, v, t=t, u=u):
                        ref, c = bufs[t // 2], t % 2 * 8 + 4 * b + u
                        ref[_ds(row(c, a * T), T), :] = v
                        ready[id(ref)] = t > 0 and (u, a, b) == (3, 1, 1)
                        if t and a == 0 and isinstance(i, int) and i == 0:
                            ref[_ds(row(c, -PAD), PAD), :] = jnp.broadcast_to(v[0:1], (PAD, T))
                    tasks += unit(lhs, op['w' + 'qkv'[t]], u, emit)
            return tasks

        def history(src, dst, which=(1, 2)):
            for t in which:
                for c in range(t % 2 * 8, t % 2 * 8 + 8):
                    dst[t // 2][_ds(row(c, -PAD), PAD), :] = src[t // 2][_ds(row(c, TM - PAD), PAD), :]

        def slot(stage, w, r):
            return stage_v[2 * stage + r // RB % 2], (w * 2 + r // T) * RB + r % RB

        def att(bufs, first=False):
            scale = DH ** -0.5
            qk, v = bufs

            def grab(stage, r):
                pace(slot(stage, 0, r)[0])
                return [ref[_ds(o, RA), :] for ref, o in (slot(stage, w, r) for w in range(W))]

            def drop(stage, r, vals):
                for w, t in enumerate(vals):
                    ref, o = slot(stage, w, r)
                    ref[_ds(o, RA), :] = t

            def scores(r):
                def run():
                    assert ready[id(qk)]
                    pace(qk)
                    q = [qk[_ds(row(c, r), RA), :] for c in range(8)]
                    drop(0, r, (_sum([lax.mul(q[c], qk[_ds(row(8 + c, r - DIL * w), RA), :]) for c in range(8)])
                                for w in range(W)))
                return (15 * RA / 8, run)

            def fold(r):
                def run():
                    lane = lax.broadcasted_iota(I32, (RA, T), 1)
                    ps = grab(0, r)
                    for bit in (16, 1):
                        low = (lane & bit) == 0
                        ps = [p + jnp.where(low, pltpu.roll(p, T - bit, 1), pltpu.roll(p, bit, 1)) for p in ps]
                    if first and r < DIL * W:
                        pos = lax.broadcasted_iota(I32, (RA, T), 0) + r
                        ps = [jnp.where(pos >= DIL * w, p, -1e9 / scale) for w, p in enumerate(ps)]
                    drop(1, r, ps)
                return (8 * RA / 8, run)

            def softmax(r):
                def run():
                    lg = grab(1, r)
                    m = functools.reduce(jnp.maximum, lg)
                    e = [jnp.exp2((p - m) * (scale * math.log2(math.e))) for p in lg]
                    inv = 1.0 / _sum(e)
                    drop(2, r, [t * inv for t in e])
                return (7 * RA / 8, run)

            def mix(r):
                def run():
                    assert ready[id(v)]
                    pace(v)
                    p = grab(2, r)
                    drop(3, r, (_sum([lax.mul(p[w], v[_ds(row(c, r - DIL * w), RA), :]) for w in range(W)])
                                for c in range(8)))
                return (15 * RA / 8, run)

            def combo(r):
                def run():
                    pace(slot(3, 0, r)[0])
                    for c in range(4):
                        op['oa'].put(r, c, _seven(_LHS, [ref[_ds(o, 16), :] for ref, o in (
                            slot(3, cc, a + r) for a in (0, T) for cc in (c, 4 + c))]))
                return (8, run)
            gs = range(0, T, RB)
            return _stagger([[[f(a + r) for a in (0, T) for r in range(g, g + RB, RA)] for g in gs]
                             for f in (scores, fold, softmax, mix)] + [
                [[combo(r) for r in range(g, g + RB, 16)] for g in gs]])

        def proj(i):
            tasks = []
            for u in range(4):
                def emit(a, b, v, u=u):
                    c, r = 4 * b + u, i * TM + a * T
                    h_v[_ds(c * S + r, T), :] = x_v[_ds(r, T, 16), _tile(c)].astype(F32) + v
                tasks += unit(op['oa'], op['wo'], u, emit)
            return tasks

        def z1_at(i, c, r, n):
            return _ds((c // 2 * S + i * TM + r) // 2, n // 2), _tile(c % 2)

        def up(i):
            tasks = []
            for u in range(7):
                def emit(a, b, v, u=u):
                    c = 7 * (b % 2) + u
                    if b < 2:
                        z1_v[z1_at(i, c, a * Q, Q)] = pltpu.bitcast(_gelu(v).astype(BF16), I32)
                    else:
                        gz_v[_ds(c * TM + a * Q, Q), :] = _gelu(v)
                tasks += unit(op['ha'], op['win'], u, emit)
            return tasks

        def bias_prep():
            def task(k):
                def run():
                    bias_v[_ds(k * T, T), :] = jnp.broadcast_to(b_v[...].astype(F32)[k:k + 1, :], (T, T)).T
                return (4, run)
            return [task(k) for k in range(S // T)]

        def gate_step(i, _):
            last[0] = None
            y_v = (qk0, qk1)

            def gated(c, r, v):
                z = pltpu.bitcast(z1_v[z1_at(i, c, r, v.shape[0])], BF16).astype(F32)
                return z * (v + bias_v[_ds(i * TM + r, v.shape[0]), :])

            y = {}

            def emit1(a, b, v):
                y[a, b] = gated(12 + b, a * T, v)
                if len(y) == 4:
                    op['ya1'].put(0, 0, _seven(_LHS, [y[0, 0], y[0, 1], y[1, 0], y[1, 1]]))
            main, sides = unit(op['sa1'], op['z21'], 0, emit1), []
            for u in range(3):
                def emit2(a, b, v, u=u):
                    y_v[u % 2][_ds((4 * a + b) * Q, Q), :] = gated(3 * b + u, a * Q, v)
                main += unit(op['sa2'], op['z22'], u, emit2)
                side = []
                for r in range(0, Q, 16):
                    side.append(expand2(_LHS, y_v[u % 2], lambda a, b, r=r, u=u: y_v[u % 2][
                        _ds((4 * a + b) * Q + r, 16), :], op['ya2'], r, u))
                t0 = (1792 + (u + 1) * 3136 + 1) / 16800
                sides.append(([t for ts in zip(*side) for t in ts], t0, t0 + (0.15 if u < 2 else 0.045)))
            for u in range(4):
                def emit3(a, b, v, u=u):
                    at = _ds((4 * b + u) * S + i * TM + a * T, T)
                    h_v[at, :] = h_v[at, :] + v
                main += unit(op['ya1'], op['wd1'], u, emit3)
            for u in range(2):
                def emit4(a, b, v, u=u):
                    c, r = 2 * b + u, i * TM + a * Q
                    out_v[_ds(r, Q, 16), _tile(c)] = (h_v[_ds(c * S + r, Q), :] + v).astype(BF16)
                main += unit(op['ya2'], op['wd2'], u, emit4)
            nxt = jnp.minimum(i + 1, NB - 1)
            go('p2', _overlap(main, *sides, (sp_prep1(nxt), 0.11, 0.6), (sp_prep2(nxt), 0.72, 0.96, due(ops_v, 0.99))))
            rows = _ds(i * TM, TM, 16)
            pltpu.make_async_copy(out_v.at[rows], out_hbm.at[rows], osem).start()
            last[0] = None

        def go(name, tasks):
            if scopes:
                with jax.named_scope(name):
                    for _, f in tasks:
                        f()
            else:
                for _, f in tasks:
                    f()

        def wait(*keys):
            for k in keys:
                copies[k].wait()

        first, cur = (qk1, v1), (qk0, v0)

        def mixer_step(i, _):
            last[0] = None
            history(cur, cur)
            go('p1', _overlap(
                qkv(i, op['xa'], cur, (0, 1, 2)) + up(i - 1) + proj(i),
                (ln_z(i - 2) + ln_h(i - 1), 0.0, f1, due(z2_v, fz)), (att(cur), f3, f2),
                (ln_x(jnp.minimum(i + 1, NB - 1), op['xa']), fx, fy, due(ops_v, 0.99))))
            last[0] = None

        if only:
            lax.fori_loop(2, NB, mixer_step if only == 1 else gate_step, None)
            dyn = _ds(zero * 16, 16)
            out_v[0:16, 0:T] = (h_v[dyn, :] + gz_v[dyn, :] + (z2_v[dyn, 0:T] + z1_v[dyn, 0:T] + ops_v[dyn, 0:T]).astype(F32)).astype(BF16)
            pltpu.make_async_copy(out_v.at[0:S], out_hbm, osem).start()
            pltpu.make_async_copy(out_v.at[0:S], out_hbm, osem).wait()
            return

        start('x0', x_hbm.at[0:TM], x_v.at[0:TM])
        QC = D // 2 // nq
        for k in range(nq):
            for a in (0, D // 2):
                start(('q', k, a), wqkv_hbm.at[a + k * QC:a + (k + 1) * QC, 0:D],
                      raw_a.at[a + k * QC:a + (k + 1) * QC, 0:D])
        start('k', wqkv_hbm.at[:, D:2 * D], raw_a.at[0:D, D:2 * D])
        start('v', wqkv_hbm.at[:, 2 * D:], raw_a.at[D:2 * D, 0:D])
        start('x1', x_hbm.at[TM:2 * TM], x_v.at[TM:2 * TM])
        start('wo', wo_hbm, raw_a.at[D:2 * D, D:2 * D])
        start('win', win_hbm, raw_b.at[0:D])
        start('x', x_hbm.at[2 * TM:], x_v.at[2 * TM:S])
        start('b', b_hbm, b_v)

        wait('x0')
        go('lnx', ln_x(0, op['xa']))
        for k in range(nq):
            wait(('q', k, 0), ('q', k, D // 2))
            go('wq', qkv_prep(0, k * QC, (k + 1) * QC))
        wait('k')
        go('q0', _overlap(qkv(0, op['xa'], first, (0,)), (qkv_prep(1), 0.0, 0.9)))
        wait('v', 'x1')
        go('k0', _overlap(qkv(0, op['xa'], first, (1,)), (qkv_prep(2), 0.0, 0.9)))
        wait('wo')
        main = qkv(0, op['xa'], first, (2,)) + [(0, lambda: history(first, cur))] + qkv(1, op['xb'], cur, (0, 1))
        go('s1', _overlap(main, (ln_x(1, op['xb']), 0.0, 0.28), (att(first, True), 0.1, 0.93),
                          (wo_prep(), 0.0, 0.9)))
        wait('win')
        go('s2', _overlap(proj(0) + qkv(1, op['xb'], cur, (2,)),
                          (win_prep(range(3)), 0.0, 0.95), (ln_h(0), 0.51, 0.92)))
        wait('x', 'b')
        go('s3', _overlap(up(0) + proj(1), (win_prep(range(3, 7)), 0.0, 0.6), (att(cur), 0.0, 0.72),
                          (ln_x(2, op['xa']), 0.7, 0.95, due(ops_v, 0.98))))
        start('wsp', wsp_hbm, raw_a.at[0:S])
        for k in range(2):
            start(('wd', k), wout_hbm.at[k * FH // 2:(k + 1) * FH // 2], raw_b.at[0:FH // 2, k * D:(k + 1) * D])
        lax.fori_loop(2, NB, mixer_step, None)
        wait('wsp', ('wd', 0), ('wd', 1))
        go('t0', ln_z(NB - 2) + ln_h(NB - 1))
        go('t1', _overlap(up(NB - 1), (wd_prep() + sp_prep1(0) + sp_prep2(0) + bias_prep(), 0.0, 0.95,
                                       due(ops_v, 0.985))))
        last[0] = None
        go('t2', ln_z(NB - 1))
        lax.fori_loop(0, NB, gate_step, None)
        pltpu.make_async_copy(out_v.at[0:S], out_hbm, osem).wait()

    def fn(A_x, A_wqkv, A_wo, B_x, B_w_in, B_w_sp, B_b_sp, B_w_out):
        del B_x
        hbm = pl.BlockSpec(memory_space=pl.ANY)
        vm = pltpu.VMEM
        out = pl.pallas_call(
            kernel,
            out_shape=jax.ShapeDtypeStruct((S, D), BF16),
            in_specs=[hbm] * 7,
            out_specs=hbm,
            scratch_shapes=[
                vm((S + PAD, D), BF16), vm((S + PAD, S), BF16), vm((D + PAD, 2 * FH), BF16),
                vm((_rows(_EARLY, _LATE) + _rows(_BOTH) + 8, 2 * T), I32), vm((_rows(_Z2) + 8, 2 * T), I32),
                *[vm((n * (TM + PAD) + PAD, T), F32) for n in (16, 8, 16, 8)],
                vm((8 * S + PAD, T), F32), vm((14 * TM + PAD, T), F32), vm((7 * S // 2, 2 * T), I32),
                vm((6 * TM, T), F32), vm((2 * T, T), F32), vm((8 * Q, T), F32),
                vm((S, T), F32), vm((S // T, T), BF16),
                pltpu.SemaphoreType.DMA((24,)), pltpu.SemaphoreType.DMA(()),
                *[vm((16 * RB + 8, T), F32)] * 8, *[vm((16 * 16 + 8, T), F32)] * 4,
            ],
            compiler_params=pltpu.CompilerParams(vmem_limit_bytes=124 * 1024 * 1024,
                                                 flags=({flags: True} if flags else None)),
        )(A_x.reshape(S, D), A_wqkv, A_wo, B_w_in, B_w_sp, B_b_sp.reshape(S // T, T), B_w_out)
        return out.reshape(1, S, D)
    return fn


@jax.jit
def pallas_sequential_preLN__sliding_local_dilated__mixer_gmlp__prompt_kernel(
        A_x, A_wqkv, A_wo, B_x, B_w_in, B_w_sp, B_b_sp, B_w_out):
    return build()(A_x, A_wqkv, A_wo, B_x, B_w_in, B_w_sp, B_b_sp, B_w_out)
```

```python
import functools
import math

import numpy as np
import jax
import jax.numpy as jnp
from jax import lax
import jax.experimental.pallas as pl
import jax.experimental.pallas.tpu as pltpu

S, D, FH = 2048, 1024, 1792
H, DH, W, DIL = 32, 32, 8, 2
EPS = 1e-5
F32, BF16, I32 = jnp.float32, jnp.bfloat16, jnp.int32
T = 128
Q = 64
TM = 2 * T
NB = S // TM
PAD = 16


def _gelu(x):
    c = math.sqrt(2.0 / math.pi)
    u = x * (c + (c * 0.044715) * (x * x))
    hx = 0.5 * x
    return hx + hx * jnp.tanh(u)


def _skew(parts, axis, unit):
    return [c if i == 0 else pltpu.roll(c, unit * i, axis) for i, c in enumerate(parts)]


def _unskew(parts, axis, unit):
    n = parts[0].shape[axis]
    idx = lax.broadcasted_iota(I32, parts[0].shape, axis)
    x = [parts[-j % 8] for j in range(8)]
    for b in (1, 2, 4):
        on = (idx & (b * unit)) != 0
        x = [jnp.where(on, x[(j - b) % 8], x[j]) for j in range(8)]
    return [t if j == 0 else pltpu.roll(t, n - unit * j, axis) for j, t in enumerate(x)]


_LHS = (((1, 0, 0), (1, 1, 1)), ((1, 1, 0), (1, 1, 1)), ((1, 0, 0),), ((1, 1, 1),),
        ((1, 0, 0), (1, 0, 1)), ((1, 1, 0), (-1, 0, 0)), ((1, 0, 1), (-1, 1, 1)))
_RHS = (((1, 0, 0), (1, 1, 1)), ((1, 0, 0),), ((1, 0, 1), (-1, 1, 1)), ((1, 1, 0), (-1, 0, 0)),
        ((1, 1, 1),), ((1, 0, 0), (1, 0, 1)), ((1, 1, 0), (1, 1, 1)))


def _combine(terms, get):
    v = get(*terms[0][1:])
    for sign, a, b in terms[1:]:
        v = (lax.add if sign > 0 else lax.sub)(v, get(a, b))
    return v


def _seven(table, quad):
    return [_combine(terms, lambda a, b: quad[2 * a + b]) for terms in table]


def _sum(xs):
    return functools.reduce(lax.add, xs)


def _overlap(main, *sides):
    total, t, ev = sum(c for c, _ in main), 0.0, []
    for c, f in main:
        ev.append((t / total, 1, c, f))
        t += c
    for side, lo, hi, *due in sides:
        ev += [(when, 0, 0.0, f) for d in due for when, f in d]
        total, t = sum(c for c, _ in side), 0.0
        for c, f in side:
            ev.append((lo + (hi - lo) * t / total, 0, 0.0, f))
            t += c
    ev.sort(key=lambda e: e[:2])
    return [(e[2], e[3]) for e in ev]


def _stagger(stages):
    n, out = len(stages[0]), []
    for k in range(n + len(stages) - 1):
        now = [st[k - s] for s, st in enumerate(stages) if 0 <= k - s < n]
        now = [((j + 0.5) / len(g), s, t) for s, g in enumerate(now) for j, t in enumerate(g)]
        out += [t for _, _, t in sorted(now, key=lambda e: e[:2])]
    return out


def _zip(*lists):
    return [t for step in zip(*lists) for part in step for t in part]


def _tile(c):
    return slice(c * T, (c + 1) * T)


def _ds(start, n, align=8):
    if isinstance(start, int):
        return pl.ds(lax.add(np.int32(start), np.int32(0)), n)
    return pl.ds(pl.multiple_of(start, align), n)


class _Operand:
    def __init__(self, ref, base, levels, rows, nt):
        self.ref, self.base, self.levels, self.rows, self.nt = ref, base, levels, rows, nt

    @staticmethod
    def size(levels, rows, nt):
        return (7 ** levels * nt + 1) // 2 * rows // 2

    def shifted(self, i, step):
        size = self.size(self.levels, self.rows, self.nt) - (self.rows - step) // 2
        return _Operand(self.ref.at[_ds(self.base + i * (step // 2), size)], 0, self.levels, self.rows, self.nt)

    def at(self, j, r, c, n):
        g = j * self.nt + c
        return _ds(self.base + g // 2 * self.rows // 2 + r // 2, n // 2), _tile(g % 2)

    def put(self, r, c, mats, first=0):
        for j, t in enumerate(mats):
            self.ref[self.at(first + j, r, c, t.shape[0])] = pltpu.bitcast(lax.convert_element_type(t, BF16), I32)

    def col(self, j, c, ks):
        return pltpu.bitcast(self.ref[self.at(j, ks[0] * T, c, len(ks) * T)], BF16)

    def full(self, j, ks, r, n, zeros=()):
        cols = [self.ref[self.at(j, r, c, n)] for c in ks]
        for z in zeros:
            cols[-1] = jnp.concatenate([cols[-1][:-8], cols[-1][-8:] | z], 0)
        return jnp.concatenate([pltpu.bitcast(c, BF16) for c in cols], 1)


_EARLY = dict(wq=(1, D // 2, 4), wk=(1, D // 2, 4), wv=(1, D // 2, 4), wo=(1, D // 2, 4),
              xa=(1, T, 4), xb=(1, T, 4), oa=(1, T, 4))
_LATE = dict(wd2=(2, 3 * T, 2), wd1=(1, T, 4), sa2=(2, Q, 4), sa1=(1, T, 8))
_BOTH = dict(win=(2, D // 4, 7), ha=(2, Q, 2), ya2=(2, Q, 3), ya1=(1, T, 1))
_Z2 = dict(z22=(2, S // 4, 3), z21=(1, S // 2, 1))


def _rows(*tables):
    return max(sum(_Operand.size(*s) for s in t.values()) for t in tables)


def build(RA=8, RB=64, RS=16, scopes=False, only=None, m1=0, m2=0, nq=2, mrows=128, stage_w=False, cut=2, G=32, grouped=False, direct=True, wm=2,
          flags=None, **tune):
    F = tune.get
    macc = (m1, m2)

    def kernel(x_hbm, wqkv_hbm, wo_hbm, win_hbm, wsp_hbm, b_hbm, wout_hbm, out_hbm,
               x_v, raw_a, raw_b, ops_v, mlp_v, z2_v, p_v, qk0, v0, qk1, v1, h_v, gz_v, z1_v, stat_v,
               bias_v, b_v, sems, osem, bar, *small):
        out_v, stage_v, tmp_v = x_v, small[:8], small[8:14]
        perm_v, acc_v = small[14:18], small[18:]
        op = {}
        for ref, top, table in ((ops_v, 0, _EARLY), (ops_v, 0, _LATE), (mlp_v, 0, _BOTH),
                                (z2_v, 0, _Z2)):
            for name, shape in table.items():
                op[name] = _Operand(ref, top, *shape)
                top += _Operand.size(*shape)

        op['hb'] = _Operand(mlp_v, op['ya2'].base, 2, Q, 2)

        zero, zero2 = lax.fori_loop(0, 2, lambda _, c: (c[1] ^ 1, c[0] ^ 1), (0, 0))
        copies, last, paced, ready, pending, turn = {}, [None], {}, {}, [], [0]

        def pace(ref):
            if last[0] is None or paced.get(id(ref)) is last[0]:
                return
            paced[id(ref)] = last[0]
            n = 8 if ref.dtype == F32 else 16
            ref[_ds(zero * n + (ref.shape[0] - n), n, n), 0:T] = last[0][0:n].astype(ref.dtype)

        for ref in (ops_v, mlp_v, z2_v):
            ref[_ds(ref.shape[0] - 8, 8), 0:T] = jnp.zeros((8, T), I32)

        p_v[_ds(W * TM, 8), :] = jnp.zeros((8, T), F32)

        def due(ref, *times):
            def run():
                if ref is p_v:
                    return pending.append(pltpu.bitcast(p_v[_ds(zero * 8 + W * TM, 8), :], I32))
                pending.append(ref[_ds(zero * 8 + (ref.shape[0] - 8), 8), 0:T])
            return [(when, run) for when in times]

        def start(key, src, dst):
            copies[key] = pltpu.make_async_copy(src, dst, sems.at[len(copies)])
            if not only:
                copies[key].start()

        class Partial:
            def __init__(self, level, base, rows):
                self.level, self.base, self.rows, self.v = level, base + 8 * (2 - level), rows, {}

            def __setitem__(self, n, v):
                if n < macc[self.level - 1]:
                    acc_v[self.base + n][_ds(zero * 8, self.rows), :] = v
                else:
                    self.v[n] = v

            def __getitem__(self, n):
                if n < macc[self.level - 1]:
                    return acc_v[self.base + n][_ds(zero2 * 8, self.rows), :]
                return self.v[n]

        def unit(lhs, rhs, u, emit, ks=None):
            n = min(lhs.rows, mrows)
            return [t for r in range(0, lhs.rows, n) for t in products(
                lhs, rhs, u, lambda a, b, v, r=r: emit(a * lhs.rows + r, b, v), ks or range(lhs.nt), r, n, lhs.levels, 0)]

        def products(lhs, rhs, u, emit, ks, r0, rows, level, first):
            if level == 0:
                def run():
                    last[0] = jnp.dot(lhs.full(first, ks, r0, rows, pending), rhs.col(first, u, ks), preferred_element_type=F32)
                    pending.clear()
                    emit(0, 0, last[0])
                return [(len(ks) * rows / 4, run)]
            h = 2 ** (level - 1)
            state = {(i, j): Partial(level, (i * h + j) * 2, rows) for i in range(h) for j in range(h)}

            def step(n):
                def take(i, j, m):
                    s = state[i, j]
                    if n == 0:
                        s[0] = m
                    elif n == 1:
                        s[0], s[1] = s[0] + m, m
                    elif n == 2:
                        emit(h + i, j, m + s[1])
                        s[1] = m
                    elif n == 3:
                        s[0], s[1] = s[0] + m, m - s[1]
                    elif n == 4:
                        emit(i, j, s[0] - m)
                        s[0] = m
                    elif n == 5:
                        emit(i, h + j, m + s[0])
                        s[1] = s[1] + m
                    else:
                        emit(h + i, h + j, s[1] + m)
                return take
            return [t for n, r in enumerate((6, 3, 1, 0, 4, 2, 5))
                    for t in products(lhs, rhs, u, step(n), ks, r0, rows, level - 1, first * 7 + r)]

        def expand2(table, ref, get, dst, r, c):
            def task(group):
                def run():
                    pace(ref)
                    load = functools.cache(get)
                    for r1 in group:
                        quad = [_combine(table[r1], lambda a, b: load(2 * a + i, 2 * b + j))
                                for i in (0, 1) for j in (0, 1)]
                        dst.put(r, c, _seven(table, quad), 7 * r1)
                return (3 * len(group), run)
            if not grouped:
                return [task([r1]) for r1 in (6, 3, 1, 0, 4, 2, 5)]
            return [task(g) for g in (((3, 6, 1), (2, 4, 5, 0)) if table is _LHS else ((4, 6, 2), (1, 3, 5, 0)))]

        def staged2(table, src, make, cost, dst, jobs, pair):
            if direct and src is not raw_a:
                return [t for job in jobs for t in expand2(
                    table, src, lambda a, b, job=job: make(job, a, [b])[0], dst, *job)]
            fill, use = [], []
            for n, job in enumerate(jobs):
                ref = tmp_v[2 * pair + n % 2]

                def task(a, job=job, ref=ref):
                    def run():
                        pace(src)
                        for b, t in enumerate(make(job, a)):
                            ref[_ds((4 * a + b) * 16, 16), :] = t
                    return (cost, run)
                fill.append([task(a) for a in range(4)])
                use.append(expand2(table, ref, lambda a, b, ref=ref: ref[_ds((4 * a + b) * 16, 16), :], dst, *job[:2]))
            return _stagger([fill, use])

        def ln_stats(src, load, nt, stat):
            def mean(r):
                def run():
                    pace(src)
                    m = jnp.sum(_sum([load(r, c, RS) for c in range(nt)]), axis=-1, keepdims=True) * (1.0 / (nt * T))
                    stat_v[_ds(stat + r, RS), :] = jnp.broadcast_to(m, (RS, T))
                return (wm * nt * RS / 64, run)

            def rstd(r):
                def run():
                    pace(src)
                    m = stat_v[_ds(stat + r, RS), :]
                    v = [load(r, c, RS) - m for c in range(nt)]
                    var = jnp.sum(_sum([t * t for t in v]), axis=-1, keepdims=True) * (1.0 / (nt * T))
                    stat_v[_ds(stat + TM + r, RS), :] = jnp.broadcast_to(lax.rsqrt(var + EPS), (RS, T))
                return (3 * nt * RS / 64, run)

            def norm(r, cs):
                m, inv = stat_v[_ds(stat + r, 16), :], stat_v[_ds(stat + TM + r, 16), :]
                return [(load(r, c, 16) - m) * inv for c in cs]
            return [[f(g) for g in range(0, TM, RS)] for f in (mean, rstd)], norm

        def x_blk(i):
            return x_v.at[_ds(i * TM, TM, 16)]

        def h_blk(i):
            return h_v.at[_ds(i * TM, 7 * S + TM)]

        def ln_x(i, dst):
            x = x_blk(i)
            stats, norm = ln_stats(x_v, lambda r, c, n: x[_ds(r, n), _tile(c)].astype(F32), 8, 0)

            def task(r, c):
                def run():
                    pace(x_v)
                    dst.put(r, c, _seven(_LHS, norm(r, (c, 4 + c)) + norm(T + r, (c, 4 + c))))
                return (5, run)
            return stats[0] + stats[1], [task(r, c) for r in range(0, T, 16) for c in range(4)]

        def ln_h(i, dst):
            h = h_blk(i)
            stats, norm = ln_stats(h_v, lambda r, c, n: h[_ds(c * S + r, n), :], 8, 2 * TM)
            return stats + [staged2(_LHS, h_v, lambda job, a, bs=range(4): norm(a * Q + job[0], [job[1] + 2 * b for b in bs]), 2, dst,
                                   [(r, c) for c in range(2) for r in range(0, Q, 16)], 2)]

        def ln_z(i, gz_v):
            stats, norm = ln_stats(gz_v, lambda r, c, n: gz_v[_ds(c * TM + r, n), :], 14, 4 * TM)
            z21, z22 = op['z21'].shifted(i, T), op['z22'].shifted(i, Q)

            def task(r):
                def run():
                    pace(gz_v)
                    z21.put(r, 0, _seven(_RHS, norm(r, (12, 13)) + norm(T + r, (12, 13))))
                return (4, run)
            return stats + [[task(r) for r in range(0, T, 16)] + staged2(
                _RHS, gz_v, lambda job, a, bs=range(4): norm(a * Q + job[0], [job[1] + 3 * b for b in bs]), 2, z22,
                [(r, c) for c in range(3) for r in range(0, Q, 16)], 0)]

        def raw_tile(ref, r, c):
            return ref[_ds(r, 16, 16), _tile(c)]

        def win_prep(i, n):
            src, dst = raw_b.at[_ds(i * n, 3 * D // 4 + n, 16)], op['win'].shifted(i, n)
            jobs = [(r, u) for r in range(0, n, 16) for u in range(7)]
            if stage_w:
                return staged2(_RHS, raw_b, lambda job, a: [
                    raw_tile(src, a * (D // 4) + job[0], 7 * b + job[1]).astype(F32) for b in range(4)], 1.5, dst, jobs, 1)
            return [t for r, u in jobs for t in expand2(
                _RHS, raw_b, lambda a, b, r=r, u=u: raw_tile(src, a * (D // 4) + r, 7 * b + u).astype(F32), dst, r, u)]

        def wd_tile(k, r, c, src=raw_b):
            return raw_tile(src, k % 7 * T + r, k // 7 * 8 + c).astype(F32)

        def wd_prep1():
            def task(r, c):
                def run():
                    pace(raw_b)
                    op['wd1'].put(r, c, _seven(_RHS, [wd_tile(k, r, cc) for k in (12, 13) for cc in (c, 4 + c)]))
                return (3.5, run)
            return [task(r, c) for c in range(4) for r in range(0, T, 16)]

        def wd_prep2(i):
            w = op['wd2']
            src = raw_b.at[_ds(i * 32, 6 * T + 32, 16)]
            dst = _Operand(w.ref.at[_ds(w.base + i * 16, w.size(2, 3 * T, 2) - 48)], 0, 2, 3 * T, 2)
            return [t for r in (0, 16) for k in range(3) for u in range(2) for t in expand2(
                _RHS, raw_b, lambda a, b, r=r, k=k, u=u: wd_tile(3 * a + k, r, 2 * b + u, src), dst, k * T + r, u)]

        def sp_prep1(i, blocks=range(NB)):
            src = raw_a.at[_ds(i * TM, TM, 16)]

            def task(r, b):
                def run():
                    pace(raw_a)
                    op['sa1'].put(r, b, _seven(_LHS, [raw_tile(src, a + r, 2 * b + cc).astype(F32)
                                                      for a in (0, T) for cc in (0, 1)]))
                return (3.5, run)
            return [task(r, b) for b in blocks for r in range(0, T, 16)]

        def sp_prep2(i):
            src = raw_a.at[_ds(i * TM, TM, 16)]

            def make(job, a):
                low = lax.broadcasted_iota(I32, (8, T), 1) < Q
                out = []
                for cc in (0, 1):
                    u, v = (pltpu.bitcast(raw_tile(src, a * Q + job[0], 4 * job[1] + 2 * k + cc), I32)
                            for k in (0, 1))
                    out += [jnp.where(low, u, pltpu.roll(v, Q, 1)), jnp.where(low, pltpu.roll(u, Q, 1), v)]
                return [pltpu.bitcast(t, BF16).astype(F32) for t in out]
            return staged2(_LHS, raw_a, make, 2, op['sa2'], [(r, c) for c in range(4) for r in range(0, Q, 16)], 1)

        def qkv_prep(t, lo=0, hi=D // 2):
            def where(stage, r):
                return perm_v[2 * stage + r // G % 2], (r // (D // 2) * G + r % G) * 4

            def drop(stage, r, vals):
                ref, o = where(stage, r)
                for c, v in enumerate(vals):
                    ref[_ds(o + 8 * c, 8), :] = pltpu.bitcast(v, F32)

            def grab(stage, r, cs):
                ref, o = where(stage, r)
                pace(ref)
                return [pltpu.bitcast(ref[_ds(o + 8 * c, 8), :], I32) for c in cs]

            def skew(r):
                def run():
                    pace(raw_a)
                    drop(0, r, _skew([pltpu.bitcast(raw_tile(raw_a, t // 2 * D + r, t % 2 * 8 + c), I32)
                                      for c in range(8)], 1, 2))
                return (3, run)

            def unskew(r):
                return (4, lambda: drop(1, r, _unskew(grab(0, r, range(8)), 1, 2)))

            def store(r, c):
                def run():
                    op['w' + 'qkv'[t]].put(r, c, _seven(_RHS, [
                        pltpu.bitcast(p, BF16).astype(F32) for a in (0, D // 2) for p in grab(1, a + r, (c, 4 + c))]))
                return (3, run)
            gs = range(lo, hi, G)
            return _stagger([[[f(a + r) for r in range(g, g + G, 16) for a in (0, D // 2)] for g in gs]
                             for f in (skew, unskew)] + [
                [[store(r, c) for r in range(g, g + G, 16) for c in range(4)] for g in gs]])

        def wo_prep():
            def task(g, c):
                def run():
                    pace(raw_a)
                    hv = [[pltpu.bitcast(p, BF16).astype(F32) for p in _unskew(_skew(
                        [pltpu.bitcast(raw_tile(raw_a, D + i * T + g, 8 + cc), I32) for i in range(8)], 0, 1), 0, 1)]
                        for cc in (c, 4 + c)]
                    for j in range(4):
                        op['wo'].put(j * T + g, c, _seven(_RHS, [hv[0][j], hv[1][j], hv[0][4 + j], hv[1][4 + j]]))
                return (22, run)
            return [task(g, c) for c in range(4) for g in range(0, T, 16)]

        def row(c, r):
            return c * (TM + PAD) + PAD + r

        def qkv(i, lhs, bufs, which):
            tasks = []
            for t in which:
                for u in range(4):
                    def emit(a, b, v, t=t, u=u):
                        ref, c = bufs[t // 2], t % 2 * 8 + 4 * b + u
                        ref[_ds(row(c, a), v.shape[0]), :] = v
                        ready[id(ref)] = t > 0 and (u, a + v.shape[0], b) == (3, TM, 1)
                        if t and a == 0 and isinstance(i, int) and i == 0:
                            ref[_ds(row(c, -PAD), PAD), :] = jnp.broadcast_to(v[0:1], (PAD, T))
                    tasks += unit(lhs, op['w' + 'qkv'[t]], u, emit)
            return tasks

        def history(src, dst, which=(1, 2)):
            for t in which:
                for c in range(t % 2 * 8, t % 2 * 8 + 8):
                    dst[t // 2][_ds(row(c, -PAD), PAD), :] = src[t // 2][_ds(row(c, TM - PAD), PAD), :]

        def slot(stage, w, r):
            if stage == cut - 1:
                return p_v, w * TM + r
            return stage_v[2 * stage + r // RB % 2], (w * 2 + r // T) * RB + r % RB

        def att(bufs, part, first=False):
            scale = DH ** -0.5
            qk, v = bufs

            def grab(stage, r):
                pace(slot(stage, 0, r)[0])
                return [ref[_ds(o, RA), :] for ref, o in (slot(stage, w, r) for w in range(W))]

            def drop(stage, r, vals):
                for w, t in enumerate(vals):
                    ref, o = slot(stage, w, r)
                    ref[_ds(o, RA), :] = t

            def scores(r):
                def run():
                    assert ready[id(qk)]
                    pace(qk)
                    q = [qk[_ds(row(c, r), RA), :] for c in range(8)]
                    drop(0, r, (_sum([lax.mul(q[c], qk[_ds(row(8 + c, r - DIL * w), RA), :]) for c in range(8)])
                                for w in range(W)))
                return (15 * RA / 8, run)

            def fold(r):
                def run():
                    lane = lax.broadcasted_iota(I32, (RA, T), 1)
                    ps = grab(0, r)
                    for bit in (16, 1):
                        low = (lane & bit) == 0
                        ps = [p + jnp.where(low, pltpu.roll(p, T - bit, 1), pltpu.roll(p, bit, 1)) for p in ps]
                    if first and r < DIL * W:
                        pos = lax.broadcasted_iota(I32, (RA, T), 0) + r
                        ps = [jnp.where(pos >= DIL * w, p, -1e9 / scale) for w, p in enumerate(ps)]
                    drop(1, r, ps)
                return (8 * RA / 8, run)

            def softmax(r):
                def run():
                    lg = grab(1, r)
                    m = functools.reduce(jnp.maximum, lg)
                    e = [jnp.exp2((p - m) * (scale * math.log2(math.e))) for p in lg]
                    inv = 1.0 / _sum(e)
                    drop(2, r, [t * inv for t in e])
                return (7 * RA / 8, run)

            def mix(r):
                def run():
                    assert ready[id(v)]
                    pace(v)
                    p = grab(2, r)
                    drop(3, r, (_sum([lax.mul(p[w], v[_ds(row(c, r - DIL * w), RA), :]) for w in range(W)])
                                for c in range(8)))
                return (15 * RA / 8, run)

            def combo(r):
                def run():
                    pace(slot(3, 0, r)[0])
                    for c in range(4):
                        op['oa'].put(r, c, _seven(_LHS, [ref[_ds(o, 16), :] for ref, o in (
                            slot(3, cc, a + r) for a in (0, T) for cc in (c, 4 + c))]))
                return (8, run)
            gs = range(0, T, RB)
            st = [[[f(a + r) for a in (0, T) for r in range(g, g + RB, RA)] for g in gs]
                  for f in (scores, fold, softmax, mix)] + [[[combo(r) for r in range(g, g + RB, 16)] for g in gs]]
            return _stagger(st[cut:] if part else st[:cut])

        def proj(i):
            tasks, x, h = [], x_blk(i), h_blk(i)
            for u in range(4):
                def emit(a, b, v, u=u):
                    c, n = 4 * b + u, v.shape[0]
                    h[_ds(c * S + a, n), :] = x[_ds(a, n), _tile(c)].astype(F32) + v
                tasks += unit(op['oa'], op['wo'], u, emit)
            return tasks

        def z1_blk(i):
            return z1_v.at[_ds(i * T, 3 * S + T)]

        def z1_at(c, r, n):
            return _ds((c // 2 * S + r) // 2, n // 2), _tile(c % 2)

        def up(i, lhs, gz_v):
            tasks, z1 = [], z1_blk(i)
            for u in range(7):
                def emit(a, b, v, u=u):
                    c = 7 * (b % 2) + u
                    if b < 2:
                        z1[z1_at(c, a, Q)] = pltpu.bitcast(v.astype(BF16), I32)
                    else:
                        gz_v[_ds(c * TM + a, Q), :] = _gelu(v)
                tasks += unit(lhs, op['win'], u, emit)
            return tasks

        def bias_prep():
            def task(k):
                def run():
                    bias_v[_ds(k * T, T), :] = jnp.broadcast_to(b_v[...].astype(F32)[k:k + 1, :], (T, T)).T
                return (4, run)
            return [task(k) for k in range(S // T)]

        def part_at(c, r, n):
            return _ds(c * TM + r, n)

        def gate_head(units):
            tasks = []
            for u in units:
                if u == 3:
                    def emit(a, b, v):
                        qk1[part_at(12 + b, a, v.shape[0]), :] = v
                    tasks += unit(op['sa1'], op['z21'], 0, emit, range(6))
                else:
                    def emit(a, b, v, u=u):
                        qk1[part_at(3 * b + u, a, Q), :] = v
                    tasks += unit(op['sa2'], op['z22'], u, emit, range(3))
            return tasks

        def gate_step(i, _, rest=False, extra=()):
            last[0] = None
            y_v, z1, h, out, bias = (v0, v1), z1_blk(i), h_blk(i), x_blk(i), bias_v.at[_ds(i * TM, TM)]

            def gated(c, r, v):
                if rest:
                    v = v + qk1[part_at(c, r, v.shape[0]), :]
                z = pltpu.bitcast(z1[z1_at(c, r, v.shape[0])], BF16).astype(F32)
                return _gelu(z) * (v + bias[_ds(r, v.shape[0]), :])

            y = {}

            def emit1(a, b, v):
                y[a // T, b] = gated(12 + b, a, v)
                if len(y) == 4:
                    op['ya1'].put(a % T, 0, _seven(_LHS, [y[0, 0], y[0, 1], y[1, 0], y[1, 1]]))
                    y.clear()
            main, marks, sides = unit(op['sa1'], op['z21'], 0, emit1, range(6, 8) if rest else None), [], []
            for u in range(3):
                def emit2(a, b, v, u=u):
                    y_v[u % 2][_ds(4 * a + b * Q, Q), :] = gated(3 * b + u, a, v)
                marks.append(sum(c for c, _ in main))
                main += unit(op['sa2'], op['z22'], u, emit2, range(3, 4) if rest else None)
                side = [expand2(_LHS, y_v[u % 2], lambda a, b, r=r, u=u: y_v[u % 2][_ds((4 * a + b) * Q + r, 16), :],
                                op['ya2'], r, u) for r in range(0, Q, 16)]
                sides.append([t for ts in zip(*side) for t in ts])
            marks.append(sum(c for c, _ in main))
            for u in range(4):
                def emit3(a, b, v, u=u):
                    at = _ds((4 * b + u) * S + a, v.shape[0])
                    h[at, :] = h[at, :] + v
                main += unit(op['ya1'], op['wd1'], u, emit3)
            marks.append(sum(c for c, _ in main))
            for u in range(2):
                def emit4(a, b, v, u=u):
                    c = 2 * b + u
                    out[_ds(a, Q), _tile(c)] = (h[_ds(c * S + a, Q), :] + v).astype(BF16)
                main += unit(op['ya2'], op['wd2'], u, emit4)
            t = [(m + 1) / sum(c for c, _ in main) for m in marks]
            g = 'g' if rest else 'p'
            nxt = i + 1 if isinstance(i, int) else jnp.minimum(i + 1, NB - 1)
            go('g0' if rest else 'p2', _overlap(main, *[(s, t[u + 1], t[u + 1] + F(g + str(u), 0.85) * (t[u + 2] - t[u + 1])) for u, s in enumerate(sides)],
                              (sp_prep1(nxt), t[0], F(g + '3', 0.9 if rest else 0.6)),
                              (sp_prep2(nxt), t[4], F(g + '4', 0.96), due(ops_v, 0.99)), *extra))
            rows = _ds(i * TM, TM, 16)
            if not only:
                pltpu.make_async_copy(out_v.at[rows], out_hbm.at[rows], osem).start()
            last[0] = None

        def go(name, tasks):
            if only and only != name:
                for k in (qk0, qk1, v0, v1):
                    ready[id(k)] = True
                return

            def run():
                for _, f in tasks:
                    f()
            if scopes:
                with jax.named_scope(name):
                    run()
            else:
                run()

        def wait(*keys):
            for k in () if only else keys:
                copies[k].wait()

        first, cur = (qk1, v1), (qk0, v0)
        xa, xb, ha, hb = (op[n] for n in ('xa', 'xb', 'ha', 'hb'))

        def hist(t):
            return [(0, lambda: history(cur, cur, (t,)))]

        def attn_step(i, _):
            last[0], ready[id(v0)] = None, True
            if isinstance(i, int):
                name, extra = 'a2', [(_zip(ln_h(0, ha)), F('c0', 0.0), F('c1', 0.539), due(mlp_v, F('c1', 0.539) + F('c2', 0.023))),
                                     (win_prep(15, 16), F('c3', 0.6), F('c4', 0.869), due(mlp_v, 0.97))]
            else:
                name, extra = 'a', [(win_prep(i - 3, 48), F('a0', 0.001), F('a1', 0.95),
                                     due(mlp_v, F('a2', 0.25), F('a3', 0.45), F('a4', 0.619), F('a5', 0.85)))]
            stats, norm = ln_x(i + 1 if isinstance(i, int) else jnp.minimum(i + 1, NB - 1), xa)
            go(name, _overlap(
                hist(1) + qkv(i, xa, cur, (0, 1)) + hist(2) + qkv(i, xa, cur, (2,)) + proj(i - 1),
                (att(cur, 1), 0.0, F('a6', 0.49)), (att(cur, 0), 0.501, F('a7', 0.888)),
                (stats, F('a8', 0.379), F('a9', 0.75)), (norm, 0.751, F('aa', 0.96), due(ops_v, 0.99)), *extra))
            last[0] = None

        def up_step(j, _):
            last[0] = None
            i = 2 * j + 1
            sides = []
            for t, z, h in ((0.0, ln_z(i - 1, gz_v), ln_h(i + 1, ha)), (0.501, ln_z(i, qk1), ln_h(i + 2, hb))):
                sides += [(z[0] + z[1], t, t + F('b0', 0.13)),
                          (z[2], t + F('b0', 0.13), t + F('b1', 0.331), due(z2_v, t + F('b1', 0.331) + F('b2', 0.022))),
                          (h[0] + h[1], t + F('b3', 0.25), t + F('b4', 0.347)),
                          (h[2], t + F('b4', 0.347), t + F('b5', 0.47))]
            wd = wd_prep2(j)
            go('b', _overlap(up(i, hb, qk1) + up(i + 1, ha, gz_v), *sides, ([], 0, 0, due(mlp_v, 0.99)),
                             *[(wd[k * len(wd) // 2:(k + 1) * len(wd) // 2], t + F('b6', 0.011), t + F('b7', 0.119),
                                due(ops_v, t + F('b7', 0.119) + F('b8', 0.01))) for k, t in enumerate((0.0, 0.5))]))
            last[0] = None

        if only:
            for ref in (raw_a, raw_b, x_v):
                ref[_ds(zero * 16, 16, 16), 0:T] = jnp.zeros((16, T), BF16)
            for ref in (h_v, gz_v, qk0, qk1, v0, v1, bias_v, p_v):
                ref[_ds(zero * 8, 8), :] = jnp.zeros((8, T), F32)
            z1_v[_ds(zero * 8, 8), 0:T] = jnp.zeros((8, T), I32)

        start('x0', x_hbm.at[0:TM], x_v.at[0:TM])
        QC = D // 2 // nq
        for k in range(nq):
            for a in (0, D // 2):
                start(('q', k, a), wqkv_hbm.at[a + k * QC:a + (k + 1) * QC, 0:D],
                      raw_a.at[a + k * QC:a + (k + 1) * QC, 0:D])
        start('x1', x_hbm.at[TM:2 * TM], x_v.at[TM:2 * TM])
        start('k', wqkv_hbm.at[:, D:2 * D], raw_a.at[0:D, D:2 * D])
        start('v', wqkv_hbm.at[:, 2 * D:], raw_a.at[D:2 * D, 0:D])
        start('wo', wo_hbm, raw_a.at[D:2 * D, D:2 * D])
        start('x2', x_hbm.at[2 * TM:4 * TM], x_v.at[2 * TM:4 * TM])
        start('win', win_hbm, raw_b.at[0:D])
        start('x', x_hbm.at[4 * TM:], x_v.at[4 * TM:S])
        start('b', b_hbm, b_v)

        wait('x0')
        go('lnx', sum(ln_x(0, xa), []))
        for k in range(nq):
            wait(('q', k, 0), ('q', k, D // 2), *(['x1'] if k == nq - 1 else []))
            go('wq', qkv_prep(0, k * QC, (k + 1) * QC))
        go('q0', _overlap(qkv(0, xa, first, (0,)), (sum(ln_x(1, xb), []), 0.0, F('q0', 0.9), due(ops_v, 0.965))))
        wait('k')
        go('q1', _overlap(qkv(1, xb, cur, (0,)), (qkv_prep(1), 0.0, F('q1', 0.9), due(ops_v, 0.965))))
        wait('v')
        go('k', _overlap(qkv(0, xa, first, (1,)) + qkv(1, xb, cur, (1,)),
                         (qkv_prep(2), 0.0, F('k0', 0.71), due(ops_v, F('k1', 0.852))),
                         (att(first, 0, True), 0.501, F('k2', 0.901))))
        wait('wo', 'x2')
        go('v', _overlap(qkv(0, xa, first, (2,)) + [(0, lambda: history(first, cur))] + qkv(1, xb, cur, (2,)) + proj(0),
                         (wo_prep(), 0.0, F('v0', 0.33), due(ops_v, F('v1', 0.444))),
                         (att(first, 1), F('v2', 0.3), F('v3', 0.564)), (att(cur, 0), F('v4', 0.34), F('v5', 0.875)),
                         (sum(ln_x(2, xa), []), F('v6', 0.34), F('v7', 0.97), due(ops_v, 0.985))))
        wait('win')
        attn_step(2, None)
        wait('x', 'b')
        start('wsp', wsp_hbm, raw_a.at[0:S])
        lax.fori_loop(3, NB, attn_step, None)
        for k in range(2):
            start(('wd', k), wout_hbm.at[k * FH // 2:(k + 1) * FH // 2], raw_b.at[0:FH // 2, k * D:(k + 1) * D])
        go('t1', _overlap(up(0, ha, gz_v) + proj(NB - 1), (att(cur, 1), 0.0, F('t0', 0.65)),
                          (_zip(ln_h(1, hb)) + bias_prep(), F('t1', 0.55), F('t2', 0.95), due(mlp_v, 0.97))))
        wait('wsp', ('wd', 0), ('wd', 1))
        lax.fori_loop(0, 3, up_step, None)
        z6, z7 = ln_z(NB - 2, gz_v), ln_z(NB - 1, qk0)
        go('t2', _overlap(up(NB - 1, hb, qk0) + gate_head([3, 0, 1, 2]),
                          (z6[0] + z6[1], 0.0, F('u0', 0.15)), (z6[2], F('u0', 0.15), F('u1', 0.356), due(z2_v, 0.5)),
                          (sp_prep1(0) + wd_prep1(), 0.0, F('u2', 0.2), due(ops_v, 0.3)),
                          (sp_prep2(0), F('u3', 0.35), F('u4', 0.583)),
                          (z7[0] + z7[1], 0.567, F('u5', 0.7)), (z7[2], F('u5', 0.7), F('u6', 0.95), due(z2_v, 0.99)),
                          (wd_prep2(3), F('u7', 0.577), F('u8', 0.744), due(ops_v, F('u8', 0.744) + 0.03))))
        pl.semaphore_signal(bar, 1)
        pl.semaphore_wait(bar, 1)
        gate_step(0, None, True)
        lax.fori_loop(1, NB, gate_step, None)
        if only:
            dyn = _ds(zero * 16, 16)
            out_v[0:16, 0:T] = (h_v[dyn, :] + gz_v[dyn, :] + p_v[dyn, :] + qk0[dyn, :] + v0[dyn, :] + qk1[dyn, :] + v1[dyn, :] + out_v[_ds(zero * 16, 16, 16), 0:T] + (
                z2_v[dyn, 0:T] + z1_v[dyn, 0:T] + ops_v[dyn, 0:T] + mlp_v[dyn, 0:T]).astype(F32)).astype(BF16)
            pltpu.make_async_copy(out_v.at[0:S], out_hbm, osem).start()
        pltpu.make_async_copy(out_v.at[0:S], out_hbm, osem).wait()

    def fn(A_x, A_wqkv, A_wo, B_x, B_w_in, B_w_sp, B_b_sp, B_w_out):
        del B_x
        hbm = pl.BlockSpec(memory_space=pl.ANY)
        vm = pltpu.VMEM
        out = pl.pallas_call(
            kernel,
            out_shape=jax.ShapeDtypeStruct((S, D), BF16),
            in_specs=[hbm] * 7,
            out_specs=hbm,
            scratch_shapes=[
                vm((S + PAD, D), BF16), vm((S + PAD, S), BF16), vm((D + PAD, 2 * FH), BF16),
                vm((_rows(_EARLY, _LATE) + 8, 2 * T), I32), vm((_rows(_BOTH) + 8, 2 * T), I32),
                vm((_rows(_Z2) + 8, 2 * T), I32), vm((W * TM + 16, T), F32),
                *[vm((n * (TM + PAD) + PAD, T), F32) for n in (16, 8, 16, 8)],
                vm((8 * S + PAD, T), F32), vm((14 * TM + PAD, T), F32), vm((7 * S // 2, 2 * T), I32),
                vm((6 * TM, T), F32),
                vm((S, T), F32), vm((S // T, T), BF16),
                pltpu.SemaphoreType.DMA((24,)), pltpu.SemaphoreType.DMA(()), pltpu.SemaphoreType.REGULAR(()),
                *[vm((16 * RB + 8, T), F32)] * 8, *[vm((16 * 16 + 8, T), F32)] * 6, *[vm((8 * G + 8, T), F32)] * 4,
                *[vm((T, T), F32)] * 10,
            ],
            compiler_params=pltpu.CompilerParams(vmem_limit_bytes=126 * 1024 * 1024,
                                                 flags=({flags: True} if flags else None)),
        )(A_x.reshape(S, D), A_wqkv, A_wo, B_w_in, B_w_sp, B_b_sp.reshape(S // T, T), B_w_out)
        return out.reshape(1, S, D)
    return fn


@jax.jit
def pallas_sequential_preLN__sliding_local_dilated__mixer_gmlp__prompt_kernel(
        A_x, A_wqkv, A_wo, B_x, B_w_in, B_w_sp, B_b_sp, B_w_out):
    return build()(A_x, A_wqkv, A_wo, B_x, B_w_in, B_w_sp, B_b_sp, B_w_out)
```

```python
import functools
import math

import numpy as np
import jax
import jax.numpy as jnp
from jax import lax
import jax.experimental.pallas as pl
import jax.experimental.pallas.tpu as pltpu

S, D, FH = 2048, 1024, 1792
H, DH, W, DIL = 32, 32, 8, 2
EPS = 1e-5
F32, BF16, I32 = jnp.float32, jnp.bfloat16, jnp.int32
T = 128
Q = 64
TM = 2 * T
NB = S // TM
PAD = 16


def _gelu(x):
    c = math.sqrt(2.0 / math.pi)
    u = x * (c + (c * 0.044715) * (x * x))
    hx = 0.5 * x
    return hx + hx * jnp.tanh(u)


def _skew(parts, axis, unit):
    return [c if i == 0 else pltpu.roll(c, unit * i, axis) for i, c in enumerate(parts)]


def _unskew(parts, axis, unit):
    n = parts[0].shape[axis]
    idx = lax.broadcasted_iota(I32, parts[0].shape, axis)
    x = [parts[-j % 8] for j in range(8)]
    for b in (1, 2, 4):
        on = (idx & (b * unit)) != 0
        x = [jnp.where(on, x[(j - b) % 8], x[j]) for j in range(8)]
    return [t if j == 0 else pltpu.roll(t, n - unit * j, axis) for j, t in enumerate(x)]


_LHS = (((1, 0, 0), (1, 1, 1)), ((1, 1, 0), (1, 1, 1)), ((1, 0, 0),), ((1, 1, 1),),
        ((1, 0, 0), (1, 0, 1)), ((1, 1, 0), (-1, 0, 0)), ((1, 0, 1), (-1, 1, 1)))
_RHS = (((1, 0, 0), (1, 1, 1)), ((1, 0, 0),), ((1, 0, 1), (-1, 1, 1)), ((1, 1, 0), (-1, 0, 0)),
        ((1, 1, 1),), ((1, 0, 0), (1, 0, 1)), ((1, 1, 0), (1, 1, 1)))


def _combine(terms, get):
    v = get(*terms[0][1:])
    for sign, a, b in terms[1:]:
        v = (lax.add if sign > 0 else lax.sub)(v, get(a, b))
    return v


def _seven(table, quad):
    return [_combine(terms, lambda a, b: quad[2 * a + b]) for terms in table]


def _sum(xs):
    return functools.reduce(lax.add, xs)


def _overlap(main, *sides):
    total, t, ev = sum(c for c, _ in main), 0.0, []
    for c, f in main:
        ev.append((t / total, 1, c, f))
        t += c
    for side, lo, hi, *due in sides:
        ev += [(when, 0, 0.0, f) for d in due for when, f in d]
        total, t = sum(c for c, _ in side), 0.0
        for c, f in side:
            ev.append((lo + (hi - lo) * t / total, 0, 0.0, f))
            t += c
    ev.sort(key=lambda e: e[:2])
    return [(e[2], e[3]) for e in ev]


def _stagger(stages):
    n, out = len(stages[0]), []
    for k in range(n + len(stages) - 1):
        now = [st[k - s] for s, st in enumerate(stages) if 0 <= k - s < n]
        now = [((j + 0.5) / len(g), s, t) for s, g in enumerate(now) for j, t in enumerate(g)]
        out += [t for _, _, t in sorted(now, key=lambda e: e[:2])]
    return out


def _zip(*lists):
    return [t for step in zip(*lists) for part in step for t in part]


def _cost(tasks):
    return sum(c for c, _ in tasks)


def _tile(c):
    return slice(c * T, (c + 1) * T)


def _ds(start, n, align=8):
    if isinstance(start, int):
        return pl.ds(lax.add(np.int32(start), np.int32(0)), n)
    return pl.ds(pl.multiple_of(start, align), n)


class _Operand:
    def __init__(self, ref, base, levels, rows, nt):
        self.ref, self.base, self.levels, self.rows, self.nt = ref, base, levels, rows, nt

    @staticmethod
    def size(levels, rows, nt):
        return (7 ** levels * nt + 1) // 2 * rows // 2

    def shifted(self, i, step):
        size = self.size(self.levels, self.rows, self.nt) - (self.rows - step) // 2
        return _Operand(self.ref.at[_ds(self.base + i * (step // 2), size)], 0, self.levels, self.rows, self.nt)

    def at(self, j, r, c, n):
        g = j * self.nt + c
        return _ds(self.base + g // 2 * self.rows // 2 + r // 2, n // 2), _tile(g % 2)

    def put(self, r, c, mats, first=0):
        for j, t in enumerate(mats):
            self.ref[self.at(first + j, r, c, t.shape[0])] = pltpu.bitcast(lax.convert_element_type(t, BF16), I32)

    def col(self, j, c, ks):
        return pltpu.bitcast(self.ref[self.at(j, ks[0] * T, c, len(ks) * T)], BF16)

    def full(self, j, ks, r, n, zeros=()):
        cols = [self.ref[self.at(j, r, c, n)] for c in ks]
        for z in zeros:
            cols[-1] = jnp.concatenate([cols[-1][:-8], cols[-1][-8:] | z], 0)
        return jnp.concatenate([pltpu.bitcast(c, BF16) for c in cols], 1)


_EARLY = dict(wq=(1, D // 2, 4), wk=(1, D // 2, 4), wv=(1, D // 2, 4), wo=(1, D // 2, 4),
              xa=(1, T, 4), xb=(1, T, 4), oa=(1, T, 4))
_LATE = dict(wd2=(2, 3 * T, 2), wd1=(1, T, 4), sa2=(2, Q, 4), sa1=(1, T, 8))
_BOTH = dict(win=(2, D // 4, 7), ha=(2, Q, 2), ya2=(2, Q, 3), ya1=(1, T, 1))
_Z2 = dict(z22=(2, S // 4, 3), z21=(1, S // 2, 1))


def _rows(*tables):
    return max(sum(_Operand.size(*s) for s in t.values()) for t in tables)


def build(RA=8, RB=64, RS=16, scopes=False, only=None, m1=0, m2=0, nq=4, stop=False, split_out=True, head=2, ahead=5, mrows=128, stage_w=False, cut=2, G=32, grouped=False, direct=True, wm=2,
          flags=None, **tune):
    F = tune.get
    macc = (m1, m2)

    def kernel(x_hbm, wqkv_hbm, wo_hbm, win_hbm, wsp_hbm, b_hbm, wout_hbm, out_hbm,
               x_v, raw_a, raw_b, ops_v, mlp_v, z2_v, p_v, qk0, v0, qk1, v1, h_v, gz_v, z1_v, stat_v,
               bias_v, b_v, sems, osem, bar, *small):
        out_v, stage_v, tmp_v = x_v, small[:8], small[8:14]
        perm_v, acc_v = small[14:18], small[18:]
        op = {}
        for ref, top, table in ((ops_v, 0, _EARLY), (ops_v, 0, _LATE), (mlp_v, 0, _BOTH),
                                (z2_v, 0, _Z2)):
            for name, shape in table.items():
                op[name] = _Operand(ref, top, *shape)
                top += _Operand.size(*shape)

        op['hb'] = _Operand(mlp_v, op['ya2'].base, 2, Q, 2)

        zero, zero2 = lax.fori_loop(0, 2, lambda _, c: (c[1] ^ 1, c[0] ^ 1), (0, 0))
        copies, last, paced, ready, pending, busy = {}, [None], {}, {}, [], [0]

        def pace(ref):
            if last[0] is None or paced.get(id(ref)) is last[0]:
                return
            paced[id(ref)] = last[0]
            n = 8 if ref.dtype == F32 else 16
            ref[_ds(zero * n + (ref.shape[0] - n), n, n), 0:T] = last[0][0:n].astype(ref.dtype)

        for ref in (ops_v, mlp_v, z2_v):
            ref[_ds(ref.shape[0] - 8, 8), 0:T] = jnp.zeros((8, T), I32)

        p_v[_ds(W * TM, 8), :] = jnp.zeros((8, T), F32)

        def due(ref, *times):
            def run():
                if ref is p_v:
                    return pending.append(pltpu.bitcast(p_v[_ds(zero * 8 + W * TM, 8), :], I32))
                pending.append(ref[_ds(zero * 8 + (ref.shape[0] - 8), 8), 0:T])
            return [(when, run) for when in times]

        def start(key, src, dst):
            copies[key] = pltpu.make_async_copy(src, dst, sems.at[len(copies)])
            if not only:
                copies[key].start()

        class Partial:
            def __init__(self, level, base, rows):
                self.level, self.base, self.rows, self.v = level, base + 8 * (2 - level), rows, {}

            def __setitem__(self, n, v):
                if n < macc[self.level - 1]:
                    acc_v[self.base + n][_ds(zero * 8, self.rows), :] = v
                else:
                    self.v[n] = v

            def __getitem__(self, n):
                if n < macc[self.level - 1]:
                    return acc_v[self.base + n][_ds(zero2 * 8, self.rows), :]
                return self.v[n]

        def unit(lhs, rhs, u, emit, ks=None):
            n = min(lhs.rows, mrows)
            return [t for r in range(0, lhs.rows, n) for t in products(
                lhs, rhs, u, lambda a, b, v, r=r: emit(a * lhs.rows + r, b, v), ks or range(lhs.nt), r, n, lhs.levels, 0)]

        def products(lhs, rhs, u, emit, ks, r0, rows, level, first):
            if level == 0:
                def run():
                    last[0] = jnp.dot(lhs.full(first, ks, r0, rows, pending), rhs.col(first, u, ks), preferred_element_type=F32)
                    pending.clear()
                    emit(0, 0, last[0])
                return [(len(ks) * rows / 4, run)]
            h = 2 ** (level - 1)
            state = {(i, j): Partial(level, (i * h + j) * 2, rows) for i in range(h) for j in range(h)}

            def step(n):
                def take(i, j, m):
                    s = state[i, j]
                    if n == 0:
                        s[0] = m
                    elif n == 1:
                        s[0], s[1] = s[0] + m, m
                    elif n == 2:
                        emit(h + i, j, m + s[1])
                        s[1] = m
                    elif n == 3:
                        s[0], s[1] = s[0] + m, m - s[1]
                    elif n == 4:
                        emit(i, j, s[0] - m)
                        s[0] = m
                    elif n == 5:
                        emit(i, h + j, m + s[0])
                        s[1] = s[1] + m
                    else:
                        emit(h + i, h + j, s[1] + m)
                return take
            return [t for n, r in enumerate((6, 3, 1, 0, 4, 2, 5))
                    for t in products(lhs, rhs, u, step(n), ks, r0, rows, level - 1, first * 7 + r)]

        def expand2(table, ref, get, dst, r, c):
            def task(group):
                def run():
                    pace(ref)
                    load = functools.cache(get)
                    for r1 in group:
                        quad = [_combine(table[r1], lambda a, b: load(2 * a + i, 2 * b + j))
                                for i in (0, 1) for j in (0, 1)]
                        dst.put(r, c, _seven(table, quad), 7 * r1)
                return (3 * len(group), run)
            if not grouped:
                return [task([r1]) for r1 in (6, 3, 1, 0, 4, 2, 5)]
            return [task(g) for g in (((3, 6, 1), (2, 4, 5, 0)) if table is _LHS else ((4, 6, 2), (1, 3, 5, 0)))]

        def staged2(table, src, make, cost, dst, jobs, pair):
            if direct and src is not raw_a:
                return [t for job in jobs for t in expand2(
                    table, src, lambda a, b, job=job: make(job, a, [b])[0], dst, *job)]
            fill, use = [], []
            for n, job in enumerate(jobs):
                ref = tmp_v[2 * pair + n % 2]

                def task(a, job=job, ref=ref):
                    def run():
                        pace(src)
                        for b, t in enumerate(make(job, a)):
                            ref[_ds((4 * a + b) * 16, 16), :] = t
                    return (cost, run)
                fill.append([task(a) for a in range(4)])
                use.append(expand2(table, ref, lambda a, b, ref=ref: ref[_ds((4 * a + b) * 16, 16), :], dst, *job[:2]))
            return _stagger([fill, use])

        def ln_stats(src, load, nt, stat):
            def mean(r):
                def run():
                    assert ready.get(id(src), True)
                    pace(src)
                    m = jnp.sum(_sum([load(r, c, RS) for c in range(nt)]), axis=-1, keepdims=True) * (1.0 / (nt * T))
                    stat_v[_ds(stat + r, RS), :] = jnp.broadcast_to(m, (RS, T))
                return (wm * nt * RS / 64, run)

            def rstd(r):
                def run():
                    pace(src)
                    m = stat_v[_ds(stat + r, RS), :]
                    v = [load(r, c, RS) - m for c in range(nt)]
                    var = jnp.sum(_sum([t * t for t in v]), axis=-1, keepdims=True) * (1.0 / (nt * T))
                    stat_v[_ds(stat + TM + r, RS), :] = jnp.broadcast_to(lax.rsqrt(var + EPS), (RS, T))
                return (3 * nt * RS / 64, run)

            def norm(r, cs):
                m, inv = stat_v[_ds(stat + r, 16), :], stat_v[_ds(stat + TM + r, 16), :]
                return [(load(r, c, 16) - m) * inv for c in cs]
            return [[f(g) for g in range(0, TM, RS)] for f in (mean, rstd)], norm

        def x_blk(i):
            return x_v.at[_ds(i * TM, TM, 16)]

        def h_blk(i):
            return h_v.at[_ds(i * TM, 7 * S + TM)]

        def ln_x(i, dst):
            x = x_blk(i)
            stats, norm = ln_stats(x_v, lambda r, c, n: x[_ds(r, n), _tile(c)].astype(F32), 8, 0)

            def task(r, c):
                def run():
                    pace(x_v)
                    dst.put(r, c, _seven(_LHS, norm(r, (c, 4 + c)) + norm(T + r, (c, 4 + c))))
                return (5, run)
            return stats[0] + stats[1], [task(r, c) for r in range(0, T, 16) for c in range(4)]

        def ln_h(i, dst):
            h = h_blk(i)
            stats, norm = ln_stats(h_v, lambda r, c, n: h[_ds(c * S + r, n), :], 8, 2 * TM)
            return stats + [staged2(_LHS, h_v, lambda job, a, bs=range(4): norm(a * Q + job[0], [job[1] + 2 * b for b in bs]), 2, dst,
                                   [(r, c) for c in range(2) for r in range(0, Q, 16)], 2)]

        def ln_z(i, gz_v):
            stats, norm = ln_stats(gz_v, lambda r, c, n: gz_v[_ds(c * TM + r, n), :], 14, 4 * TM)
            z21, z22 = op['z21'].shifted(i, T), op['z22'].shifted(i, Q)

            def task(r):
                def run():
                    pace(gz_v)
                    z21.put(r, 0, _seven(_RHS, norm(r, (12, 13)) + norm(T + r, (12, 13))))
                return (4, run)
            return stats + [[task(r) for r in range(0, T, 16)] + staged2(
                _RHS, gz_v, lambda job, a, bs=range(4): norm(a * Q + job[0], [job[1] + 3 * b for b in bs]), 2, z22,
                [(r, c) for c in range(3) for r in range(0, Q, 16)], 0)]

        def raw_tile(ref, r, c):
            return ref[_ds(r, 16, 16), _tile(c)]

        def win_prep(i, n):
            src, dst = raw_b.at[_ds(i * n, 3 * D // 4 + n, 16)], op['win'].shifted(i, n)
            jobs = [(r, u) for r in range(0, n, 16) for u in range(7)]
            if stage_w:
                return staged2(_RHS, raw_b, lambda job, a: [
                    raw_tile(src, a * (D // 4) + job[0], 7 * b + job[1]).astype(F32) for b in range(4)], 1.5, dst, jobs, 1)
            return [t for r, u in jobs for t in expand2(
                _RHS, raw_b, lambda a, b, r=r, u=u: raw_tile(src, a * (D // 4) + r, 7 * b + u).astype(F32), dst, r, u)]

        def wd_tile(k, r, c, src=raw_b):
            return raw_tile(src, k % 7 * T + r, k // 7 * 8 + c).astype(F32)

        def wd_prep1():
            def task(r, c):
                def run():
                    pace(raw_b)
                    op['wd1'].put(r, c, _seven(_RHS, [wd_tile(k, r, cc) for k in (12, 13) for cc in (c, 4 + c)]))
                return (3.5, run)
            return [task(r, c) for c in range(4) for r in range(0, T, 16)]

        def wd_prep2(i):
            w = op['wd2']
            src = raw_b.at[_ds(i * 32, 6 * T + 32, 16)]
            dst = _Operand(w.ref.at[_ds(w.base + i * 16, w.size(2, 3 * T, 2) - 48)], 0, 2, 3 * T, 2)
            return [t for r in (0, 16) for k in range(3) for u in range(2) for t in expand2(
                _RHS, raw_b, lambda a, b, r=r, k=k, u=u: wd_tile(3 * a + k, r, 4 * u + b, src), dst, k * T + r, u)]

        def sp_prep1(i, blocks=range(NB)):
            src = raw_a.at[_ds(i * TM, TM, 16)]

            def task(r, b):
                def run():
                    pace(raw_a)
                    op['sa1'].put(r, b, _seven(_LHS, [raw_tile(src, a + r, 2 * b + cc).astype(F32)
                                                      for a in (0, T) for cc in (0, 1)]))
                return (3.5, run)
            return [task(r, b) for b in blocks for r in range(0, T, 16)]

        def sp_prep2(i):
            src = raw_a.at[_ds(i * TM, TM, 16)]

            def make(job, a):
                low = lax.broadcasted_iota(I32, (8, T), 1) < Q
                out = []
                for cc in (0, 1):
                    u, v = (pltpu.bitcast(raw_tile(src, a * Q + job[0], 4 * job[1] + 2 * k + cc), I32)
                            for k in (0, 1))
                    out += [jnp.where(low, u, pltpu.roll(v, Q, 1)), jnp.where(low, pltpu.roll(u, Q, 1), v)]
                return [pltpu.bitcast(t, BF16).astype(F32) for t in out]
            return staged2(_LHS, raw_a, make, 2, op['sa2'], [(r, c) for c in range(4) for r in range(0, Q, 16)], 1)

        def qkv_prep(t, k):
            def where(stage, r):
                return perm_v[2 * stage + r // G % 2], (r // (D // 2) * G + r % G) * 4

            def drop(stage, r, vals):
                ref, o = where(stage, r)
                for c, v in enumerate(vals):
                    ref[_ds(o + 8 * c, 8), :] = pltpu.bitcast(v, F32)

            def grab(stage, r, cs):
                ref, o = where(stage, r)
                pace(ref)
                return [pltpu.bitcast(ref[_ds(o + 8 * c, 8), :], I32) for c in cs]

            def skew(r):
                def run():
                    pace(raw_a)
                    drop(0, r, _skew([pltpu.bitcast(raw_tile(raw_a, t // 2 * D + r, t % 2 * 8 + c), I32)
                                      for c in range(8)], 1, 2))
                return (3, run)

            def unskew(r):
                return (4, lambda: drop(1, r, _unskew(grab(0, r, range(8)), 1, 2)))

            def store(r, c):
                def run():
                    op['w' + 'qkv'[t]].put(r, c, _seven(_RHS, [
                        pltpu.bitcast(p, BF16).astype(F32) for a in (0, D // 2) for p in grab(1, a + r, (c, 4 + c))]))
                return (3, run)
            gs = range(k * T, (k + 1) * T, G)
            return [[[f(a + r) for r in range(g, g + G, 16) for a in (0, D // 2)] for g in gs]
                    for f in (skew, unskew)] + [
                [[store(r, c) for r in range(g, g + G, 16) for c in range(4)] for g in gs]]

        def wo_prep():
            def task(g, c):
                def run():
                    pace(raw_a)
                    hv = [[pltpu.bitcast(p, BF16).astype(F32) for p in _unskew(_skew(
                        [pltpu.bitcast(raw_tile(raw_a, D + i * T + g, 8 + cc), I32) for i in range(8)], 0, 1), 0, 1)]
                        for cc in (c, 4 + c)]
                    for j in range(4):
                        op['wo'].put(j * T + g, c, _seven(_RHS, [hv[0][j], hv[1][j], hv[0][4 + j], hv[1][4 + j]]))
                return (22, run)
            return [task(g, c) for c in range(4) for g in range(0, T, 16)]

        def row(c, r):
            return c * (TM + PAD) + PAD + r

        def qkv(i, lhs, bufs, which, ks=range(4)):
            tasks = []
            for t in which:
                for u in range(4):
                    def emit(a, b, v, t=t, u=u):
                        ref, c = bufs[t // 2], t % 2 * 8 + 4 * b + u
                        if ks[0]:
                            v = v + ref[_ds(row(c, a), v.shape[0]), :]
                        ref[_ds(row(c, a), v.shape[0]), :] = v
                        ready[id(ref)] = t > 0 and ks[-1] == 3 and (u, a + v.shape[0], b) == (3, TM, 1)
                        if t and a == 0 and isinstance(i, int) and i == 0:
                            ref[_ds(row(c, -PAD), PAD), :] = jnp.broadcast_to(v[0:1], (PAD, T))
                    tasks += unit(lhs, op['w' + 'qkv'[t]], u, emit, ks)
            return tasks

        def history(src, dst, which=(1, 2)):
            for t in which:
                for c in range(t % 2 * 8, t % 2 * 8 + 8):
                    dst[t // 2][_ds(row(c, -PAD), PAD), :] = src[t // 2][_ds(row(c, TM - PAD), PAD), :]

        def att(bufs, part, first=False, logits=p_v):
            def slot(stage, w, r):
                if stage == cut - 1:
                    return logits, w * TM + r
                return stage_v[2 * stage + r // RB % 2], (w * 2 + r // T) * RB + r % RB

            scale = DH ** -0.5
            qk, v = bufs

            def grab(stage, r):
                pace(slot(stage, 0, r)[0])
                return [ref[_ds(o, RA), :] for ref, o in (slot(stage, w, r) for w in range(W))]

            def drop(stage, r, vals):
                for w, t in enumerate(vals):
                    ref, o = slot(stage, w, r)
                    ref[_ds(o, RA), :] = t

            def scores(r):
                def run():
                    assert ready[id(qk)]
                    pace(qk)
                    q = [qk[_ds(row(c, r), RA), :] for c in range(8)]
                    drop(0, r, (_sum([lax.mul(q[c], qk[_ds(row(8 + c, r - DIL * w), RA), :]) for c in range(8)])
                                for w in range(W)))
                return (15 * RA / 8, run)

            def fold(r):
                def run():
                    lane = lax.broadcasted_iota(I32, (RA, T), 1)
                    ps = grab(0, r)
                    for bit in (16, 1):
                        low = (lane & bit) == 0
                        ps = [p + jnp.where(low, pltpu.roll(p, T - bit, 1), pltpu.roll(p, bit, 1)) for p in ps]
                    if first and r < DIL * W:
                        pos = lax.broadcasted_iota(I32, (RA, T), 0) + r
                        ps = [jnp.where(pos >= DIL * w, p, -1e9 / scale) for w, p in enumerate(ps)]
                    drop(1, r, ps)
                return (8 * RA / 8, run)

            def softmax(r):
                def run():
                    lg = grab(1, r)
                    m = functools.reduce(jnp.maximum, lg)
                    e = [jnp.exp2((p - m) * (scale * math.log2(math.e))) for p in lg]
                    inv = 1.0 / _sum(e)
                    drop(2, r, [t * inv for t in e])
                return (7 * RA / 8, run)

            def mix(r):
                def run():
                    assert ready[id(v)]
                    pace(v)
                    p = grab(2, r)
                    drop(3, r, (_sum([lax.mul(p[w], v[_ds(row(c, r - DIL * w), RA), :]) for w in range(W)])
                                for c in range(8)))
                return (15 * RA / 8, run)

            def combo(r):
                def run():
                    pace(slot(3, 0, r)[0])
                    for c in range(4):
                        assert not busy[0]
                        op['oa'].put(r, c, _seven(_LHS, [ref[_ds(o, 16), :] for ref, o in (
                            slot(3, cc, a + r) for a in (0, T) for cc in (c, 4 + c))]))
                return (8, run)
            gs = range(0, T, RB)
            st = [[[f(a + r) for a in (0, T) for r in range(g, g + RB, RA)] for g in gs]
                  for f in (scores, fold, softmax, mix)] + [[[combo(r) for r in range(g, g + RB, 16)] for g in gs]]
            return _stagger(st[cut:] if part else st[:cut])

        def proj(i):
            tasks, x, h = [], x_blk(i), h_blk(i)
            for u in range(4):
                def emit(a, b, v, u=u):
                    c, n = 4 * b + u, v.shape[0]
                    busy[0] = (u, a + n, b) != (3, TM, 1)
                    h[_ds(c * S + a, n), :] = x[_ds(a, n), _tile(c)].astype(F32) + v
                tasks += unit(op['oa'], op['wo'], u, emit)
            return tasks

        def z1_blk(i):
            return z1_v.at[_ds(i * T, 3 * S + T)]

        def z1_at(c, r, n):
            return _ds((c // 2 * S + r) // 2, n // 2), _tile(c % 2)

        def up(i, lhs, gz_v):
            tasks, z1 = [], z1_blk(i)
            for u in range(7):
                def emit(a, b, v, u=u):
                    c = 7 * (b % 2) + u
                    ready[id(gz_v)] = (u, a, b) == (6, 3 * Q, 3)
                    if b < 2:
                        z1[z1_at(c, a, Q)] = pltpu.bitcast(v.astype(BF16), I32)
                    else:
                        gz_v[_ds(c * TM + a, Q), :] = _gelu(v)
                tasks += unit(lhs, op['win'], u, emit)
            return tasks

        def bias_prep():
            def task(k):
                def run():
                    bias_v[_ds(k * T, T), :] = jnp.broadcast_to(b_v[...].astype(F32)[k:k + 1, :], (T, T)).T
                return (4, run)
            return [task(k) for k in range(S // T)]

        def part_at(c, r, n):
            return _ds(c * TM + r, n)

        def gate_head(units):
            tasks = []
            for u in units:
                if u == 3:
                    def emit(a, b, v):
                        qk1[part_at(12 + b, a, v.shape[0]), :] = v
                    tasks += unit(op['sa1'], op['z21'], 0, emit, range(2 * head))
                else:
                    def emit(a, b, v, u=u):
                        qk1[part_at(3 * b + u, a, Q), :] = v
                    tasks += unit(op['sa2'], op['z22'], u, emit, range(head))
            return tasks

        def gate_step(i, _, rest=False, extra=()):
            last[0] = None
            y_v, z1, h, out, bias = (v0, v1), z1_blk(i), h_blk(i), x_blk(i), bias_v.at[_ds(i * TM, TM)]

            def gated(c, r, v):
                if rest:
                    v = v + qk1[part_at(c, r, v.shape[0]), :]
                z = pltpu.bitcast(z1[z1_at(c, r, v.shape[0])], BF16).astype(F32)
                return _gelu(z) * (v + bias[_ds(r, v.shape[0]), :])

            y = {}

            def emit1(a, b, v):
                y[a // T, b] = gated(12 + b, a, v)
                if len(y) == 4:
                    op['ya1'].put(a % T, 0, _seven(_LHS, [y[0, 0], y[0, 1], y[1, 0], y[1, 1]]))
                    y.clear()
            main, marks, sides = unit(op['sa1'], op['z21'], 0, emit1, range(2 * head, 8) if rest else None), [], []
            for u in range(3):
                def emit2(a, b, v, u=u):
                    y_v[u % 2][_ds(4 * a + b * Q, Q), :] = gated(3 * b + u, a, v)
                marks.append(sum(c for c, _ in main))
                main += unit(op['sa2'], op['z22'], u, emit2, range(head, 4) if rest else None)
                side = [expand2(_LHS, y_v[u % 2], lambda a, b, r=r, u=u: y_v[u % 2][_ds((4 * a + b) * Q + r, 16), :],
                                op['ya2'], r, u) for r in range(0, Q, 16)]
                sides.append([t for ts in zip(*side) for t in ts])
            marks.append(sum(c for c, _ in main))
            for u in range(4):
                def emit3(a, b, v, u=u):
                    at = _ds((4 * b + u) * S + a, v.shape[0])
                    h[at, :] = h[at, :] + v
                main += unit(op['ya1'], op['wd1'], u, emit3)
            marks.append(sum(c for c, _ in main))
            for u in range(2):
                def emit4(a, b, v, u=u):
                    c = 4 * u + b
                    out[_ds(a, Q), _tile(c)] = (h[_ds(c * S + a, Q), :] + v).astype(BF16)
                main += unit(op['ya2'], op['wd2'], u, emit4)
                if not only and split_out:
                    at = _ds(i * TM, TM, 16), slice(u * D // 2, (u + 1) * D // 2)
                    main.append((0, pltpu.make_async_copy(out_v.at[at], out_hbm.at[at], osem).start))
            t = [(m + 1) / sum(c for c, _ in main) for m in marks]
            g = 'g' if rest else 'p'
            nxt = i + 1 if isinstance(i, int) else jnp.minimum(i + 1, NB - 1)
            go('g0' if rest else 'p2', _overlap(main, *[(s, t[u + 1], t[u + 1] + F(g + str(u), (0.94, 0.99, 0.767)[u] if rest else (0.453, 0.593, 0.911)[u]) * (t[u + 2] - t[u + 1])) for u, s in enumerate(sides)],
                              (sp_prep1(nxt), t[0], F(g + '3', 0.97 if rest else 0.6)),
                              (sp_prep2(nxt), t[4], F(g + '4', 0.96 if rest else 0.98), due(ops_v, 0.99)), *extra))
            rows = _ds(i * TM, TM, 16)
            if not only and not split_out:
                pltpu.make_async_copy(out_v.at[rows], out_hbm.at[rows], osem).start()
            last[0] = None

        def go(name, tasks):
            if only and only != name:
                for k in (qk0, qk1, v0, v1, gz_v):
                    ready[id(k)] = True
                return

            def run():
                for _, f in tasks:
                    f()
            if scopes:
                with jax.named_scope(name):
                    run()
            else:
                run()

        def barrier():
            pl.semaphore_signal(bar, 1)
            pl.semaphore_wait(bar, 1)

        def wait(*keys):
            for k in () if only else keys:
                copies[k].wait()

        first, cur = (qk1, v1), (qk0, v0)
        xa, xb, ha, hb = (op[n] for n in ('xa', 'xb', 'ha', 'hb'))

        def hist(t):
            return [(0, lambda: history(cur, cur, (t,)))]

        def attn_step(i, _):
            last[0], ready[id(v0)] = None, True
            if isinstance(i, int):
                h = ln_h(0, ha)
                name, extra = 'a2', [(h[0] + h[1], F('c0', 0.299), F('c1', 0.51)),
                                     (h[2], F('c1', 0.51), F('c2', 0.98), due(mlp_v, 0.99)),
                                     (win_prep(3, 64), 0.0, F('c3', 0.806), due(mlp_v, 0.25, 0.45, 0.65, 0.85))]
            else:
                stats, norm = ln_x(i + 1, xa)
                name, extra = 'a', [(stats, F('a8', 0.379), F('a9', 0.75)),
                                    (norm, 0.751, F('aa', 0.96), due(ops_v, 0.99)),
                                    (win_prep(i - 3, 48), F('a0', 0.001), F('a1', 0.95),
                                     due(mlp_v, F('a2', 0.25), F('a3', 0.45), F('a4', 0.619), F('a5', 0.85)))]
            go(name, _overlap(
                hist(1) + qkv(i, xa, cur, (0, 1)) + hist(2) + qkv(i, xa, cur, (2,)) + proj(i - 1),
                (att(cur, 1), 0.0, F('a6', 0.49)), (att(cur, 0), 0.501, F('a7', 0.888)), *extra))
            last[0] = None

        def up_step(j, _):
            last[0] = None
            i = 2 * j + 1
            sides = []
            for t, z, h in ((0.0, ln_z(i - 1, gz_v), ln_h(i + 1, ha)), (0.501, ln_z(i, qk1), ln_h(i + 2, hb))):
                sides += [(z[0] + z[1], t, t + F('b0', 0.13)),
                          (z[2], t + F('b0', 0.13), t + F('b1', 0.331), due(z2_v, t + F('b1', 0.331) + F('b2', 0.022))),
                          (h[0] + h[1], t + F('b3', 0.25), t + F('b4', 0.347)),
                          (h[2], t + F('b4', 0.347), t + F('b5', 0.47))]
            wd = wd_prep2(j)
            go('b', _overlap(up(i, hb, qk1) + up(i + 1, ha, gz_v), *sides, ([], 0, 0, due(mlp_v, 0.99)),
                             *[(wd[k * len(wd) // 2:(k + 1) * len(wd) // 2], t + F('b6', 0.011), t + F('b7', 0.119),
                                due(ops_v, t + F('b7', 0.119) + F('b8', 0.01))) for k, t in enumerate((0.0, 0.5))]))
            last[0] = None

        if only:
            for ref in (raw_a, raw_b, x_v):
                ref[_ds(zero * 16, 16, 16), 0:T] = jnp.zeros((16, T), BF16)
            for ref in (h_v, gz_v, qk0, qk1, v0, v1, bias_v, p_v):
                ref[_ds(zero * 8, 8), :] = jnp.zeros((8, T), F32)
            z1_v[_ds(zero * 8, 8), 0:T] = jnp.zeros((8, T), I32)

        def start_rows(t, k):
            for r in (k * T, D // 2 + k * T):
                start((t, r), wqkv_hbm.at[r:r + T, t * D:(t + 1) * D],
                      raw_a.at[t // 2 * D + r:t // 2 * D + r + T, t % 2 * D:(t % 2 + 1) * D])

        later = [lambda: start('x0', x_hbm.at[0:TM], x_v.at[0:TM]),
                 lambda: start('x1', x_hbm.at[TM:2 * TM], x_v.at[TM:2 * TM]),
                 *[functools.partial(start_rows, t, k) for t in range(3) for k in range(4)],
                 lambda: start('wo', wo_hbm, raw_a.at[D:2 * D, D:2 * D]),
                 lambda: start('x2a', x_hbm.at[2 * TM:3 * TM], x_v.at[2 * TM:3 * TM]),
                 lambda: start('x2', x_hbm.at[3 * TM:4 * TM], x_v.at[3 * TM:4 * TM]),
                 lambda: start('win', win_hbm, raw_b.at[0:D]),
                 lambda: start('x', x_hbm.at[4 * TM:], x_v.at[4 * TM:S]),
                 lambda: start('b', b_hbm, b_v)]

        def more(n):
            for _ in range(min(n, len(later))):
                later.pop(0)()

        def arrive(*chunks):
            wait(*[(t, a + k * T) for t, k in chunks for a in (0, D // 2)])
            more(len(chunks) + (chunks[-1] == (1, 3)) * 2)
            return _stagger([sum(st, []) for st in zip(*[qkv_prep(t, k) for t, k in chunks])])

        more(ahead)
        for i, dst in enumerate((xa, xb)):
            wait(f'x{i}')
            more(1)
            go('lnx', sum(ln_x(i, dst), []))
        go('wq', arrive((0, 0)))
        for n, (t, ks, chunks) in enumerate((
                (0, [0], [(0, 1)]), (0, [1], [(0, 2)]), (0, [2], [(0, 3), (1, 0)]), (0, [3], [(1, 1)]),
                (1, [0, 1], [(1, 2), (1, 3)]), (1, [2, 3], [(2, 0), (2, 1), (2, 2)]))):
            go(f'q{n}', _overlap(qkv(0, xa, cur, (t,), ks) + qkv(1, xb, first, (t,), ks),
                                 (arrive(*chunks), 0.0, F(f'q{n}', 0.85), due(ops_v, 0.98))))
        side = arrive((2, 3))
        more(9)
        if stop:
            wait('wo', 'x2', 'win', 'x', 'b')
            dyn = _ds(zero * 16, 16)
            out_v[0:16, 0:T] = (qk0[dyn, :] + qk1[dyn, :] + p_v[dyn, :] + ops_v[dyn, 0:T].astype(F32)).astype(BF16)
            pltpu.make_async_copy(out_v.at[0:16], out_hbm.at[0:16], osem).start()
            pltpu.make_async_copy(out_v.at[0:16], out_hbm.at[0:16], osem).wait()
            return
        wait('wo', 'x2a')
        go('v', _overlap(qkv(0, xa, cur, (2,), [0, 1, 2]) + qkv(0, xa, cur, (2,), [3])
                         + [(0, lambda: history(cur, first))] + qkv(1, xb, first, (2,)),
                         (side, 0.0, F('v0', 0.31)), (att(cur, 0, True), F('v1', 0.0), F('v2', 0.7)),
                         (sum(ln_x(2, xa), []), 0.501, F('v3', 0.95), due(ops_v, 0.985)),
                         (wo_prep()[:16], F('v4', 0.2), F('v5', 0.6), due(ops_v, F('v5', 0.6) + 0.05))))
        wait('x2')
        stats, norm = ln_x(3, xa)
        go('w', _overlap([(0, lambda: history(first, cur, (1,)))] + qkv(2, xa, cur, (0, 1)) + proj(0)
                         + [(0, lambda: history(first, cur, (2,)))] + qkv(2, xa, cur, (2,)) + proj(1),
                         (att(cur, 1), 0.0, F('w0', 0.39)), (wo_prep()[16:], 0.0, F('w1', 0.39)),
                         (att(first, 0, False, gz_v), F('w2', 0.025), F('w3', 0.464)),
                         (att(first, 1, False, gz_v), F('w3', 0.464), F('w4', 0.79)),
                         (att(cur, 0), F('w5', 0.55), F('w6', 0.905)),
                         (stats, F('w7', 0.4), F('w8', 0.8)), (norm, 0.801, F('w9', 0.95), due(ops_v, 0.99))))
        wait('win', 'x', 'b')
        start('wsp', wsp_hbm, raw_a.at[0:S])
        lax.fori_loop(3, NB - 1, attn_step, None)
        attn_step(NB - 1, None)
        for k in range(2):
            start(('wd', k), wout_hbm.at[k * FH // 2:(k + 1) * FH // 2], raw_b.at[0:FH // 2, k * D:(k + 1) * D])
        barrier()
        go('t1', _overlap(up(0, ha, gz_v) + proj(NB - 1), (att(cur, 1), 0.0, F('t0', 0.65)),
                          (_zip(ln_h(1, hb)) + bias_prep(), F('t1', 0.55), F('t2', 0.95), due(mlp_v, 0.97))))
        wait('wsp', ('wd', 0), ('wd', 1))
        lax.fori_loop(0, 3, up_step, None)
        z6, z7 = ln_z(NB - 2, gz_v), ln_z(NB - 1, qk0)
        main = up(NB - 1, hb, qk0), gate_head([3, 0, 1, 2])
        mid = (_cost(main[0]) + 1) / _cost(main[0] + main[1])
        go('t2', _overlap(main[0] + main[1],
                          (z6[0] + z6[1], 0.0, F('u0', 0.114)), (z6[2], F('u0', 0.114), F('u1', 0.356), due(z2_v, 0.5)),
                          (sp_prep1(0) + wd_prep1(), 0.0, F('u2', 0.2), due(ops_v, 0.3)),
                          (sp_prep2(0), F('u3', 0.35), F('u4', 0.696)),
                          (z7[0] + z7[1], mid, F('u5', 0.76)), (z7[2], F('u5', 0.76), F('u6', 0.95), due(z2_v, 0.99)),
                          (wd_prep2(3), F('u7', 0.371), F('u8', 0.762), due(ops_v, F('u8', 0.762) + 0.03))))
        barrier()
        gate_step(0, None, True)
        lax.fori_loop(1, NB, gate_step, None)
        if only:
            dyn = _ds(zero * 16, 16)
            out_v[0:16, 0:T] = (h_v[dyn, :] + gz_v[dyn, :] + p_v[dyn, :] + qk0[dyn, :] + v0[dyn, :] + qk1[dyn, :] + v1[dyn, :] + out_v[_ds(zero * 16, 16, 16), 0:T] + (
                z2_v[dyn, 0:T] + z1_v[dyn, 0:T] + ops_v[dyn, 0:T] + mlp_v[dyn, 0:T]).astype(F32)).astype(BF16)
            pltpu.make_async_copy(out_v.at[0:S], out_hbm, osem).start()
        pltpu.make_async_copy(out_v.at[0:S], out_hbm, osem).wait()

    def fn(A_x, A_wqkv, A_wo, B_x, B_w_in, B_w_sp, B_b_sp, B_w_out):
        del B_x
        hbm = pl.BlockSpec(memory_space=pl.ANY)
        vm = pltpu.VMEM
        out = pl.pallas_call(
            kernel,
            out_shape=jax.ShapeDtypeStruct((S, D), BF16),
            in_specs=[hbm] * 7,
            out_specs=hbm,
            scratch_shapes=[
                vm((S + PAD, D), BF16), vm((S + PAD, S), BF16), vm((D + PAD, 2 * FH), BF16),
                vm((_rows(_EARLY, _LATE) + 8, 2 * T), I32), vm((_rows(_BOTH) + 8, 2 * T), I32),
                vm((_rows(_Z2) + 8, 2 * T), I32), vm((W * TM + 16, T), F32),
                *[vm((n * (TM + PAD) + PAD, T), F32) for n in (16, 8, 16, 8)],
                vm((8 * S + PAD, T), F32), vm((14 * TM + PAD, T), F32), vm((7 * S // 2, 2 * T), I32),
                vm((6 * TM, T), F32),
                vm((S, T), F32), vm((S // T, T), BF16),
                pltpu.SemaphoreType.DMA((36,)), pltpu.SemaphoreType.DMA(()), pltpu.SemaphoreType.REGULAR(()),
                *[vm((16 * RB + 8, T), F32)] * 8, *[vm((16 * 16 + 8, T), F32)] * 6, *[vm((8 * G + 8, T), F32)] * 4,
                *[vm((T, T), F32)] * 10,
            ],
            compiler_params=pltpu.CompilerParams(vmem_limit_bytes=126 * 1024 * 1024,
                                                 flags=({flags: True} if flags else None)),
        )(A_x.reshape(S, D), A_wqkv, A_wo, B_w_in, B_w_sp, B_b_sp.reshape(S // T, T), B_w_out)
        return out.reshape(1, S, D)
    return fn


@jax.jit
def pallas_sequential_preLN__sliding_local_dilated__mixer_gmlp__prompt_kernel(
        A_x, A_wqkv, A_wo, B_x, B_w_in, B_w_sp, B_b_sp, B_w_out):
    return build()(A_x, A_wqkv, A_wo, B_x, B_w_in, B_w_sp, B_b_sp, B_w_out)
```

```python
import functools
import math

import numpy as np
import jax
import jax.numpy as jnp
from jax import lax
import jax.experimental.pallas as pl
import jax.experimental.pallas.tpu as pltpu

S, D, FH = 2048, 1024, 1792
DH, W, DIL = 32, 8, 2
EPS = 1e-5
F32, BF16, I32 = jnp.float32, jnp.bfloat16, jnp.int32
T = 128
Q = 64
TM = 2 * T
NB = S // TM
PAD = 16
G = 32
HEAD = 2


def _gelu2(h):
    c = math.sqrt(2.0 / math.pi)
    return h + h * jnp.tanh(h * (2 * c + (8 * c * 0.044715) * (h * h)))


def _skew(parts, axis, unit):
    return [c if i == 0 else pltpu.roll(c, unit * i, axis) for i, c in enumerate(parts)]


def _unskew(parts, axis, unit):
    n = parts[0].shape[axis]
    idx = lax.broadcasted_iota(I32, parts[0].shape, axis)
    x = [parts[-j % 8] for j in range(8)]
    for b in (1, 2, 4):
        on = (idx & (b * unit)) != 0
        x = [jnp.where(on, x[(j - b) % 8], x[j]) for j in range(8)]
    return [t if j == 0 else pltpu.roll(t, n - unit * j, axis) for j, t in enumerate(x)]


_LHS = (((1, 0, 0), (1, 1, 1)), ((1, 1, 0), (1, 1, 1)), ((1, 0, 0),), ((1, 1, 1),),
        ((1, 0, 0), (1, 0, 1)), ((1, 1, 0), (-1, 0, 0)), ((1, 0, 1), (-1, 1, 1)))
_RHS = (((1, 0, 0), (1, 1, 1)), ((1, 0, 0),), ((1, 0, 1), (-1, 1, 1)), ((1, 1, 0), (-1, 0, 0)),
        ((1, 1, 1),), ((1, 0, 0), (1, 0, 1)), ((1, 1, 0), (1, 1, 1)))
_ORDER = (6, 3, 1, 0, 4, 2, 5)


def _combine(terms, get):
    v = get(*terms[0][1:])
    for sign, a, b in terms[1:]:
        v = (lax.add if sign > 0 else lax.sub)(v, get(a, b))
    return v


def _seven(table, quad):
    return [_combine(terms, lambda a, b: quad[2 * a + b]) for terms in table]


def _sum(xs):
    return functools.reduce(lax.add, xs)


def _cost(tasks):
    return sum(c for c, _ in tasks)


def _overlap(main, *sides):
    total, t, ev = _cost(main), 0.0, []
    for c, f in main:
        ev.append((t / total, 1, f))
        t += c
    for side, lo, hi, *timed in sides:
        ev += [(when, 0, f) for events in timed for when, f in events]
        total, t = _cost(side), 0.0
        for c, f in side:
            ev.append((lo + (hi - lo) * t / total, 0, f))
            t += c
    for _, _, f in sorted(ev, key=lambda e: e[:2]):
        f()


def _stagger(stages):
    n, out = len(stages[0]), []
    for k in range(n + len(stages) - 1):
        now = [st[k - s] for s, st in enumerate(stages) if 0 <= k - s < n]
        now = [((j + 0.5) / len(g), s, t) for s, g in enumerate(now) for j, t in enumerate(g)]
        out += [t for _, _, t in sorted(now, key=lambda e: e[:2])]
    return out


def _run(tasks):
    for _, f in tasks:
        f()


def _tile(c):
    return slice(c * T, (c + 1) * T)


def _ds(start, n, align=8):
    if isinstance(start, int):
        return pl.ds(lax.add(np.int32(start), np.int32(0)), n)
    return pl.ds(pl.multiple_of(start, align), n)


class _Operand:
    def __init__(self, ref, base, levels, rows, nt):
        self.ref, self.base, self.levels, self.rows, self.nt = ref, base, levels, rows, nt

    @staticmethod
    def size(levels, rows, nt):
        return (7 ** levels * nt + 1) // 2 * rows // 2

    def shifted(self, i, step, most=None):
        size = self.size(self.levels, self.rows, self.nt) - (most or self.rows - step) // 2
        return _Operand(self.ref.at[_ds(self.base + i * (step // 2), size)], 0, self.levels, self.rows, self.nt)

    def at(self, j, r, c, n):
        g = j * self.nt + c
        return _ds(self.base + g // 2 * self.rows // 2 + r // 2, n // 2), _tile(g % 2)

    def put(self, r, c, mats, first=0):
        for j, t in enumerate(mats):
            self.ref[self.at(first + j, r, c, t.shape[0])] = pltpu.bitcast(lax.convert_element_type(t, BF16), I32)

    def rhs(self, j, c, ks):
        return pltpu.bitcast(self.ref[self.at(j, ks[0] * T, c, len(ks) * T)], BF16)

    def lhs(self, j, ks, zeros):
        cols = [self.ref[self.at(j, 0, c, self.rows)] for c in ks]
        for z in zeros:
            cols[-1] = jnp.concatenate([cols[-1][:-8], cols[-1][-8:] | z], 0)
        return jnp.concatenate([pltpu.bitcast(c, BF16) for c in cols], 1)


_EARLY = dict(wq=(1, D // 2, 4), wk=(1, D // 2, 4), wv=(1, D // 2, 4), wo=(1, D // 2, 4),
              xa=(1, T, 4), xb=(1, T, 4), oa=(1, T, 4))
_LATE = dict(wd2=(2, 3 * T, 2), wd1=(1, T, 4), sa2=(2, Q, 4), sa1=(1, T, 8))
_MLP = dict(win=(2, D // 4, 7), ha=(2, Q, 2), ya2=(2, Q, 3), ya1=(1, T, 1))
_Z2 = dict(z22=(2, S // 4, 3), z21=(1, S // 2, 1))


def _rows(*tables):
    return max(sum(_Operand.size(*s) for s in t.values()) for t in tables) + 8


def _kernel(x_hbm, wqkv_hbm, wo_hbm, win_hbm, wsp_hbm, b_hbm, wout_hbm, out_hbm,
            x_v, raw_a, raw_b, ops_v, mlp_v, z2_v, p_v, qk0, v0, qk1, v1, h_v, gz_v, z1_v, stat_v,
            bias_v, b_v, sems, osem, bar, *small):
    stage_v, tmp_v, perm_v = small[:6], small[6:8], small[8:]
    op = {}
    for ref, table in ((ops_v, _EARLY), (ops_v, _LATE), (mlp_v, _MLP), (z2_v, _Z2)):
        top = 0
        for name, shape in table.items():
            op[name] = _Operand(ref, top, *shape)
            top += _Operand.size(*shape)
    xa, xb, ha = op['xa'], op['xb'], op['ha']
    hb = _Operand(mlp_v, op['ya2'].base, *_MLP['ha'])

    zero = lax.fori_loop(0, 2, lambda _, c: c ^ 1, 0)
    last, paced, pending = [None], {}, []
    ready, busy = {}, [False]

    def pace(ref):
        if last[0] is None or paced.get(id(ref)) is last[0]:
            return
        paced[id(ref)] = last[0]
        n = 8 if ref.dtype == F32 else 16
        ref[_ds(zero * n + (ref.shape[0] - n), n, n), 0:T] = last[0][0:n].astype(ref.dtype)

    for ref in (ops_v, mlp_v, z2_v):
        ref[_ds(ref.shape[0] - 8, 8), 0:T] = jnp.zeros((8, T), I32)

    def due(ref, *times):
        def run():
            pending.append(ref[_ds(zero * 8 + (ref.shape[0] - 8), 8), 0:T])
        return [(when, run) for when in times]

    def barrier():
        pl.semaphore_signal(bar, 1)
        pl.semaphore_wait(bar, 1)

    def products(lhs, rhs, u, emit, ks, level, first):
        if level == 0:
            def run():
                last[0] = jnp.dot(lhs.lhs(first, ks, pending), rhs.rhs(first, u, ks), preferred_element_type=F32)
                pending.clear()
                emit(0, 0, last[0])
            return [(len(ks) * lhs.rows / 4, run)]
        h = 2 ** (level - 1)
        state = {(i, j): [None, None] for i in range(h) for j in range(h)}

        def step(n):
            def take(i, j, m):
                s = state[i, j]
                if n == 0:
                    s[0] = m
                elif n == 1:
                    s[:] = s[0] + m, m
                elif n == 2:
                    emit(h + i, j, m + s[1])
                    s[1] = m
                elif n == 3:
                    s[:] = s[0] + m, m - s[1]
                elif n == 4:
                    emit(i, j, s[0] - m)
                    s[0] = m
                elif n == 5:
                    emit(i, h + j, m + s[0])
                    s[1] = s[1] + m
                else:
                    emit(h + i, h + j, s[1] + m)
            return take
        return [t for n, r in enumerate(_ORDER) for t in products(lhs, rhs, u, step(n), ks, level - 1, first * 7 + r)]

    def unit(lhs, rhs, u, emit, ks=None):
        return products(lhs, rhs, u, lambda a, b, v: emit(a * lhs.rows, b, v), ks or range(lhs.nt), lhs.levels, 0)

    def expand2(table, ref, get, dst, r, c):
        def task(r1):
            def run():
                pace(ref)
                quad = [_combine(table[r1], lambda a, b: get(2 * a + i, 2 * b + j)) for i in (0, 1) for j in (0, 1)]
                dst.put(r, c, _seven(table, quad), 7 * r1)
            return (3, run)
        return [task(r1) for r1 in _ORDER]

    def layer_norm(src, load, nt, stat, gain=1.0):
        def mean(r):
            def run():
                assert ready.get(id(src), True)
                pace(src)
                m = jnp.sum(_sum([load(r, c) for c in range(nt)]), axis=-1, keepdims=True) * (1.0 / (nt * T))
                stat_v[_ds(stat + r, 16), :] = jnp.broadcast_to(m, (16, T))
            return (nt / 2, run)

        def rstd(r):
            def run():
                pace(src)
                m = stat_v[_ds(stat + r, 16), :]
                v = [load(r, c) - m for c in range(nt)]
                var = jnp.sum(_sum([t * t for t in v]), axis=-1, keepdims=True) * (1.0 / (nt * T))
                inv = lax.rsqrt(var + EPS)
                stat_v[_ds(stat + TM + r, 16), :] = jnp.broadcast_to(inv if gain == 1.0 else gain * inv, (16, T))
            return (3 * nt / 4, run)

        def norm(r, c):
            m, inv = stat_v[_ds(stat + r, 16), :], stat_v[_ds(stat + TM + r, 16), :]
            return (load(r, c) - m) * inv
        return [f(r) for f in (mean, rstd) for r in range(0, TM, 16)], norm

    def raw_tile(ref, r, c):
        return ref[_ds(r, 16, 16), _tile(c)]

    def x_blk(i):
        return x_v.at[_ds(i * TM, TM, 16)]

    def h_blk(i):
        return h_v.at[_ds(i * TM, 7 * S + TM)]

    def ln_x(i, dst):
        x = x_blk(i)
        stats, norm = layer_norm(x_v, lambda r, c: raw_tile(x, r, c).astype(F32), 8, 0)

        def task(r, c):
            def run():
                pace(x_v)
                dst.put(r, c, _seven(_LHS, [norm(a + r, b + c) for a in (0, T) for b in (0, 4)]))
            return (5, run)
        return stats, [task(r, c) for r in range(0, T, 16) for c in range(4)]

    def ln_h(i, dst):
        h = h_blk(i)
        stats, norm = layer_norm(h_v, lambda r, c: h[_ds(c * S + r, 16), :], 8, 2 * TM, 0.5)
        return stats, [t for c in range(2) for r in range(0, Q, 16) for t in expand2(
            _LHS, h_v, lambda a, b, r=r, c=c: norm(a * Q + r, 2 * b + c), dst, r, c)]

    def ln_z(i, gz):
        stats, norm = layer_norm(gz, lambda r, c: gz[_ds(c * TM + r, 16), :], 14, 4 * TM)
        z21, z22 = op['z21'].shifted(i, T), op['z22'].shifted(i, Q)

        def task(r):
            def run():
                pace(gz)
                z21.put(r, 0, _seven(_RHS, [norm(a + r, c) for a in (0, T) for c in (12, 13)]))
            return (4, run)
        return stats, [task(r) for r in range(0, T, 16)] + [
            t for c in range(3) for r in range(0, Q, 16) for t in expand2(
                _RHS, gz, lambda a, b, r=r, c=c: norm(a * Q + r, 3 * b + c), z22, r, c)]

    def win_prep(i, n):
        src, dst = raw_b.at[_ds(i * n, 3 * D // 4 + n, 16)], op['win'].shifted(i, n)
        return [t for r in range(0, n, 16) for u in range(7) for t in expand2(
            _RHS, raw_b, lambda a, b, r=r, u=u: raw_tile(src, a * (D // 4) + r, 7 * b + u).astype(F32), dst, r, u)]

    def wd_tile(src, k, r, c):
        return raw_tile(src, k % 7 * T + r, k // 7 * 8 + c).astype(F32)

    def wd_prep1():
        def task(r, c):
            def run():
                pace(raw_b)
                op['wd1'].put(r, c, _seven(_RHS, [wd_tile(raw_b, k, r, b + c) for k in (12, 13) for b in (0, 4)]))
            return (3.5, run)
        return [task(r, c) for c in range(4) for r in range(0, T, 16)]

    def wd_prep2(i):
        src, dst = raw_b.at[_ds(i * 32, 6 * T + 32, 16)], op['wd2'].shifted(i, 32, 96)
        return [t for r in (0, 16) for k in range(3) for u in range(2) for t in expand2(
            _RHS, raw_b, lambda a, b, r=r, k=k, u=u: wd_tile(src, 3 * a + k, r, 4 * u + b), dst, k * T + r, u)]

    def sp_prep1(i):
        src = raw_a.at[_ds(i * TM, TM, 16)]

        def task(r, b):
            def run():
                pace(raw_a)
                op['sa1'].put(r, b, _seven(_LHS, [raw_tile(src, a + r, 2 * b + c).astype(F32)
                                                  for a in (0, T) for c in (0, 1)]))
            return (3.5, run)
        return [task(r, b) for b in range(NB) for r in range(0, T, 16)]

    def sp_prep2(i):
        src = raw_a.at[_ds(i * TM, TM, 16)]

        def gather(ref, r, c, a):
            def run():
                pace(raw_a)
                low, out = lax.broadcasted_iota(I32, (8, T), 1) < Q, []
                for half in (0, 1):
                    u, v = (pltpu.bitcast(raw_tile(src, a * Q + r, 4 * c + 2 * k + half), I32) for k in (0, 1))
                    out += [jnp.where(low, u, pltpu.roll(v, Q, 1)), jnp.where(low, pltpu.roll(u, Q, 1), v)]
                for b, t in enumerate([pltpu.bitcast(t, BF16).astype(F32) for t in out]):
                    ref[_ds((4 * a + b) * 16, 16), :] = t
            return (2, run)
        jobs = [(tmp_v[r // 16 % 2], r, c) for c in range(4) for r in range(0, Q, 16)]
        return _stagger([[[gather(*job, a) for a in range(4)] for job in jobs],
                         [expand2(_LHS, ref, lambda a, b, ref=ref: ref[_ds((4 * a + b) * 16, 16), :], op['sa2'], r, c)
                          for ref, r, c in jobs]])

    def qkv_prep(t, k):
        def where(stage, r):
            return perm_v[2 * stage + r // G % 2], (r // (D // 2) * G + r % G) * 4

        def drop(stage, r, vals):
            ref, o = where(stage, r)
            for c, v in enumerate(vals):
                ref[_ds(o + 8 * c, 8), :] = pltpu.bitcast(v, F32)

        def grab(stage, r, cs):
            ref, o = where(stage, r)
            pace(ref)
            return [pltpu.bitcast(ref[_ds(o + 8 * c, 8), :], I32) for c in cs]

        def skew(r):
            def run():
                pace(raw_a)
                drop(0, r, _skew([pltpu.bitcast(raw_tile(raw_a, t // 2 * D + r, t % 2 * 8 + c), I32)
                                  for c in range(8)], 1, 2))
            return (3, run)

        def unskew(r):
            return (4, lambda: drop(1, r, _unskew(grab(0, r, range(8)), 1, 2)))

        def store(r, c):
            def run():
                op['w' + 'qkv'[t]].put(r, c, _seven(_RHS, [
                    pltpu.bitcast(p, BF16).astype(F32) for a in (0, D // 2) for p in grab(1, a + r, (c, 4 + c))]))
            return (3, run)
        gs = range(k * T, (k + 1) * T, G)
        return [[[f(a + r) for r in range(g, g + G, 16) for a in (0, D // 2)] for g in gs]
                for f in (skew, unskew)] + [[[store(r, c) for r in range(g, g + G, 16) for c in range(4)] for g in gs]]

    def wo_prep():
        def task(g, c):
            def run():
                pace(raw_a)
                hv = [[pltpu.bitcast(p, BF16).astype(F32) for p in _unskew(_skew(
                    [pltpu.bitcast(raw_tile(raw_a, D + i * T + g, 8 + b + c), I32) for i in range(8)], 0, 1), 0, 1)]
                    for b in (0, 4)]
                for j in range(4):
                    op['wo'].put(j * T + g, c, _seven(_RHS, [hv[0][j], hv[1][j], hv[0][4 + j], hv[1][4 + j]]))
            return (22, run)
        return [task(g, c) for c in range(4) for g in range(0, T, 16)]

    def bias_prep():
        def task(k):
            def run():
                bias_v[_ds(k * T, T), :] = jnp.broadcast_to(b_v[...].astype(F32)[k:k + 1, :], (T, T)).T
            return (4, run)
        return [task(k) for k in range(S // T)]

    def row(c, r):
        return c * (TM + PAD) + PAD + r

    def qkv(lhs, bufs, which, ks=range(4), first=False):
        tasks = []
        for t in which:
            for u in range(4):
                def emit(a, b, v, t=t, u=u):
                    ref, c = bufs[t // 2], t % 2 * 8 + 4 * b + u
                    if ks[0]:
                        v = v + ref[_ds(row(c, a), T), :]
                    ref[_ds(row(c, a), T), :] = v
                    ready[id(ref)] = t > 0 and ks[-1] == 3 and (u, a, b) == (3, T, 1)
                    if first and t and a == 0:
                        ref[_ds(row(c, -PAD), PAD), :] = jnp.broadcast_to(v[0:1], (PAD, T))
                tasks += unit(lhs, op['w' + 'qkv'[t]], u, emit, ks)
        return tasks

    def history(src, dst, *which):
        def run():
            for t in which:
                for c in range(t % 2 * 8, t % 2 * 8 + 8):
                    dst[t // 2][_ds(row(c, -PAD), PAD), :] = src[t // 2][_ds(row(c, TM - PAD), PAD), :]
        return [(0, run)]

    scale = DH ** -0.5

    def slot(stage, w, r):
        return stage_v[2 * stage + r // Q % 2], (w * 2 + r // T) * Q + r % Q

    def grab(where, r):
        pace(where(0, r)[0])
        return [ref[_ds(o, 8), :] for ref, o in (where(w, r) for w in range(W))]

    def drop(where, r, vals):
        for w, t in enumerate(vals):
            ref, o = where(w, r)
            ref[_ds(o, 8), :] = t

    def by_group(f):
        return [[f(a + r) for a in (0, T) for r in range(g, g + Q, 8)] for g in (0, Q)]

    raw, prob, mixed = (functools.partial(slot, s) for s in range(3))

    def logits(bufs, dst, first=False):
        qk = bufs[0]

        def scores(r):
            def run():
                assert ready[id(qk)]
                pace(qk)
                q = [qk[_ds(row(c, r), 8), :] for c in range(8)]
                drop(raw, r, (_sum([lax.mul(q[c], qk[_ds(row(8 + c, r - DIL * w), 8), :]) for c in range(8)])
                              for w in range(W)))
            return (15, run)

        def fold(r):
            def run():
                ps = grab(raw, r)
                for bit in (16, 1):
                    low = (lax.broadcasted_iota(I32, (8, T), 1) & bit) == 0
                    ps = [p + jnp.where(low, pltpu.roll(p, T - bit, 1), pltpu.roll(p, bit, 1)) for p in ps]
                if first and r < DIL * W:
                    pos = lax.broadcasted_iota(I32, (8, T), 0) + r
                    ps = [jnp.where(pos >= DIL * w, p, -1e9 / scale) for w, p in enumerate(ps)]
                drop(lambda w, r: (dst, w * TM + r), r, ps)
            return (8, run)
        return _stagger([by_group(scores), by_group(fold)])

    def attend(bufs, src):
        v = bufs[1]

        def softmax(r):
            def run():
                lg = grab(lambda w, r: (src, w * TM + r), r)
                m = functools.reduce(jnp.maximum, lg)
                e = [jnp.exp2((p - m) * (scale * math.log2(math.e))) for p in lg]
                inv = 1.0 / _sum(e)
                drop(prob, r, [t * inv for t in e])
            return (7, run)

        def mix(r):
            def run():
                assert ready[id(v)]
                pace(v)
                p = grab(prob, r)
                drop(mixed, r, (_sum([lax.mul(p[w], v[_ds(row(c, r - DIL * w), 8), :]) for w in range(W)])
                                for c in range(8)))
            return (15, run)

        def combo(r):
            def run():
                assert not busy[0]
                pace(mixed(0, r)[0])
                for c in range(4):
                    op['oa'].put(r, c, _seven(_LHS, [ref[_ds(o, 16), :] for ref, o in (
                        mixed(b + c, a + r) for a in (0, T) for b in (0, 4))]))
            return (8, run)
        return _stagger([by_group(softmax), by_group(mix), [[combo(g + r) for r in range(0, Q, 16)] for g in (0, Q)]])

    def proj(i):
        tasks, x, h = [], x_blk(i), h_blk(i)
        for u in range(4):
            def emit(a, b, v, u=u):
                c = 4 * b + u
                busy[0] = (u, a, b) != (3, T, 1)
                h[_ds(c * S + a, T), :] = x[_ds(a, T), _tile(c)].astype(F32) + v
            tasks += unit(op['oa'], op['wo'], u, emit)
        return tasks

    def z1_blk(i):
        return z1_v.at[_ds(i * T, 3 * S + T)]

    def z1_at(c, r, n):
        return _ds((c // 2 * S + r) // 2, n // 2), _tile(c % 2)

    def up(i, lhs, gz):
        tasks, z1 = [], z1_blk(i)
        for u in range(7):
            def emit(a, b, v, u=u):
                c = 7 * (b % 2) + u
                ready[id(gz)] = (u, a, b) == (6, 3 * Q, 3)
                if b < 2:
                    z1[z1_at(c, a, Q)] = pltpu.bitcast(v.astype(BF16), I32)
                else:
                    gz[_ds(c * TM + a, Q), :] = _gelu2(v)
            tasks += unit(lhs, op['win'], u, emit)
        return tasks

    def gate_head():
        def park(c):
            def emit(a, b, v):
                qk1[_ds(c(b) * TM + a, v.shape[0]), :] = v
            return emit
        tasks = unit(op['sa1'], op['z21'], 0, park(lambda b: 12 + b), range(2 * HEAD))
        for u in range(3):
            tasks += unit(op['sa2'], op['z22'], u, park(lambda b, u=u: 3 * b + u), range(HEAD))
        return tasks

    def gate_step(i, _, rest=False):
        last[0] = None
        z1, h, out, bias = z1_blk(i), h_blk(i), x_blk(i), bias_v.at[_ds(i * TM, TM)]
        extra = [(wd_prep2(3), 0.0, 0.244)] if rest else []

        def gated(c, r, v):
            n = v.shape[0]
            if rest:
                v = v + qk1[_ds(c * TM + r, n), :]
            return _gelu2(pltpu.bitcast(z1[z1_at(c, r, n)], BF16).astype(F32)) * (v + bias[_ds(r, n), :])

        y = {}

        def gate1(a, b, v):
            y[a, b] = gated(12 + b, a, v)
            if len(y) == 4:
                op['ya1'].put(0, 0, _seven(_LHS, [y[0, 0], y[0, 1], y[T, 0], y[T, 1]]))
        main, marks, sides = unit(op['sa1'], op['z21'], 0, gate1, range(2 * HEAD * rest, 8)), [], []
        for u in range(3):
            ref = (v0, v1)[u % 2]

            def gate2(a, b, v, u=u, ref=ref):
                ref[_ds(4 * a + b * Q, Q), :] = gated(3 * b + u, a, v)
            marks.append(_cost(main))
            main += unit(op['sa2'], op['z22'], u, gate2, range(HEAD * rest, 4))
            side = [expand2(_LHS, ref, lambda a, b, r=r, ref=ref: ref[_ds((4 * a + b) * Q + r, 16), :],
                            op['ya2'], r, u) for r in range(0, Q, 16)]
            sides.append([t for ts in zip(*side) for t in ts])
        marks.append(_cost(main))
        for u in range(4):
            def down1(a, b, v, u=u):
                at = _ds((4 * b + u) * S + a, T)
                h[at, :] = h[at, :] + v
            main += unit(op['ya1'], op['wd1'], u, down1)
        marks.append(_cost(main))
        for u in range(2):
            def down2(a, b, v, u=u):
                c = 4 * u + b
                out[_ds(a, Q), _tile(c)] = (h[_ds(c * S + a, Q), :] + v).astype(BF16)
                if a % T == Q and b % 2 == 1:
                    at = _ds(i * TM + a - Q, T, 16), slice((c - 1) * T, (c + 1) * T)
                    pltpu.make_async_copy(x_v.at[at], out_hbm.at[at], osem).start()
            main += unit(op['ya2'], op['wd2'], u, down2)
        t = [(m + 1) / _cost(main) for m in marks]
        span = (0.99, 0.99, 0.789) if rest else (0.453, 0.593, 0.911)
        nxt = i + 1 if rest else jnp.minimum(i + 1, NB - 1)
        _overlap(main, *[(s, t[u + 1], t[u + 1] + span[u] * (t[u + 2] - t[u + 1])) for u, s in enumerate(sides)],
                 (sp_prep1(nxt), t[0], 0.97 if rest else 0.6), (sp_prep2(nxt), t[4], 0.98, due(ops_v, 0.99)), *extra)
        last[0] = None

    cur, alt = (qk0, v0), (qk1, v1)

    def attn_step(i, _):
        last[0] = None
        if isinstance(i, int):
            stats, sums = ln_h(0, ha)
            extra = [(stats, 0.299, 0.51), (sums, 0.51, 0.98, due(mlp_v, 0.99)),
                     (win_prep(3, 64), 0.0, 0.806, due(mlp_v, 0.25, 0.45, 0.65, 0.85))]
        else:
            stats, sums = ln_x(i + 1, xa)
            extra = [(stats, 0.379, 0.75), (sums, 0.751, 0.96, due(ops_v, 0.99)),
                     (win_prep(i - 3, 48), 0.001, 0.95, due(mlp_v, 0.25, 0.45, 0.619, 0.85))]
        _overlap(history(cur, cur, 1) + qkv(xa, cur, (0, 1)) + history(cur, cur, 2) + qkv(xa, cur, (2,)) + proj(i - 1),
                 (attend(cur, p_v), 0.0, 0.49), (logits(cur, p_v), 0.501, 0.888), *extra)
        last[0] = None

    def up_step(j, _):
        last[0] = None
        i, sides = 2 * j + 1, []
        for t, z, h in ((0.0, ln_z(i - 1, gz_v), ln_h(i + 1, ha)), (0.501, ln_z(i, qk1), ln_h(i + 2, hb))):
            sides += [(z[0], t, t + 0.13), (z[1], t + 0.13, t + 0.331, due(z2_v, t + 0.331 + 0.022)),
                      (h[0], t + 0.25, t + 0.347), (h[1], t + 0.347, t + 0.47)]
        wd = wd_prep2(j)
        _overlap(up(i, hb, qk1) + up(i + 1, ha, gz_v), *sides, ([], 0, 0, due(mlp_v, 0.99)),
                 *[(wd[k * len(wd) // 2:(k + 1) * len(wd) // 2], t + 0.011, t + 0.119, due(ops_v, t + 0.119 + 0.01))
                   for k, t in enumerate((0.0, 0.5))])
        last[0] = None

    copies = {}

    def start(key, src, dst):
        copies[key] = pltpu.make_async_copy(src, dst, sems.at[len(copies)])
        copies[key].start()

    def wait(*keys):
        for k in keys:
            copies[k].wait()

    def start_rows(t, k):
        for r in (k * T, D // 2 + k * T):
            start((t, r), wqkv_hbm.at[r:r + T, t * D:(t + 1) * D],
                  raw_a.at[t // 2 * D + r:t // 2 * D + r + T, t % 2 * D:(t % 2 + 1) * D])

    def start_x(lo, hi):
        start(('x', lo), x_hbm.at[lo * TM:hi * TM], x_v.at[lo * TM:hi * TM])

    queue = [lambda: start_rows(0, 0), lambda: start_x(0, 1), lambda: start_x(1, 2),
             *[functools.partial(start_rows, t, k) for t in range(3) for k in range(4)][1:],
             lambda: start('wo', wo_hbm, raw_a.at[D:2 * D, D:2 * D]), lambda: start_x(2, 3), lambda: start_x(3, 4),
             lambda: start('win', win_hbm, raw_b.at[0:D]), lambda: start_x(4, NB), lambda: start('b', b_hbm, b_v)]

    def more(n):
        for _ in range(min(n, len(queue))):
            queue.pop(0)()

    def arrive(*chunks, ahead=0):
        wait(*[(t, a + k * T) for t, k in chunks for a in (0, D // 2)])
        more(len(chunks) + ahead)
        return _stagger([sum(st, []) for st in zip(*[qkv_prep(t, k) for t, k in chunks])])

    more(5)
    _run(arrive((0, 0)))
    wait(('x', 0))
    more(1)
    _run(sum(ln_x(0, xa), []))
    wait(('x', 1))
    more(1)
    _overlap(qkv(xa, cur, (0,), [0]), (sum(ln_x(1, xb), []), 0.0, 0.86))
    _overlap(qkv(xb, alt, (0,), [0]), (arrive((0, 1)), 0.0, 0.8))
    for t, ks, chunks, ahead, hi in (
            (0, [1], [(0, 2)], 0, 0.85), (0, [2], [(0, 3)], 0, 0.85), (0, [3], [(1, 0), (1, 1)], 0, 0.97),
            (1, [0, 1], [(1, 2), (1, 3)], 2, 0.745), (1, [2, 3], [(2, 0), (2, 1), (2, 2)], 0, 0.963)):
        _overlap(qkv(xa, cur, (t,), ks, True) + qkv(xb, alt, (t,), ks),
                 (arrive(*chunks, ahead=ahead), 0.0, hi, due(ops_v, 0.98)))
    side = arrive((2, 3), ahead=len(queue))
    wait('wo', ('x', 2))
    _overlap(qkv(xa, cur, (2,), [0, 1, 2], True) + qkv(xa, cur, (2,), [3], True) + history(cur, alt, 1, 2)
             + qkv(xb, alt, (2,)),
             (side, 0.0, 0.31), (logits(cur, p_v, True), 0.0, 0.7),
             (sum(ln_x(2, xa), []), 0.501, 0.95, due(ops_v, 0.985)), (wo_prep()[:16], 0.2, 0.6, due(ops_v, 0.6 + 0.05)))
    wait(('x', 3))
    stats, sums = ln_x(3, xa)
    _overlap(history(alt, cur, 1) + qkv(xa, cur, (0, 1)) + proj(0) + history(alt, cur, 2) + qkv(xa, cur, (2,)) + proj(1),
             (attend(cur, p_v), 0.0, 0.39), (wo_prep()[16:], 0.0, 0.39),
             (logits(alt, gz_v), 0.025, 0.464), (attend(alt, gz_v), 0.464, 0.79), (logits(cur, p_v), 0.55, 0.905),
             (stats, 0.4, 0.8), (sums, 0.801, 0.95, due(ops_v, 0.99)))
    wait('win', ('x', 4), 'b')
    start('wsp', wsp_hbm, raw_a.at[0:S])
    lax.fori_loop(3, NB - 1, attn_step, None)
    attn_step(NB - 1, None)
    for k in range(2):
        start(('wd', k), wout_hbm.at[k * FH // 2:(k + 1) * FH // 2], raw_b.at[0:FH // 2, k * D:(k + 1) * D])
    barrier()
    _overlap(up(0, ha, gz_v) + proj(NB - 1), (attend(cur, p_v), 0.0, 0.559),
             (sum(ln_h(1, hb), []) + bias_prep(), 0.55, 0.95, due(mlp_v, 0.97)))
    wait('wsp', ('wd', 0), ('wd', 1))
    lax.fori_loop(0, NB // 2 - 1, up_step, None)
    z6, z7 = ln_z(NB - 2, gz_v), ln_z(NB - 1, qk0)
    main = up(NB - 1, hb, qk0), gate_head()
    mid = (_cost(main[0]) + 1) / _cost(main[0] + main[1])
    _overlap(main[0] + main[1], (z6[0], 0.0, 0.15), (z6[1], 0.15, 0.459, due(z2_v, 0.5)),
             (wd_prep1() + sp_prep1(0), 0.0, 0.2, due(ops_v, 0.2 + 0.04)), (sp_prep2(0), 0.458, 0.696),
             (z7[0], mid, 0.783), (z7[1], 0.783, 0.97, due(z2_v, 0.99)))
    barrier()
    gate_step(0, None, True)
    lax.fori_loop(1, NB, gate_step, None)
    pltpu.make_async_copy(x_v.at[0:S], out_hbm, osem).wait()


@jax.jit
def pallas_sequential_preLN__sliding_local_dilated__mixer_gmlp__prompt_kernel(
        A_x, A_wqkv, A_wo, B_x, B_w_in, B_w_sp, B_b_sp, B_w_out):
    del B_x
    hbm, vm = pl.BlockSpec(memory_space=pl.ANY), pltpu.VMEM
    out = pl.pallas_call(
        _kernel,
        out_shape=jax.ShapeDtypeStruct((S, D), BF16),
        in_specs=[hbm] * 7,
        out_specs=hbm,
        scratch_shapes=[
            vm((S + PAD, D), BF16),
            vm((S + PAD, S), BF16),
            vm((D + PAD, 2 * FH), BF16),
            vm((_rows(_EARLY, _LATE), 2 * T), I32), vm((_rows(_MLP), 2 * T), I32), vm((_rows(_Z2), 2 * T), I32),
            vm((W * TM + PAD, T), F32),
            *[vm((n * (TM + PAD) + PAD, T), F32) for n in (16, 8, 16, 8)],
            vm((8 * S + PAD, T), F32), vm((14 * TM + PAD, T), F32), vm((7 * S // 2, 2 * T), I32),
            vm((6 * TM, T), F32), vm((S, T), F32), vm((S // T, T), BF16),
            pltpu.SemaphoreType.DMA((36,)), pltpu.SemaphoreType.DMA(()), pltpu.SemaphoreType.REGULAR(()),
            *[vm((16 * Q + 8, T), F32)] * 6, *[vm((16 * 16 + 8, T), F32)] * 2, *[vm((8 * G + 8, T), F32)] * 4,
        ],
        compiler_params=pltpu.CompilerParams(vmem_limit_bytes=126 * 1024 * 1024),
    )(A_x.reshape(S, D), A_wqkv, A_wo, B_w_in, B_w_sp, B_b_sp.reshape(S // T, T), B_w_out)
    return out.reshape(1, S, D)
```

```python
import functools
import math

import numpy as np
import jax
import jax.numpy as jnp
from jax import lax
import jax.experimental.pallas as pl
import jax.experimental.pallas.tpu as pltpu

S, D, FH = 2048, 1024, 1792
DH, W, DIL = 32, 8, 2
EPS = 1e-5
F32, BF16, I32 = jnp.float32, jnp.bfloat16, jnp.int32
T = 128
Q = 64
TM = 2 * T
NB = S // TM
PAD = 16
G = 32
HEAD = 2


def _gelu2(h):
    c = math.sqrt(2.0 / math.pi)
    return h + h * jnp.tanh(h * (2 * c + (8 * c * 0.044715) * (h * h)))


def _skew(parts, axis, unit):
    return [c if i == 0 else pltpu.roll(c, unit * i, axis) for i, c in enumerate(parts)]


def _unskew(parts, axis, unit):
    n = parts[0].shape[axis]
    idx = lax.broadcasted_iota(I32, parts[0].shape, axis)
    x = [parts[-j % 8] for j in range(8)]
    for b in (1, 2, 4):
        on = (idx & (b * unit)) != 0
        x = [jnp.where(on, x[(j - b) % 8], x[j]) for j in range(8)]
    return [t if j == 0 else pltpu.roll(t, n - unit * j, axis) for j, t in enumerate(x)]


_LHS = (((1, 0, 0), (1, 1, 1)), ((1, 1, 0), (1, 1, 1)), ((1, 0, 0),), ((1, 1, 1),),
        ((1, 0, 0), (1, 0, 1)), ((1, 1, 0), (-1, 0, 0)), ((1, 0, 1), (-1, 1, 1)))
_RHS = (((1, 0, 0), (1, 1, 1)), ((1, 0, 0),), ((1, 0, 1), (-1, 1, 1)), ((1, 1, 0), (-1, 0, 0)),
        ((1, 1, 1),), ((1, 0, 0), (1, 0, 1)), ((1, 1, 0), (1, 1, 1)))
_ORDER = (6, 3, 1, 0, 4, 2, 5)


def _combine(terms, get):
    v = get(*terms[0][1:])
    for sign, a, b in terms[1:]:
        v = (lax.add if sign > 0 else lax.sub)(v, get(a, b))
    return v


def _seven(table, quad):
    return [_combine(terms, lambda a, b: quad[2 * a + b]) for terms in table]


def _sum(xs):
    return functools.reduce(lax.add, xs)


def _cost(tasks):
    return sum(c for c, _ in tasks)


def _merge(main, *sides):
    span, t, ev = _cost(main), 0.0, []
    for c, f in main:
        ev.append((t / span, 1, c / span, f))
        t += c
    for side, lo, hi, *timed in sides:
        ev += [(when, 0, 0.0, f) for events in timed for when, f in events]
        total, t = _cost(side), 0.0
        for c, f in side:
            ev.append((lo + (hi - lo) * t / total, 0, 0.0, f))
            t += c
    t0, span = 0.0, 1.0
    for when, _, c, f in sorted(ev, key=lambda e: e[:2]):
        if c:
            t0, span = when, c
        yield min(0.999, (when - t0) / span), f


def _stagger(stages):
    n, out = len(stages[0]), []
    for k in range(n + len(stages) - 1):
        now = [st[k - s] for s, st in enumerate(stages) if 0 <= k - s < n]
        now = [((j + 0.5) / len(g), s, t) for s, g in enumerate(now) for j, t in enumerate(g)]
        out += [t for _, _, t in sorted(now, key=lambda e: e[:2])]
    return out


def _run(tasks):
    for _, f in tasks:
        f()


def _tile(c):
    return slice(c * T, (c + 1) * T)


def _ds(start, n, align=8):
    if isinstance(start, int):
        return pl.ds(lax.add(np.int32(start), np.int32(0)), n)
    return pl.ds(pl.multiple_of(start, align), n)


class _Operand:
    def __init__(self, ref, base, levels, rows, nt):
        self.ref, self.base, self.levels, self.rows, self.nt = ref, base, levels, rows, nt

    @staticmethod
    def size(levels, rows, nt):
        return (7 ** levels * nt + 1) // 2 * rows // 2

    def shifted(self, i, step, most=None):
        size = self.size(self.levels, self.rows, self.nt) - (most or self.rows - step) // 2
        return _Operand(self.ref.at[_ds(self.base + i * (step // 2), size)], 0, self.levels, self.rows, self.nt)

    def at(self, j, r, c, n):
        g = j * self.nt + c
        return _ds(self.base + g // 2 * self.rows // 2 + r // 2, n // 2), _tile(g % 2)

    def put(self, r, c, mats, first=0):
        for j, t in enumerate(mats):
            self.ref[self.at(first + j, r, c, t.shape[0])] = pltpu.bitcast(lax.convert_element_type(t, BF16), I32)

    def rhs(self, j, c, ks):
        return pltpu.bitcast(self.ref[self.at(j, ks[0] * T, c, len(ks) * T)], BF16)

    def lhs(self, j, ks, zeros):
        cols = [self.ref[self.at(j, 0, c, self.rows)] for c in ks]
        for z in zeros:
            cols[-1] = jnp.concatenate([cols[-1][:-8], cols[-1][-8:] | z], 0)
        return jnp.concatenate([pltpu.bitcast(c, BF16) for c in cols], 1)


_EARLY = dict(wq=(1, D // 2, 4), wk=(1, D // 2, 4), wv=(1, D // 2, 4), wo=(1, D // 2, 4),
              xa=(1, T, 4), xb=(1, T, 4), oa=(1, T, 4))
_LATE = dict(wd2=(2, 3 * T, 2), wd1=(1, T, 4), sa2=(2, Q, 4), sa1=(1, T, 8))
_MLP = dict(win=(2, D // 4, 7), ha=(2, Q, 2), ya2=(2, Q, 3), ya1=(1, T, 1))
_Z2 = dict(z22=(2, S // 4, 3), z21=(1, S // 2, 1))


def _rows(*tables):
    return max(sum(_Operand.size(*s) for s in t.values()) for t in tables) + 8


def _kernel(x_hbm, wqkv_hbm, wo_hbm, win_hbm, wsp_hbm, b_hbm, wout_hbm, out_hbm,
            x_v, raw_a, raw_b, ops_v, mlp_v, z2_v, p_v, qk0, v0, qk1, v1, h_v, gz_v, z1_v, stat_v,
            bias_v, b_v, sems, osem, bar, *small):
    stage_v, tmp_v, perm_v = small[:6], small[6:8], small[8:]
    op = {}
    for ref, table in ((ops_v, _EARLY), (ops_v, _LATE), (mlp_v, _MLP), (z2_v, _Z2)):
        top = 0
        for name, shape in table.items():
            op[name] = _Operand(ref, top, *shape)
            top += _Operand.size(*shape)
    xa, xb, ha = op['xa'], op['xb'], op['ha']
    hb = _Operand(mlp_v, op['ya2'].base, *_MLP['ha'])

    zero = lax.fori_loop(0, 2, lambda _, c: c ^ 1, 0)
    last, phase, paced, pending = [None], [0.0], {}, []
    ready, busy = {}, [False]

    def overlap(main, *sides):
        for phase[0], f in _merge(main, *sides):
            f()

    def pace(ref):
        if last[0] is None:
            return
        r = int(phase[0] * (last[0].shape[0] // 32)) * 32
        old = paced.get(id(ref), (None, 0))
        if old[0] is not last[0] or old[1] != r:
            paced[id(ref)] = last[0], r
            n = 8 if ref.dtype == F32 else 16
            ref[_ds(zero * n + (ref.shape[0] - n), n, n), 0:T] = last[0][r:r + n].astype(ref.dtype)

    for ref in (ops_v, mlp_v, z2_v):
        ref[_ds(ref.shape[0] - 8, 8), 0:T] = jnp.zeros((8, T), I32)

    def due(ref, *times):
        def run():
            pending.append(ref[_ds(zero * 8 + (ref.shape[0] - 8), 8), 0:T])
        return [(when, run) for when in times]

    def barrier():
        pl.semaphore_signal(bar, 1)
        pl.semaphore_wait(bar, 1)

    def products(lhs, rhs, u, emit, ks, level, first):
        if level == 0:
            def run():
                last[0] = jnp.dot(lhs.lhs(first, ks, pending), rhs.rhs(first, u, ks), preferred_element_type=F32)
                pending.clear()
                emit(0, 0, last[0])
            return [(len(ks) * lhs.rows / 4, run)]
        h = 2 ** (level - 1)
        state = {(i, j): [None, None] for i in range(h) for j in range(h)}

        def step(n):
            def take(i, j, m):
                s = state[i, j]
                if n == 0:
                    s[0] = m
                elif n == 1:
                    s[:] = s[0] + m, m
                elif n == 2:
                    emit(h + i, j, m + s[1])
                    s[1] = m
                elif n == 3:
                    s[:] = s[0] + m, m - s[1]
                elif n == 4:
                    emit(i, j, s[0] - m)
                    s[0] = m
                elif n == 5:
                    emit(i, h + j, m + s[0])
                    s[1] = s[1] + m
                else:
                    emit(h + i, h + j, s[1] + m)
            return take
        return [t for n, r in enumerate(_ORDER) for t in products(lhs, rhs, u, step(n), ks, level - 1, first * 7 + r)]

    def unit(lhs, rhs, u, emit, ks=None):
        return products(lhs, rhs, u, lambda a, b, v: emit(a * lhs.rows, b, v), ks or range(lhs.nt), lhs.levels, 0)

    def expand2(table, ref, get, dst, r, c):
        def task(r1):
            def run():
                pace(ref)
                quad = [_combine(table[r1], lambda a, b: get(2 * a + i, 2 * b + j)) for i in (0, 1) for j in (0, 1)]
                dst.put(r, c, _seven(table, quad), 7 * r1)
            return (3, run)
        return [task(r1) for r1 in _ORDER]

    def layer_norm(src, load, nt, stat, gain=1.0):
        def mean(r):
            def run():
                assert ready.get(id(src), True)
                pace(src)
                m = jnp.sum(_sum([load(r, c) for c in range(nt)]), axis=-1, keepdims=True) * (1.0 / (nt * T))
                stat_v[_ds(stat + r, 16), :] = jnp.broadcast_to(m, (16, T))
            return (nt / 2, run)

        def rstd(r):
            def run():
                pace(src)
                m = stat_v[_ds(stat + r, 16), :]
                v = [load(r, c) - m for c in range(nt)]
                var = jnp.sum(_sum([t * t for t in v]), axis=-1, keepdims=True) * (1.0 / (nt * T))
                inv = lax.rsqrt(var + EPS)
                stat_v[_ds(stat + TM + r, 16), :] = jnp.broadcast_to(inv if gain == 1.0 else gain * inv, (16, T))
            return (3 * nt / 4, run)

        def norm(r, c):
            m, inv = stat_v[_ds(stat + r, 16), :], stat_v[_ds(stat + TM + r, 16), :]
            return (load(r, c) - m) * inv
        return [f(r) for f in (mean, rstd) for r in range(0, TM, 16)], norm

    def raw_tile(ref, r, c):
        return ref[_ds(r, 16, 16), _tile(c)]

    def x_blk(i):
        return x_v.at[_ds(i * TM, TM, 16)]

    def h_blk(i):
        return h_v.at[_ds(i * TM, 7 * S + TM)]

    def ln_x(i, dst):
        x = x_blk(i)
        stats, norm = layer_norm(x_v, lambda r, c: raw_tile(x, r, c).astype(F32), 8, 0)

        def task(r, c):
            def run():
                pace(x_v)
                dst.put(r, c, _seven(_LHS, [norm(a + r, b + c) for a in (0, T) for b in (0, 4)]))
            return (5, run)
        return stats, [task(r, c) for r in range(0, T, 16) for c in range(4)]

    def ln_h(i, dst):
        h = h_blk(i)
        stats, norm = layer_norm(h_v, lambda r, c: h[_ds(c * S + r, 16), :], 8, 2 * TM, 0.5)
        return stats, [t for c in range(2) for r in range(0, Q, 16) for t in expand2(
            _LHS, h_v, lambda a, b, r=r, c=c: norm(a * Q + r, 2 * b + c), dst, r, c)]

    def ln_z(i, gz):
        stats, norm = layer_norm(gz, lambda r, c: gz[_ds(c * TM + r, 16), :], 14, 4 * TM)
        z21, z22 = op['z21'].shifted(i, T), op['z22'].shifted(i, Q)

        def task(r):
            def run():
                pace(gz)
                z21.put(r, 0, _seven(_RHS, [norm(a + r, c) for a in (0, T) for c in (12, 13)]))
            return (4, run)
        return stats, [task(r) for r in range(0, T, 16)] + [
            t for c in range(3) for r in range(0, Q, 16) for t in expand2(
                _RHS, gz, lambda a, b, r=r, c=c: norm(a * Q + r, 3 * b + c), z22, r, c)]

    def win_prep(i, n):
        src, dst = raw_b.at[_ds(i * n, 3 * D // 4 + n, 16)], op['win'].shifted(i, n)
        return [t for r in range(0, n, 16) for u in range(7) for t in expand2(
            _RHS, raw_b, lambda a, b, r=r, u=u: raw_tile(
                src, a * (D // 4) + r, 14 * (b % 2) + 7 * (b // 2) + u).astype(F32), dst, r, u)]

    def wd_tile(src, k, r, c):
        return raw_tile(src, k % 7 * T + r, k // 7 * 8 + c).astype(F32)

    def wd_prep1():
        def task(r, c):
            def run():
                pace(raw_b)
                op['wd1'].put(r, c, _seven(_RHS, [wd_tile(raw_b, k, r, b + c) for k in (12, 13) for b in (0, 4)]))
            return (3.5, run)
        return [task(r, c) for c in range(4) for r in range(0, T, 16)]

    def wd_prep2(i):
        src, dst = raw_b.at[_ds(i * 32, 6 * T + 32, 16)], op['wd2'].shifted(i, 32, 96)
        return [t for r in (0, 16) for k in range(3) for u in range(2) for t in expand2(
            _RHS, raw_b, lambda a, b, r=r, k=k, u=u: wd_tile(src, 3 * a + k, r, 4 * u + b), dst, k * T + r, u)]

    def sp_prep1(i):
        src = raw_a.at[_ds(i * TM, TM, 16)]

        def task(r, b):
            def run():
                pace(raw_a)
                op['sa1'].put(r, b, _seven(_LHS, [raw_tile(src, a + r, 2 * b + c).astype(F32)
                                                  for a in (0, T) for c in (0, 1)]))
            return (3.5, run)
        return [task(r, b) for b in range(NB) for r in range(0, T, 16)]

    def sp_prep2(i):
        src = raw_a.at[_ds(i * TM, TM, 16)]

        def gather(ref, r, c, a):
            def run():
                pace(raw_a)
                low, out = lax.broadcasted_iota(I32, (8, T), 1) < Q, []
                for half in (0, 1):
                    u, v = (pltpu.bitcast(raw_tile(src, a * Q + r, 4 * c + 2 * k + half), I32) for k in (0, 1))
                    out += [jnp.where(low, u, pltpu.roll(v, Q, 1)), jnp.where(low, pltpu.roll(u, Q, 1), v)]
                for b, t in enumerate([pltpu.bitcast(t, BF16).astype(F32) for t in out]):
                    ref[_ds((4 * a + b) * 16, 16), :] = t
            return (2, run)
        jobs = [(tmp_v[r // 16 % 2], r, c) for c in range(4) for r in range(0, Q, 16)]
        return _stagger([[[gather(*job, a) for a in range(4)] for job in jobs],
                         [expand2(_LHS, ref, lambda a, b, ref=ref: ref[_ds((4 * a + b) * 16, 16), :], op['sa2'], r, c)
                          for ref, r, c in jobs]])

    def qkv_prep(t, k):
        def where(stage, r):
            return perm_v[2 * stage + r // G % 2], (r // (D // 2) * G + r % G) * 4

        def drop(stage, r, vals):
            ref, o = where(stage, r)
            for c, v in enumerate(vals):
                ref[_ds(o + 8 * c, 8), :] = pltpu.bitcast(v, F32)

        def grab(stage, r, cs):
            ref, o = where(stage, r)
            pace(ref)
            return [pltpu.bitcast(ref[_ds(o + 8 * c, 8), :], I32) for c in cs]

        def skew(r):
            def run():
                pace(raw_a)
                drop(0, r, _skew([pltpu.bitcast(raw_tile(raw_a, t // 2 * D + r, t % 2 * 8 + c), I32)
                                  for c in range(8)], 1, 2))
            return (3, run)

        def unskew(r):
            return (4, lambda: drop(1, r, _unskew(grab(0, r, range(8)), 1, 2)))

        def store(r, c):
            def run():
                op['w' + 'qkv'[t]].put(r, c, _seven(_RHS, [
                    pltpu.bitcast(p, BF16).astype(F32) for a in (0, D // 2) for p in grab(1, a + r, (c, 4 + c))]))
            return (3, run)
        gs = range(k * T, (k + 1) * T, G)
        return [[[f(a + r) for r in range(g, g + G, 16) for a in (0, D // 2)] for g in gs]
                for f in (skew, unskew)] + [[[store(r, c) for r in range(g, g + G, 16) for c in range(4)] for g in gs]]

    def wo_prep(*cs):
        def swap(g, c, ref, b):
            def run():
                pace(raw_a)
                parts = [pltpu.bitcast(raw_tile(raw_a, D + i * T + g, 8 + 4 * b + c), I32) for i in range(8)]
                for j, p in enumerate(_unskew(_skew(parts, 0, 1), 0, 1)):
                    ref[_ds((b * 8 + j) * 8, 8), :] = pltpu.bitcast(p, F32)
            return (5, run)

        def store(g, c, ref, j):
            def run():
                pace(ref)
                op['wo'].put(j * T + g, c, _seven(_RHS, [
                    pltpu.bitcast(pltpu.bitcast(ref[_ds((b * 8 + a + j) * 8, 8), :], I32), BF16).astype(F32)
                    for a in (0, 4) for b in (0, 1)]))
            return (3, run)
        jobs = [(g, c, tmp_v[g // 16 % 2]) for c in cs for g in range(0, T, 16)]
        return _stagger([[[swap(*job, b) for b in (0, 1)] for job in jobs],
                         [[store(*job, j) for j in range(4)] for job in jobs]])

    def bias_prep():
        def task(k):
            def run():
                bias_v[_ds(k * T, T), :] = jnp.broadcast_to(b_v[...].astype(F32)[k:k + 1, :], (T, T)).T
            return (4, run)
        return [task(k) for k in range(S // T)]

    def row(c, r):
        return c * (TM + PAD) + PAD + r

    def qkv(lhs, bufs, which, ks=range(4), first=False):
        tasks = []
        for t in which:
            for u in range(4):
                def emit(a, b, v, t=t, u=u):
                    ref, c = bufs[t // 2], t % 2 * 8 + 4 * b + u
                    if ks[0]:
                        v = v + ref[_ds(row(c, a), T), :]
                    ref[_ds(row(c, a), T), :] = v
                    ready[id(ref)] = t > 0 and ks[-1] == 3 and (u, a, b) == (3, T, 1)
                    if first and t and a == 0:
                        ref[_ds(row(c, -PAD), PAD), :] = jnp.broadcast_to(v[0:1], (PAD, T))
                tasks += unit(lhs, op['w' + 'qkv'[t]], u, emit, ks)
        return tasks

    def history(src, dst, *which):
        def run():
            for t in which:
                for c in range(t % 2 * 8, t % 2 * 8 + 8):
                    dst[t // 2][_ds(row(c, -PAD), PAD), :] = src[t // 2][_ds(row(c, TM - PAD), PAD), :]
        return [(0, run)]

    scale = DH ** -0.5

    def slot(stage, w, r):
        return stage_v[2 * stage + r // Q % 2], (w * 2 + r // T) * Q + r % Q

    def grab(where, r, ws=range(W)):
        pace(where(0, r)[0])
        return [ref[_ds(o, 8), :] for ref, o in (where(w, r) for w in ws)]

    def drop(where, r, vals, first=0):
        for w, t in enumerate(vals, first):
            ref, o = where(w, r)
            ref[_ds(o, 8), :] = t

    def by_group(f, n=8):
        return [[f(a + r, range(k, k + n)) for a in (0, T) for r in range(g, g + Q, 8) for k in range(0, 8, n)]
                for g in (0, Q)]

    raw, prob, mixed = (functools.partial(slot, s) for s in range(3))

    def logits(bufs, dst, first=False):
        qk = bufs[0]

        def scores(r, ws):
            def run():
                assert ready[id(qk)]
                pace(qk)
                q = [qk[_ds(row(c, r), 8), :] for c in range(8)]
                drop(raw, r, (_sum([lax.mul(q[c], qk[_ds(row(8 + c, r - DIL * w), 8), :]) for c in range(8)])
                              for w in ws), ws[0])
            return (3.75, run)

        def fold(r, ws):
            def run():
                ps = grab(raw, r, ws)
                for bit in (16, 1):
                    low = (lax.broadcasted_iota(I32, (8, T), 1) & bit) == 0
                    ps = [p + jnp.where(low, pltpu.roll(p, T - bit, 1), pltpu.roll(p, bit, 1)) for p in ps]
                if first and r < DIL * W:
                    pos = lax.broadcasted_iota(I32, (8, T), 0) + r
                    ps = [jnp.where(pos >= DIL * w, p, -1e9 / scale) for w, p in zip(ws, ps)]
                drop(lambda w, r: (dst, w * TM + r), r, ps, ws[0])
            return (11.849 / 2, run)
        return _stagger([by_group(scores, 2), by_group(fold, 4)])

    def attend(bufs, src):
        v = bufs[1]

        def softmax(r, _):
            def run():
                lg = grab(lambda w, r: (src, w * TM + r), r)
                m = functools.reduce(jnp.maximum, lg)
                e = [jnp.exp2((p - m) * (scale * math.log2(math.e))) for p in lg]
                inv = 1.0 / _sum(e)
                drop(prob, r, [t * inv for t in e])
            return (7, run)

        def mix(r, cs):
            def run():
                assert ready[id(v)]
                pace(v)
                p = grab(prob, r)
                drop(mixed, r, (_sum([lax.mul(p[w], v[_ds(row(c, r - DIL * w), 8), :]) for w in range(W)])
                                for c in cs), cs[0])
            return (3.75, run)

        def combo(r, c):
            def run():
                pace(mixed(0, r)[0])
                assert not busy[0]
                op['oa'].put(r, c, _seven(_LHS, [ref[_ds(o, 16), :] for ref, o in (
                    mixed(b + c, a + r) for a in (0, T) for b in (0, 4))]))
            return (2, run)
        return _stagger([by_group(softmax), by_group(mix, 2),
                         [[combo(g + r, c) for r in range(0, Q, 16) for c in range(4)] for g in (0, Q)]])

    def proj(i):
        tasks, x, h = [], x_blk(i), h_blk(i)
        for u in range(4):
            def emit(a, b, v, u=u):
                c = 4 * b + u
                busy[0] = (u, a, b) != (3, T, 1)
                h[_ds(c * S + a, T), :] = x[_ds(a, T), _tile(c)].astype(F32) + v
            tasks += unit(op['oa'], op['wo'], u, emit)
        return tasks

    def z1_blk(i):
        return z1_v.at[_ds(i * T, 3 * S + T)]

    def z1_at(c, r, n):
        return _ds((c // 2 * S + r) // 2, n // 2), _tile(c % 2)

    def up(i, lhs, gz):
        tasks, z1 = [], z1_blk(i)
        for u in range(7):
            def emit(a, b, v, u=u):
                c = 7 * (b // 2) + u
                ready[id(gz)] = (u, a, b) == (6, 3 * Q, 3)
                if b % 2 == 0:
                    z1[z1_at(c, a, Q)] = pltpu.bitcast(v.astype(BF16), I32)
                else:
                    gz[_ds(c * TM + a, Q), :] = _gelu2(v)
            tasks += unit(lhs, op['win'], u, emit)
        return tasks

    def gate_head():
        def park(c):
            def emit(a, b, v):
                qk1[_ds(c(b) * TM + a, v.shape[0]), :] = v
            return emit
        tasks = unit(op['sa1'], op['z21'], 0, park(lambda b: 12 + b), range(2 * HEAD))
        for u in range(3):
            tasks += unit(op['sa2'], op['z22'], u, park(lambda b, u=u: 3 * b + u), range(HEAD))
        return tasks

    def gate_step(i, _, rest=False):
        last[0] = None
        z1, h, out, bias = z1_blk(i), h_blk(i), x_blk(i), bias_v.at[_ds(i * TM, TM)]
        extra = [(wd_prep2(3), 0.0, 0.244)] if rest else []

        def gated(c, r, v):
            n = v.shape[0]
            if rest:
                v = v + qk1[_ds(c * TM + r, n), :]
            return _gelu2(pltpu.bitcast(z1[z1_at(c, r, n)], BF16).astype(F32)) * (v + bias[_ds(r, n), :])

        y = {}

        def gate1(a, b, v):
            y[a, b] = gated(12 + b, a, v)
            if len(y) == 4:
                op['ya1'].put(0, 0, _seven(_LHS, [y[0, 0], y[0, 1], y[T, 0], y[T, 1]]))
        main, marks, sides = unit(op['sa1'], op['z21'], 0, gate1, range(2 * HEAD * rest, 8)), [], []
        for u in range(3):
            ref = (v0, v1)[u % 2]

            def gate2(a, b, v, u=u, ref=ref):
                ref[_ds(4 * a + b * Q, Q), :] = gated(3 * b + u, a, v)
            marks.append(_cost(main))
            main += unit(op['sa2'], op['z22'], u, gate2, range(HEAD * rest, 4))
            side = [expand2(_LHS, ref, lambda a, b, r=r, ref=ref: ref[_ds((4 * a + b) * Q + r, 16), :],
                            op['ya2'], r, u) for r in range(0, Q, 16)]
            sides.append([t for ts in zip(*side) for t in ts])
        marks.append(_cost(main))
        for u in range(4):
            def down1(a, b, v, u=u):
                at = _ds((4 * b + u) * S + a, T)
                h[at, :] = h[at, :] + v
            main += unit(op['ya1'], op['wd1'], u, down1)
        marks.append(_cost(main))
        for u in range(2):
            def down2(a, b, v, u=u):
                c = 4 * u + b
                out[_ds(a, Q), _tile(c)] = (h[_ds(c * S + a, Q), :] + v).astype(BF16)
                if a % T == Q and b % 2 == 1:
                    at = _ds(i * TM + a - Q, T, 16), slice((c - 1) * T, (c + 1) * T)
                    pltpu.make_async_copy(x_v.at[at], out_hbm.at[at], osem).start()
            main += unit(op['ya2'], op['wd2'], u, down2)
        t = [(m + 1) / _cost(main) for m in marks]
        span = (0.99, 0.99, 0.789) if rest else (0.453, 0.593, 0.911)
        nxt = i + 1 if rest else jnp.minimum(i + 1, NB - 1)
        overlap(main, *[(s, t[u + 1], t[u + 1] + span[u] * (t[u + 2] - t[u + 1])) for u, s in enumerate(sides)],
                 (sp_prep1(nxt), t[0], 0.97 if rest else 0.6), (sp_prep2(nxt), t[4], 0.98, due(ops_v, 0.99)), *extra)
        last[0] = None

    cur, alt = (qk0, v0), (qk1, v1)

    def attn_step(i, _):
        last[0] = None
        if isinstance(i, int):
            stats, sums = ln_h(0, ha)
            extra = [(stats, 0.29, 0.51), (sums, 0.51, 0.879, due(mlp_v, 0.99)),
                     (win_prep(3, 64), 0.0, 0.962, due(mlp_v, 0.25, 0.45, 0.65, 0.85))]
        else:
            stats, sums = ln_x(i + 1, xa)
            extra = [(stats, 0.299, 0.718), (sums, 0.751, 0.98, due(ops_v, 0.99)),
                     (win_prep(i - 3, 48), 0.001, 0.885, due(mlp_v, 0.25, 0.45, 0.619, 0.85))]
        overlap(history(cur, cur, 1) + qkv(xa, cur, (0, 1)) + history(cur, cur, 2) + qkv(xa, cur, (2,)) + proj(i - 1),
                 (attend(cur, p_v), 0.0, 0.492), (logits(cur, p_v), 0.501, 0.848), *extra)
        last[0] = None

    def up_step(j, _):
        last[0] = None
        i, sides = 2 * j + 1, []
        for t, z, h in ((0.0, ln_z(i - 1, gz_v), ln_h(i + 1, ha)), (0.501, ln_z(i, qk1), ln_h(i + 2, hb))):
            sides += [(z[0], t, t + 0.13), (z[1], t + 0.13, t + 0.331, due(z2_v, t + 0.331 + 0.022)),
                      (h[0], t + 0.25, t + 0.347), (h[1], t + 0.347, t + 0.47)]
        wd = wd_prep2(j)
        overlap(up(i, hb, qk1) + up(i + 1, ha, gz_v), *sides, ([], 0, 0, due(mlp_v, 0.99)),
                 *[(wd[k * len(wd) // 2:(k + 1) * len(wd) // 2], t + 0.011, t + 0.135, due(ops_v, t + 0.135 + 0.01))
                   for k, t in enumerate((0.0, 0.5))])
        last[0] = None

    copies = {}

    def start(key, src, dst):
        copies[key] = pltpu.make_async_copy(src, dst, sems.at[len(copies)])
        copies[key].start()

    def wait(*keys):
        for k in keys:
            copies[k].wait()

    def start_rows(t, k):
        for r in (k * T, D // 2 + k * T):
            start((t, r), wqkv_hbm.at[r:r + T, t * D:(t + 1) * D],
                  raw_a.at[t // 2 * D + r:t // 2 * D + r + T, t % 2 * D:(t % 2 + 1) * D])

    def start_x(lo, hi):
        start(('x', lo), x_hbm.at[lo * TM:hi * TM], x_v.at[lo * TM:hi * TM])

    queue = [lambda: start_rows(0, 0), lambda: start_x(0, 1), lambda: start_x(1, 2),
             *[functools.partial(start_rows, t, k) for t in range(3) for k in range(4)][1:],
             lambda: start('wo', wo_hbm, raw_a.at[D:2 * D, D:2 * D]), lambda: start_x(2, 3), lambda: start_x(3, 4),
             lambda: start('win', win_hbm, raw_b.at[0:D]), lambda: start_x(4, NB), lambda: start('b', b_hbm, b_v)]

    def more(n):
        for _ in range(min(n, len(queue))):
            queue.pop(0)()

    def arrive(*chunks, ahead=0):
        wait(*[(t, a + k * T) for t, k in chunks for a in (0, D // 2)])
        more(len(chunks) + ahead)
        return _stagger([sum(st, []) for st in zip(*[qkv_prep(t, k) for t, k in chunks])])

    more(5)
    _run(arrive((0, 0)))
    wait(('x', 0))
    more(1)
    _run(sum(ln_x(0, xa), []))
    wait(('x', 1))
    more(1)
    overlap(qkv(xa, cur, (0,), [0]), (sum(ln_x(1, xb), []), 0.0, 0.86))
    overlap(qkv(xb, alt, (0,), [0]), (arrive((0, 1)), 0.0, 0.8))
    for t, ks, chunks, ahead, hi in (
            (0, [1], [(0, 2)], 0, 0.85), (0, [2], [(0, 3)], 0, 0.85), (0, [3], [(1, 0), (1, 1)], 0, 0.97),
            (1, [0, 1], [(1, 2), (1, 3)], 2, 0.745), (1, [2, 3], [(2, 0), (2, 1), (2, 2)], 0, 0.963)):
        overlap(qkv(xa, cur, (t,), ks, True) + qkv(xb, alt, (t,), ks),
                 (arrive(*chunks, ahead=ahead), 0.0, hi, due(ops_v, 0.98)))
    side = arrive((2, 3), ahead=len(queue))
    wait('wo', ('x', 2))
    overlap(qkv(xa, cur, (2,), [0, 1, 2], True) + qkv(xa, cur, (2,), [3], True) + history(cur, alt, 1, 2)
             + qkv(xb, alt, (2,)),
             (side, 0.0, 0.306), (logits(cur, p_v, True), 0.0, 0.839),
             (sum(ln_x(2, xa), []), 0.501, 0.878, due(ops_v, 0.985)),
            (wo_prep(0, 1), 0.2, 0.66, due(ops_v, 0.66 + 0.05)))
    wait(('x', 3))
    stats, sums = ln_x(3, xa)
    overlap(history(alt, cur, 1) + qkv(xa, cur, (0, 1)) + proj(0) + history(alt, cur, 2) + qkv(xa, cur, (2,)) + proj(1),
             (attend(cur, p_v), 0.0, 0.395), (wo_prep(2, 3), 0.0, 0.39),
             (logits(alt, gz_v), 0.025, 0.464), (attend(alt, gz_v), 0.464, 0.79), (logits(cur, p_v), 0.55, 0.905),
             (stats, 0.4, 0.8), (sums, 0.801, 0.95, due(ops_v, 0.99)))
    wait('win', ('x', 4), 'b')
    start('wsp', wsp_hbm, raw_a.at[0:S])
    lax.fori_loop(3, NB - 1, attn_step, None)
    attn_step(NB - 1, None)
    for k in range(2):
        start(('wd', k), wout_hbm.at[k * FH // 2:(k + 1) * FH // 2], raw_b.at[0:FH // 2, k * D:(k + 1) * D])
    barrier()
    overlap(up(0, ha, gz_v) + proj(NB - 1), (attend(cur, p_v), 0.0, 0.591),
             (sum(ln_h(1, hb), []) + bias_prep(), 0.429, 0.967, due(mlp_v, 0.97)))
    wait('wsp', ('wd', 0), ('wd', 1))
    lax.fori_loop(0, NB // 2 - 1, up_step, None)
    z6, z7 = ln_z(NB - 2, gz_v), ln_z(NB - 1, qk0)
    main = up(NB - 1, hb, qk0), gate_head()
    mid = (_cost(main[0]) + 1) / _cost(main[0] + main[1])
    overlap(main[0] + main[1], (z6[0], 0.0, 0.15), (z6[1], 0.15, 0.445, due(z2_v, 0.5)),
             (wd_prep1() + sp_prep1(0), 0.0, 0.2, due(ops_v, 0.2 + 0.04)), (sp_prep2(0), 0.448, 0.696),
             (z7[0], mid, 0.783), (z7[1], 0.783, 0.97, due(z2_v, 0.99)))
    barrier()
    gate_step(0, None, True)
    lax.fori_loop(1, NB, gate_step, None)
    pltpu.make_async_copy(x_v.at[0:S], out_hbm, osem).wait()


@jax.jit
def pallas_sequential_preLN__sliding_local_dilated__mixer_gmlp__prompt_kernel(
        A_x, A_wqkv, A_wo, B_x, B_w_in, B_w_sp, B_b_sp, B_w_out):
    del B_x
    hbm, vm = pl.BlockSpec(memory_space=pl.ANY), pltpu.VMEM
    out = pl.pallas_call(
        _kernel,
        out_shape=jax.ShapeDtypeStruct((S, D), BF16),
        in_specs=[hbm] * 7,
        out_specs=hbm,
        scratch_shapes=[
            vm((S + PAD, D), BF16),
            vm((S + PAD, S), BF16),
            vm((D + PAD, 2 * FH), BF16),
            vm((_rows(_EARLY, _LATE), 2 * T), I32), vm((_rows(_MLP), 2 * T), I32), vm((_rows(_Z2), 2 * T), I32),
            vm((W * TM + PAD, T), F32),
            *[vm((n * (TM + PAD) + PAD, T), F32) for n in (16, 8, 16, 8)],
            vm((8 * S + PAD, T), F32), vm((14 * TM + PAD, T), F32), vm((7 * S // 2, 2 * T), I32),
            vm((6 * TM, T), F32), vm((S, T), F32), vm((S // T, T), BF16),
            pltpu.SemaphoreType.DMA((36,)), pltpu.SemaphoreType.DMA(()), pltpu.SemaphoreType.REGULAR(()),
            *[vm((16 * Q + 8, T), F32)] * 6, *[vm((16 * 16 + 8, T), F32)] * 2, *[vm((8 * G + 8, T), F32)] * 4,
        ],
        compiler_params=pltpu.CompilerParams(vmem_limit_bytes=126 * 1024 * 1024),
    )(A_x.reshape(S, D), A_wqkv, A_wo, B_w_in, B_w_sp, B_b_sp.reshape(S // T, T), B_w_out)
    return out.reshape(1, S, D)
```

```python
import functools
import math

import numpy as np
import jax
import jax.numpy as jnp
from jax import lax
import jax.experimental.pallas as pl
import jax.experimental.pallas.tpu as pltpu

S, D, FH = 2048, 1024, 1792
DH, W, DIL = 32, 8, 2
EPS = 1e-5
F32, BF16, I32 = jnp.float32, jnp.bfloat16, jnp.int32
T = 128
Q = 64
TM = 2 * T
NB = S // TM
PAD = 16
G = 32
HEAD = 2


def _gelu2(h):
    c = math.sqrt(2.0 / math.pi)
    return h + h * jnp.tanh(h * (2 * c + (8 * c * 0.044715) * (h * h)))


def _skew(parts, axis, unit):
    return [c if i == 0 else pltpu.roll(c, unit * i, axis) for i, c in enumerate(parts)]


def _unskew(parts, axis, unit):
    n = parts[0].shape[axis]
    idx = lax.broadcasted_iota(I32, parts[0].shape, axis)
    x = [parts[-j % 8] for j in range(8)]
    for b in (1, 2, 4):
        on = (idx & (b * unit)) != 0
        x = [jnp.where(on, x[(j - b) % 8], x[j]) for j in range(8)]
    return [t if j == 0 else pltpu.roll(t, n - unit * j, axis) for j, t in enumerate(x)]


_LHS = (((1, 0, 0), (1, 1, 1)), ((1, 1, 0), (1, 1, 1)), ((1, 0, 0),), ((1, 1, 1),),
        ((1, 0, 0), (1, 0, 1)), ((1, 1, 0), (-1, 0, 0)), ((1, 0, 1), (-1, 1, 1)))
_RHS = (((1, 0, 0), (1, 1, 1)), ((1, 0, 0),), ((1, 0, 1), (-1, 1, 1)), ((1, 1, 0), (-1, 0, 0)),
        ((1, 1, 1),), ((1, 0, 0), (1, 0, 1)), ((1, 1, 0), (1, 1, 1)))
_ORDER = (6, 3, 1, 0, 4, 2, 5)


def _combine(terms, get):
    v = get(*terms[0][1:])
    for sign, a, b in terms[1:]:
        v = (lax.add if sign > 0 else lax.sub)(v, get(a, b))
    return v


def _seven(table, quad):
    return [_combine(terms, lambda a, b: quad[2 * a + b]) for terms in table]


def _sum(xs):
    return functools.reduce(lax.add, xs)


def _cost(tasks):
    return sum(c for c, _ in tasks)


def _merge(main, *sides):
    span, t, ev = _cost(main), 0.0, []
    for c, f in main:
        ev.append((t / span, 1, c / span, f))
        t += c
    for side, lo, hi, *timed in sides:
        ev += [(when, 0, 0.0, f) for events in timed for when, f in events]
        total, t = _cost(side), 0.0
        for c, f in side:
            ev.append((lo + (hi - lo) * t / total, 0, 0.0, f))
            t += c
    t0, span = 0.0, 1.0
    for when, _, c, f in sorted(ev, key=lambda e: e[:2]):
        if c:
            t0, span = when, c
        yield min(0.999, (when - t0) / span), f


def _stagger(stages):
    n, out = len(stages[0]), []
    for k in range(n + len(stages) - 1):
        now = [st[k - s] for s, st in enumerate(stages) if 0 <= k - s < n]
        now = [((j + 0.5) / len(g), s, t) for s, g in enumerate(now) for j, t in enumerate(g)]
        out += [t for _, _, t in sorted(now, key=lambda e: e[:2])]
    return out


def _run(tasks):
    for _, f in tasks:
        f()


def _tile(c):
    return slice(c * T, (c + 1) * T)


def _ds(start, n, align=8):
    if isinstance(start, int):
        return pl.ds(lax.add(np.int32(start), np.int32(0)), n)
    return pl.ds(pl.multiple_of(start, align), n)


class _Operand:
    def __init__(self, ref, base, levels, rows, nt):
        self.ref, self.base, self.levels, self.rows, self.nt = ref, base, levels, rows, nt

    @staticmethod
    def size(levels, rows, nt):
        return (7 ** levels * nt + 1) // 2 * rows // 2

    def shifted(self, i, step, most=None):
        size = self.size(self.levels, self.rows, self.nt) - (most or self.rows - step) // 2
        return _Operand(self.ref.at[_ds(self.base + i * (step // 2), size)], 0, self.levels, self.rows, self.nt)

    def at(self, j, r, c, n):
        g = j * self.nt + c
        return _ds(self.base + g // 2 * self.rows // 2 + r // 2, n // 2), _tile(g % 2)

    def put(self, r, c, mats, first=0):
        for j, t in enumerate(mats):
            self.ref[self.at(first + j, r, c, t.shape[0])] = pltpu.bitcast(lax.convert_element_type(t, BF16), I32)

    def rhs(self, j, c, ks):
        return pltpu.bitcast(self.ref[self.at(j, ks[0] * T, c, len(ks) * T)], BF16)

    def lhs(self, j, ks, zeros):
        cols = [self.ref[self.at(j, 0, c, self.rows)] for c in ks]
        for z in zeros:
            cols[-1] = jnp.concatenate([cols[-1][:-8], cols[-1][-8:] | z], 0)
        return jnp.concatenate([pltpu.bitcast(c, BF16) for c in cols], 1)


_EARLY = dict(wq=(1, D // 2, 4), wk=(1, D // 2, 4), wv=(1, D // 2, 4), wo=(1, D // 2, 4),
              xa=(1, T, 4), xb=(1, T, 4), oa=(1, T, 4))
_LATE = dict(wd2=(2, 3 * T, 2), wd1=(1, T, 4), sa2=(2, Q, 4), sa1=(1, T, 8))
_MLP = dict(win=(2, D // 4, 7), ha=(2, Q, 2), ya2=(2, Q, 3), ya1=(1, T, 1))
_Z2 = dict(z22=(2, S // 4, 3), z21=(1, S // 2, 1))


def _rows(*tables):
    return max(sum(_Operand.size(*s) for s in t.values()) for t in tables) + 8


def _kernel(x_hbm, wqkv_hbm, wo_hbm, win_hbm, wsp_hbm, b_hbm, wout_hbm, out_hbm,
            x_v, raw_a, raw_b, ops_v, mlp_v, z2_v, p_v, qk0, v0, qk1, v1, h_v, gz_v, z1_v, stat_v,
            bias_v, b_v, sems, osem, bar, *small):
    stage_v, tmp_v, perm_v = small[:6], small[6:8], small[8:]
    op = {}
    for ref, table in ((ops_v, _EARLY), (ops_v, _LATE), (mlp_v, _MLP), (z2_v, _Z2)):
        top = 0
        for name, shape in table.items():
            op[name] = _Operand(ref, top, *shape)
            top += _Operand.size(*shape)
    xa, xb, ha = op['xa'], op['xb'], op['ha']
    hb = _Operand(mlp_v, op['ya2'].base, *_MLP['ha'])

    zero = lax.fori_loop(0, 2, lambda _, c: c ^ 1, 0)
    last, phase, paced, pending = [None], [0.0], {}, []
    ready, busy = {}, [False]

    def overlap(main, *sides):
        for phase[0], f in _merge(main, *sides):
            f()

    def pace(ref):
        if last[0] is None:
            return
        r = int(phase[0] * (last[0].shape[0] // 32)) * 32
        old = paced.get(id(ref), (None, 0))
        if old[0] is not last[0] or old[1] != r:
            paced[id(ref)] = last[0], r
            n = 8 if ref.dtype == F32 else 16
            ref[_ds(zero * n + (ref.shape[0] - n), n, n), 0:T] = last[0][r:r + n].astype(ref.dtype)

    for ref in (ops_v, mlp_v, z2_v):
        ref[_ds(ref.shape[0] - 8, 8), 0:T] = jnp.zeros((8, T), I32)

    def due(ref, *times):
        def run():
            pending.append(ref[_ds(zero * 8 + (ref.shape[0] - 8), 8), 0:T])
        return [(when, run) for when in times]

    def barrier():
        pl.semaphore_signal(bar, 1)
        pl.semaphore_wait(bar, 1)

    def products(lhs, rhs, u, emit, ks, level, first):
        if level == 0:
            def run():
                last[0] = jnp.dot(lhs.lhs(first, ks, pending), rhs.rhs(first, u, ks), preferred_element_type=F32)
                pending.clear()
                emit(0, 0, last[0])
            return [(len(ks) * lhs.rows / 4, run)]
        h = 2 ** (level - 1)
        state = {(i, j): [None, None] for i in range(h) for j in range(h)}

        def step(n):
            def take(i, j, m):
                s = state[i, j]
                if n == 0:
                    s[0] = m
                elif n == 1:
                    s[:] = s[0] + m, m
                elif n == 2:
                    emit(h + i, j, m + s[1])
                    s[1] = m
                elif n == 3:
                    s[:] = s[0] + m, m - s[1]
                elif n == 4:
                    emit(i, j, s[0] - m)
                    s[0] = m
                elif n == 5:
                    emit(i, h + j, m + s[0])
                    s[1] = s[1] + m
                else:
                    emit(h + i, h + j, s[1] + m)
            return take
        return [t for n, r in enumerate(_ORDER) for t in products(lhs, rhs, u, step(n), ks, level - 1, first * 7 + r)]

    def unit(lhs, rhs, u, emit, ks=None):
        return products(lhs, rhs, u, lambda a, b, v: emit(a * lhs.rows, b, v), ks or range(lhs.nt), lhs.levels, 0)

    def expand2(table, ref, get, dst, r, c):
        def task(r1):
            def run():
                pace(ref)
                quad = [_combine(table[r1], lambda a, b: get(2 * a + i, 2 * b + j)) for i in (0, 1) for j in (0, 1)]
                dst.put(r, c, _seven(table, quad), 7 * r1)
            return (3, run)
        return [task(r1) for r1 in _ORDER]

    def layer_norm(src, load, nt, stat, gain=1.0):
        def mean(r):
            def run():
                assert ready.get(id(src), True)
                pace(src)
                m = jnp.sum(_sum([load(r, c) for c in range(nt)]), axis=-1, keepdims=True) * (1.0 / (nt * T))
                stat_v[_ds(stat + r, 16), :] = jnp.broadcast_to(m, (16, T))
            return (nt / 2, run)

        def rstd(r):
            def run():
                pace(src)
                m = stat_v[_ds(stat + r, 16), :]
                v = [load(r, c) - m for c in range(nt)]
                var = jnp.sum(_sum([t * t for t in v]), axis=-1, keepdims=True) * (1.0 / (nt * T))
                inv = lax.rsqrt(var + EPS)
                stat_v[_ds(stat + TM + r, 16), :] = jnp.broadcast_to(inv if gain == 1.0 else gain * inv, (16, T))
            return (3 * nt / 4, run)

        def norm(r, c):
            m, inv = stat_v[_ds(stat + r, 16), :], stat_v[_ds(stat + TM + r, 16), :]
            return (load(r, c) - m) * inv
        return [f(r) for f in (mean, rstd) for r in range(0, TM, 16)], norm

    def raw_tile(ref, r, c):
        return ref[_ds(r, 16, 16), _tile(c)]

    def x_blk(i):
        return x_v.at[_ds(i * TM, TM, 16)]

    def h_blk(i):
        return h_v.at[_ds(i * TM, 7 * S + TM)]

    def ln_x(i, dst):
        x = x_blk(i)
        stats, norm = layer_norm(x_v, lambda r, c: raw_tile(x, r, c).astype(F32), 8, 0)

        def task(r, c):
            def run():
                pace(x_v)
                dst.put(r, c, _seven(_LHS, [norm(a + r, b + c) for a in (0, T) for b in (0, 4)]))
            return (5, run)
        return stats, [task(r, c) for r in range(0, T, 16) for c in range(4)]

    def ln_h(i, dst):
        h = h_blk(i)
        stats, norm = layer_norm(h_v, lambda r, c: h[_ds(c * S + r, 16), :], 8, 2 * TM, 0.5)
        return stats, [t for c in range(2) for r in range(0, Q, 16) for t in expand2(
            _LHS, h_v, lambda a, b, r=r, c=c: norm(a * Q + r, 2 * b + c), dst, r, c)]

    def ln_z(i, gz):
        stats, norm = layer_norm(gz, lambda r, c: gz[_ds(c * TM + r, 16), :], 14, 4 * TM)
        z21, z22 = op['z21'].shifted(i, T), op['z22'].shifted(i, Q)

        def task(r):
            def run():
                pace(gz)
                z21.put(r, 0, _seven(_RHS, [norm(a + r, c) for a in (0, T) for c in (12, 13)]))
            return (4, run)
        return stats, [task(r) for r in range(0, T, 16)] + [
            t for c in range(3) for r in range(0, Q, 16) for t in expand2(
                _RHS, gz, lambda a, b, r=r, c=c: norm(a * Q + r, 3 * b + c), z22, r, c)]

    def win_prep(i, n):
        src, dst = raw_b.at[_ds(i * n, 3 * D // 4 + n, 16)], op['win'].shifted(i, n)
        return [t for r in range(0, n, 16) for u in range(7) for t in expand2(
            _RHS, raw_b, lambda a, b, r=r, u=u: raw_tile(
                src, a * (D // 4) + r, 14 * (b % 2) + 7 * (b // 2) + u).astype(F32), dst, r, u)]

    def wd_tile(src, k, r, c):
        return raw_tile(src, k % 7 * T + r, k // 7 * 8 + c).astype(F32)

    def wd_prep1():
        def task(r, c):
            def run():
                pace(raw_b)
                op['wd1'].put(r, c, _seven(_RHS, [wd_tile(raw_b, k, r, b + c) for k in (12, 13) for b in (0, 4)]))
            return (3.5, run)
        return [task(r, c) for c in range(4) for r in range(0, T, 16)]

    def wd_prep2(i):
        src, dst = raw_b.at[_ds(i * 32, 6 * T + 32, 16)], op['wd2'].shifted(i, 32, 96)
        return [t for r in (0, 16) for k in range(3) for u in range(2) for t in expand2(
            _RHS, raw_b, lambda a, b, r=r, k=k, u=u: wd_tile(src, 3 * a + k, r, 4 * u + b), dst, k * T + r, u)]

    def sp_prep1(i):
        src = raw_a.at[_ds(i * TM, TM, 16)]

        def task(r, b):
            def run():
                pace(raw_a)
                op['sa1'].put(r, b, _seven(_LHS, [raw_tile(src, a + r, 2 * b + c).astype(F32)
                                                  for a in (0, T) for c in (0, 1)]))
            return (3.5, run)
        return [task(r, b) for b in range(NB) for r in range(0, T, 16)]

    def sp_prep2(i):
        src = raw_a.at[_ds(i * TM, TM, 16)]

        def gather(ref, r, c, a):
            def run():
                pace(raw_a)
                low, out = lax.broadcasted_iota(I32, (8, T), 1) < Q, []
                for half in (0, 1):
                    u, v = (pltpu.bitcast(raw_tile(src, a * Q + r, 4 * c + 2 * k + half), I32) for k in (0, 1))
                    out += [jnp.where(low, u, pltpu.roll(v, Q, 1)), jnp.where(low, pltpu.roll(u, Q, 1), v)]
                for b, t in enumerate([pltpu.bitcast(t, BF16).astype(F32) for t in out]):
                    ref[_ds((4 * a + b) * 16, 16), :] = t
            return (2, run)
        jobs = [(tmp_v[r // 16 % 2], r, c) for c in range(4) for r in range(0, Q, 16)]
        return _stagger([[[gather(*job, a) for a in range(4)] for job in jobs],
                         [expand2(_LHS, ref, lambda a, b, ref=ref: ref[_ds((4 * a + b) * 16, 16), :], op['sa2'], r, c)
                          for ref, r, c in jobs]])

    def qkv_prep(t, k):
        def where(stage, r):
            return perm_v[2 * stage + r // G % 2], (r // (D // 2) * G + r % G) * 4

        def drop(stage, r, vals):
            ref, o = where(stage, r)
            for c, v in enumerate(vals):
                ref[_ds(o + 8 * c, 8), :] = pltpu.bitcast(v, F32)

        def grab(stage, r, cs):
            ref, o = where(stage, r)
            pace(ref)
            return [pltpu.bitcast(ref[_ds(o + 8 * c, 8), :], I32) for c in cs]

        def skew(r):
            def run():
                pace(raw_a)
                drop(0, r, _skew([pltpu.bitcast(raw_tile(raw_a, t // 2 * D + r, t % 2 * 8 + c), I32)
                                  for c in range(8)], 1, 2))
            return (3, run)

        def unskew(r):
            return (4, lambda: drop(1, r, _unskew(grab(0, r, range(8)), 1, 2)))

        def store(r, c):
            def run():
                op['w' + 'qkv'[t]].put(r, c, _seven(_RHS, [
                    pltpu.bitcast(p, BF16).astype(F32) for a in (0, D // 2) for p in grab(1, a + r, (c, 4 + c))]))
            return (3, run)
        gs = range(k * T, (k + 1) * T, G)
        return [[[f(a + r) for r in range(g, g + G, 16) for a in (0, D // 2)] for g in gs]
                for f in (skew, unskew)] + [[[store(r, c) for r in range(g, g + G, 16) for c in range(4)] for g in gs]]

    def wo_prep(*cs):
        def swap(g, c, ref, b):
            def run():
                pace(raw_a)
                parts = [pltpu.bitcast(raw_tile(raw_a, D + i * T + g, 8 + b + 2 * c), I32) for i in range(8)]
                for j, p in enumerate(_unskew(_skew(parts, 0, 1), 0, 1)):
                    ref[_ds((b * 8 + j) * 8, 8), :] = pltpu.bitcast(p, F32)
            return (5, run)

        def store(g, c, ref, j):
            def run():
                pace(ref)
                op['wo'].put(j * T + g, c, _seven(_RHS, [
                    pltpu.bitcast(pltpu.bitcast(ref[_ds((b * 8 + a + j) * 8, 8), :], I32), BF16).astype(F32)
                    for a in (0, 4) for b in (0, 1)]))
            return (3, run)
        jobs = [(g, c, tmp_v[g // 16 % 2]) for c in cs for g in range(0, T, 16)]
        return _stagger([[[swap(*job, b) for b in (0, 1)] for job in jobs],
                         [[store(*job, j) for j in range(4)] for job in jobs]])

    def bias_prep():
        def task(k):
            def run():
                bias_v[_ds(k * T, T), :] = jnp.broadcast_to(b_v[...].astype(F32)[k:k + 1, :], (T, T)).T
            return (4, run)
        return [task(k) for k in range(S // T)]

    def row(c, r):
        return c * (TM + PAD) + PAD + r

    def qkv(lhs, bufs, which, ks=range(4), first=False):
        tasks = []
        for t in which:
            for u in range(4):
                def emit(a, b, v, t=t, u=u):
                    ref, c = bufs[t // 2], t % 2 * 8 + 4 * b + u
                    if ks[0]:
                        v = v + ref[_ds(row(c, a), T), :]
                    ref[_ds(row(c, a), T), :] = v
                    ready[id(ref)] = t > 0 and ks[-1] == 3 and (u, a, b) == (3, T, 1)
                    if first and t and a == 0:
                        ref[_ds(row(c, -PAD), PAD), :] = jnp.broadcast_to(v[0:1], (PAD, T))
                tasks += unit(lhs, op['w' + 'qkv'[t]], u, emit, ks)
        return tasks

    def history(src, dst, *which):
        def run():
            for t in which:
                for c in range(t % 2 * 8, t % 2 * 8 + 8):
                    dst[t // 2][_ds(row(c, -PAD), PAD), :] = src[t // 2][_ds(row(c, TM - PAD), PAD), :]
        return [(0, run)]

    scale = DH ** -0.5

    def slot(stage, w, r):
        return stage_v[2 * stage + r // Q % 2], (w * 2 + r // T) * Q + r % Q

    def grab(where, r, ws=range(W)):
        pace(where(0, r)[0])
        return [ref[_ds(o, 8), :] for ref, o in (where(w, r) for w in ws)]

    def drop(where, r, vals, first=0):
        for w, t in enumerate(vals, first):
            ref, o = where(w, r)
            ref[_ds(o, 8), :] = t

    def by_group(f, n=8):
        return [[f(a + r, range(k, k + n)) for a in (0, T) for r in range(g, g + Q, 8) for k in range(0, 8, n)]
                for g in (0, Q)]

    raw, prob, mixed = (functools.partial(slot, s) for s in range(3))

    def logits(bufs, dst, first=False):
        qk = bufs[0]

        def scores(r, ws):
            def run():
                assert ready[id(qk)]
                pace(qk)
                q = [qk[_ds(row(c, r), 8), :] for c in range(8)]
                drop(raw, r, (_sum([lax.mul(q[c], qk[_ds(row(8 + c, r - DIL * w), 8), :]) for c in range(8)])
                              for w in ws), ws[0])
            return (3.75, run)

        def fold(r, ws):
            def run():
                ps = grab(raw, r, ws)
                for bit in (16, 1):
                    low = (lax.broadcasted_iota(I32, (8, T), 1) & bit) == 0
                    ps = [p + jnp.where(low, pltpu.roll(p, T - bit, 1), pltpu.roll(p, bit, 1)) for p in ps]
                if first and r < DIL * W:
                    pos = lax.broadcasted_iota(I32, (8, T), 0) + r
                    ps = [jnp.where(pos >= DIL * w, p, -1e9 / scale) for w, p in zip(ws, ps)]
                drop(lambda w, r: (dst, w * TM + r), r, ps, ws[0])
            return (11.849 / 2, run)
        return _stagger([by_group(scores, 2), by_group(fold, 4)])

    def attend(bufs, src):
        v = bufs[1]

        def softmax(r, _):
            def run():
                lg = grab(lambda w, r: (src, w * TM + r), r)
                m = functools.reduce(jnp.maximum, lg)
                e = [jnp.exp2((p - m) * (scale * math.log2(math.e))) for p in lg]
                inv = 1.0 / _sum(e)
                drop(prob, r, [t * inv for t in e])
            return (7, run)

        def mix(r, cs):
            def run():
                assert ready[id(v)]
                pace(v)
                p = grab(prob, r)
                drop(mixed, r, (_sum([lax.mul(p[w], v[_ds(row(c, r - DIL * w), 8), :]) for w in range(W)])
                                for c in cs), cs[0])
            return (3.75, run)

        def combo(r, c):
            def run():
                pace(mixed(0, r)[0])
                assert not busy[0]
                op['oa'].put(r, c, _seven(_LHS, [ref[_ds(o, 16), :] for ref, o in (
                    mixed(b + c, a + r) for a in (0, T) for b in (0, 4))]))
            return (2, run)
        return _stagger([by_group(softmax), by_group(mix, 2),
                         [[combo(g + r, c) for r in range(0, Q, 16) for c in range(4)] for g in (0, Q)]])

    def proj(i):
        tasks, x, h = [], x_blk(i), h_blk(i)
        for u in range(4):
            def emit(a, b, v, u=u):
                c = b + 2 * u
                busy[0] = (u, a, b) != (3, T, 1)
                h[_ds(c * S + a, T), :] = x[_ds(a, T), _tile(c)].astype(F32) + v
            tasks += unit(op['oa'], op['wo'], u, emit)
        return tasks

    def z1_blk(i):
        return z1_v.at[_ds(i * T, 3 * S + T)]

    def z1_at(c, r, n):
        return _ds((c // 2 * S + r) // 2, n // 2), _tile(c % 2)

    def up(i, lhs, gz):
        tasks, z1 = [], z1_blk(i)
        for u in range(7):
            def emit(a, b, v, u=u):
                c = 7 * (b // 2) + u
                ready[id(gz)] = (u, a, b) == (6, 3 * Q, 3)
                if b % 2 == 0:
                    z1[z1_at(c, a, Q)] = pltpu.bitcast(v.astype(BF16), I32)
                else:
                    gz[_ds(c * TM + a, Q), :] = _gelu2(v)
            tasks += unit(lhs, op['win'], u, emit)
        return tasks

    def gate_head():
        def park(c):
            def emit(a, b, v):
                qk1[_ds(c(b) * TM + a, v.shape[0]), :] = v
            return emit
        tasks = unit(op['sa1'], op['z21'], 0, park(lambda b: 12 + b), range(2 * HEAD))
        for u in range(3):
            tasks += unit(op['sa2'], op['z22'], u, park(lambda b, u=u: 3 * b + u), range(HEAD))
        return tasks

    def gate_step(i, _, rest=False):
        last[0] = None
        z1, h, out, bias = z1_blk(i), h_blk(i), x_blk(i), bias_v.at[_ds(i * TM, TM)]
        extra = [(wd_prep2(3), 0.0, 0.244)] if rest else []

        def gated(c, r, v):
            n = v.shape[0]
            if rest:
                v = v + qk1[_ds(c * TM + r, n), :]
            return _gelu2(pltpu.bitcast(z1[z1_at(c, r, n)], BF16).astype(F32)) * (v + bias[_ds(r, n), :])

        y = {}

        def gate1(a, b, v):
            y[a, b] = gated(12 + b, a, v)
            if len(y) == 4:
                op['ya1'].put(0, 0, _seven(_LHS, [y[0, 0], y[0, 1], y[T, 0], y[T, 1]]))
        main, marks, sides = unit(op['sa1'], op['z21'], 0, gate1, range(2 * HEAD * rest, 8)), [], []
        for u in range(3):
            ref = (v0, v1)[u % 2]

            def gate2(a, b, v, u=u, ref=ref):
                ref[_ds(4 * a + b * Q, Q), :] = gated(3 * b + u, a, v)
            marks.append(_cost(main))
            main += unit(op['sa2'], op['z22'], u, gate2, range(HEAD * rest, 4))
            side = [expand2(_LHS, ref, lambda a, b, r=r, ref=ref: ref[_ds((4 * a + b) * Q + r, 16), :],
                            op['ya2'], r, u) for r in range(0, Q, 16)]
            sides.append([t for ts in zip(*side) for t in ts])
        marks.append(_cost(main))
        for u in range(4):
            def down1(a, b, v, u=u):
                at = _ds((4 * b + u) * S + a, T)
                h[at, :] = h[at, :] + v
            main += unit(op['ya1'], op['wd1'], u, down1)
        marks.append(_cost(main))
        for u in range(2):
            def down2(a, b, v, u=u):
                c = 4 * u + b
                out[_ds(a, Q), _tile(c)] = (h[_ds(c * S + a, Q), :] + v).astype(BF16)
                if a % T == Q and b % 2 == 1:
                    at = _ds(i * TM + a - Q, T, 16), slice((c - 1) * T, (c + 1) * T)
                    pltpu.make_async_copy(x_v.at[at], out_hbm.at[at], osem).start()
            main += unit(op['ya2'], op['wd2'], u, down2)
        t = [(m + 1) / _cost(main) for m in marks]
        span = (0.988, 0.99, 1.9) if rest else (0.99, 0.377, 1.905)
        nxt = i + 1 if rest else jnp.minimum(i + 1, NB - 1)
        overlap(main, *[(s, t[u + 1], t[u + 1] + span[u] * (t[u + 2] - t[u + 1])) for u, s in enumerate(sides)],
                 (sp_prep1(nxt), t[0], 0.823 if rest else 0.66),
                (sp_prep2(nxt), t[4] + (-0.079 if rest else -0.046), 0.985, due(ops_v, 0.99)), *extra)
        last[0] = None

    cur, alt = (qk0, v0), (qk1, v1)

    def attn_step(i, _):
        last[0] = None
        if isinstance(i, int):
            stats, sums = ln_h(0, ha)
            extra = [(stats, 0.29, 0.51), (sums, 0.51, 0.879, due(mlp_v, 0.99)),
                     (win_prep(3, 64), 0.0, 0.962, due(mlp_v, 0.25, 0.45, 0.65, 0.85))]
        else:
            stats, sums = ln_x(i + 1, xa)
            extra = [(stats, 0.299, 0.718), (sums, 0.751, 0.98, due(ops_v, 0.99)),
                     (win_prep(i - 3, 48), 0.001, 0.885, due(mlp_v, 0.25, 0.45, 0.619, 0.85))]
        overlap(history(cur, cur, 1) + qkv(xa, cur, (0, 1)) + history(cur, cur, 2) + qkv(xa, cur, (2,)) + proj(i - 1),
                 (attend(cur, p_v), 0.0, 0.492), (logits(cur, p_v), 0.501, 0.848), *extra)
        last[0] = None

    def up_step(j, _):
        last[0] = None
        i, sides = 2 * j + 1, []
        for t, z, h in ((0.0, ln_z(i - 1, gz_v), ln_h(i + 1, ha)), (0.501, ln_z(i, qk1), ln_h(i + 2, hb))):
            sides += [(z[0], t, t + 0.13), (z[1], t + 0.13, t + 0.331, due(z2_v, t + 0.331 + 0.022)),
                      (h[0], t + 0.25, t + 0.347), (h[1], t + 0.347, t + 0.47)]
        wd = wd_prep2(j)
        overlap(up(i, hb, qk1) + up(i + 1, ha, gz_v), *sides, ([], 0, 0, due(mlp_v, 0.99)),
                 *[(wd[k * len(wd) // 2:(k + 1) * len(wd) // 2], t + 0.011, t + 0.135, due(ops_v, t + 0.135 + 0.01))
                   for k, t in enumerate((0.0, 0.5))])
        last[0] = None

    copies = {}

    def start(key, src, dst):
        copies[key] = pltpu.make_async_copy(src, dst, sems.at[len(copies)])
        copies[key].start()

    def wait(*keys):
        for k in keys:
            copies[k].wait()

    def start_rows(t, k):
        for r in (k * T, D // 2 + k * T):
            start((t, r), wqkv_hbm.at[r:r + T, t * D:(t + 1) * D],
                  raw_a.at[t // 2 * D + r:t // 2 * D + r + T, t % 2 * D:(t % 2 + 1) * D])

    def start_x(lo, hi):
        start(('x', lo), x_hbm.at[lo * TM:hi * TM], x_v.at[lo * TM:hi * TM])

    def start_wo(k):
        start(('wo', k), wo_hbm.at[:, k * D // 2:(k + 1) * D // 2],
              raw_a.at[D:2 * D, D + k * D // 2:D + (k + 1) * D // 2])

    queue = [lambda: start_rows(0, 0), lambda: start_x(0, 1), lambda: start_x(1, 2),
             *[functools.partial(start_rows, t, k) for t in range(3) for k in range(4)][1:],
             lambda: start_wo(0), lambda: start_x(2, 3), lambda: start_wo(1), lambda: start_x(3, 4),
             lambda: start('win', win_hbm, raw_b.at[0:D]), lambda: start_x(4, NB), lambda: start('b', b_hbm, b_v)]

    def more(n):
        for _ in range(min(n, len(queue))):
            queue.pop(0)()

    def arrive(*chunks, ahead=0):
        wait(*[(t, a + k * T) for t, k in chunks for a in (0, D // 2)])
        more(len(chunks) + ahead)
        return _stagger([sum(st, []) for st in zip(*[qkv_prep(t, k) for t, k in chunks])])

    more(5)
    _run(arrive((0, 0)))
    wait(('x', 0))
    more(1)
    _run(sum(ln_x(0, xa), []))
    wait(('x', 1))
    more(1)
    overlap(qkv(xa, cur, (0,), [0]), (sum(ln_x(1, xb), []), 0.0, 0.86))
    overlap(qkv(xb, alt, (0,), [0]), (arrive((0, 1)), 0.0, 0.8))
    for t, ks, chunks, ahead, hi in (
            (0, [1], [(0, 2)], 0, 0.85), (0, [2], [(0, 3)], 0, 0.85), (0, [3], [(1, 0), (1, 1)], 0, 0.97),
            (1, [0, 1], [(1, 2), (1, 3)], 2, 0.745), (1, [2, 3], [(2, 0), (2, 1), (2, 2)], 0, 0.963)):
        overlap(qkv(xa, cur, (t,), ks, True) + qkv(xb, alt, (t,), ks),
                 (arrive(*chunks, ahead=ahead), 0.0, hi, due(ops_v, 0.98)))
    side = arrive((2, 3), ahead=len(queue))
    wait(('wo', 0), ('x', 2))
    overlap(qkv(xa, cur, (2,), [0, 1, 2], True) + qkv(xa, cur, (2,), [3], True) + history(cur, alt, 1, 2)
             + qkv(xb, alt, (2,)),
             (side, 0.0, 0.306), (logits(cur, p_v, True), 0.0, 0.839),
             (sum(ln_x(2, xa), []), 0.501, 0.878, due(ops_v, 0.985)),
            (wo_prep(0, 1), 0.2, 0.66, due(ops_v, 0.66 + 0.05)))
    wait(('x', 3), ('wo', 1))
    stats, sums = ln_x(3, xa)
    overlap(history(alt, cur, 1) + qkv(xa, cur, (0, 1)) + proj(0) + history(alt, cur, 2) + qkv(xa, cur, (2,)) + proj(1),
             (attend(cur, p_v), 0.0, 0.395), (wo_prep(2, 3), 0.0, 0.39),
             (logits(alt, gz_v), 0.025, 0.464), (attend(alt, gz_v), 0.464, 0.79), (logits(cur, p_v), 0.55, 0.905),
             (stats, 0.4, 0.8), (sums, 0.801, 0.95, due(ops_v, 0.99)))
    wait('win', ('x', 4), 'b')
    start('wsp', wsp_hbm, raw_a.at[0:S])
    lax.fori_loop(3, NB - 1, attn_step, None)
    attn_step(NB - 1, None)
    for k in range(2):
        start(('wd', k), wout_hbm.at[k * FH // 2:(k + 1) * FH // 2], raw_b.at[0:FH // 2, k * D:(k + 1) * D])
    barrier()
    overlap(up(0, ha, gz_v) + proj(NB - 1), (attend(cur, p_v), 0.0, 0.591),
             (sum(ln_h(1, hb), []) + bias_prep(), 0.429, 0.967, due(mlp_v, 0.97)))
    wait('wsp', ('wd', 0), ('wd', 1))
    lax.fori_loop(0, NB // 2 - 1, up_step, None)
    z6, z7 = ln_z(NB - 2, gz_v), ln_z(NB - 1, qk0)
    main = up(NB - 1, hb, qk0), gate_head()
    mid = (_cost(main[0]) + 1) / _cost(main[0] + main[1])
    overlap(main[0] + main[1], (z6[0], 0.0, 0.15), (z6[1], 0.15, 0.445, due(z2_v, 0.5)),
             (wd_prep1() + sp_prep1(0), 0.0, 0.2, due(ops_v, 0.2 + 0.04)), (sp_prep2(0), 0.448, 0.696),
             (z7[0], mid, 0.783), (z7[1], 0.783, 0.97, due(z2_v, 0.99)))
    barrier()
    gate_step(0, None, True)
    lax.fori_loop(1, NB, gate_step, None)
    pltpu.make_async_copy(x_v.at[0:S], out_hbm, osem).wait()


@jax.jit
def pallas_sequential_preLN__sliding_local_dilated__mixer_gmlp__prompt_kernel(
        A_x, A_wqkv, A_wo, B_x, B_w_in, B_w_sp, B_b_sp, B_w_out):
    del B_x
    hbm, vm = pl.BlockSpec(memory_space=pl.ANY), pltpu.VMEM
    out = pl.pallas_call(
        _kernel,
        out_shape=jax.ShapeDtypeStruct((S, D), BF16),
        in_specs=[hbm] * 7,
        out_specs=hbm,
        scratch_shapes=[
            vm((S + PAD, D), BF16),
            vm((S + PAD, S), BF16),
            vm((D + PAD, 2 * FH), BF16),
            vm((_rows(_EARLY, _LATE), 2 * T), I32), vm((_rows(_MLP), 2 * T), I32), vm((_rows(_Z2), 2 * T), I32),
            vm((W * TM + PAD, T), F32),
            *[vm((n * (TM + PAD) + PAD, T), F32) for n in (16, 8, 16, 8)],
            vm((8 * S + PAD, T), F32), vm((14 * TM + PAD, T), F32), vm((7 * S // 2, 2 * T), I32),
            vm((6 * TM, T), F32), vm((S, T), F32), vm((S // T, T), BF16),
            pltpu.SemaphoreType.DMA((36,)), pltpu.SemaphoreType.DMA(()), pltpu.SemaphoreType.REGULAR(()),
            *[vm((16 * Q + 8, T), F32)] * 6, *[vm((16 * 16 + 8, T), F32)] * 2, *[vm((8 * G + 8, T), F32)] * 4,
        ],
        compiler_params=pltpu.CompilerParams(vmem_limit_bytes=126 * 1024 * 1024),
    )(A_x.reshape(S, D), A_wqkv, A_wo, B_w_in, B_w_sp, B_b_sp.reshape(S // T, T), B_w_out)
    return out.reshape(1, S, D)
```

```python
import functools
import math

import numpy as np
import jax
import jax.numpy as jnp
from jax import lax
import jax.experimental.pallas as pl
import jax.experimental.pallas.tpu as pltpu

S, D, FH = 2048, 1024, 1792
DH, W, DIL = 32, 8, 2
EPS = 1e-5
F32, BF16, I32 = jnp.float32, jnp.bfloat16, jnp.int32
T = 128
Q = 64
TM = 2 * T
NB = S // TM
PAD = 16
G = 32
HEAD = 2


def _gelu2(h):
    c = math.sqrt(2.0 / math.pi)
    return h + h * jnp.tanh(h * (2 * c + (8 * c * 0.044715) * (h * h)))


def _skew(parts, axis, unit):
    return [c if i == 0 else pltpu.roll(c, unit * i, axis) for i, c in enumerate(parts)]


def _unskew(parts, axis, unit):
    n = parts[0].shape[axis]
    idx = lax.broadcasted_iota(I32, parts[0].shape, axis)
    x = [parts[-j % 8] for j in range(8)]
    for b in (1, 2, 4):
        on = (idx & (b * unit)) != 0
        x = [jnp.where(on, x[(j - b) % 8], x[j]) for j in range(8)]
    return [t if j == 0 else pltpu.roll(t, n - unit * j, axis) for j, t in enumerate(x)]


_LHS = (((1, 0, 0), (1, 1, 1)), ((1, 1, 0), (1, 1, 1)), ((1, 0, 0),), ((1, 1, 1),),
        ((1, 0, 0), (1, 0, 1)), ((1, 1, 0), (-1, 0, 0)), ((1, 0, 1), (-1, 1, 1)))
_RHS = (((1, 0, 0), (1, 1, 1)), ((1, 0, 0),), ((1, 0, 1), (-1, 1, 1)), ((1, 1, 0), (-1, 0, 0)),
        ((1, 1, 1),), ((1, 0, 0), (1, 0, 1)), ((1, 1, 0), (1, 1, 1)))
_ORDER = (6, 3, 1, 0, 4, 2, 5)


def _combine(terms, get):
    v = get(*terms[0][1:])
    for sign, a, b in terms[1:]:
        v = (lax.add if sign > 0 else lax.sub)(v, get(a, b))
    return v


def _seven(table, quad):
    return [_combine(terms, lambda a, b: quad[2 * a + b]) for terms in table]


def _sum(xs):
    return functools.reduce(lax.add, xs)


def _cost(tasks):
    return sum(c for c, _ in tasks)


def _merge(main, *sides):
    span, t, ev = _cost(main), 0.0, []
    for c, f in main:
        ev.append((t / span, 1, c / span, f))
        t += c
    for side, lo, hi, *timed in sides:
        ev += [(when, 0, 0.0, f) for events in timed for when, f in events]
        total, t = _cost(side), 0.0
        for c, f in side:
            ev.append((lo + (hi - lo) * t / total, 0, 0.0, f))
            t += c
    t0, span = 0.0, 1.0
    for when, _, c, f in sorted(ev, key=lambda e: e[:2]):
        if c:
            t0, span = when, c
        yield min(0.999, (when - t0) / span), f


def _stagger(stages):
    n, out = len(stages[0]), []
    for k in range(n + len(stages) - 1):
        now = [st[k - s] for s, st in enumerate(stages) if 0 <= k - s < n]
        now = [((j + 0.5) / len(g), s, t) for s, g in enumerate(now) for j, t in enumerate(g)]
        out += [t for _, _, t in sorted(now, key=lambda e: e[:2])]
    return out


def _run(tasks):
    for _, f in tasks:
        f()


def _tile(c):
    return slice(c * T, (c + 1) * T)


def _ds(start, n, align=8):
    if isinstance(start, int):
        return pl.ds(lax.add(np.int32(start), np.int32(0)), n)
    return pl.ds(pl.multiple_of(start, align), n)


class _Operand:
    def __init__(self, ref, base, levels, rows, nt):
        self.ref, self.base, self.levels, self.rows, self.nt = ref, base, levels, rows, nt

    @staticmethod
    def size(levels, rows, nt):
        return (7 ** levels * nt + 1) // 2 * rows // 2

    def shifted(self, i, step, most=None):
        size = self.size(self.levels, self.rows, self.nt) - (most or self.rows - step) // 2
        return _Operand(self.ref.at[_ds(self.base + i * (step // 2), size)], 0, self.levels, self.rows, self.nt)

    def at(self, j, r, c, n):
        g = j * self.nt + c
        return _ds(self.base + g // 2 * self.rows // 2 + r // 2, n // 2), _tile(g % 2)

    def put(self, r, c, mats, first=0):
        for j, t in enumerate(mats):
            self.ref[self.at(first + j, r, c, t.shape[0])] = pltpu.bitcast(lax.convert_element_type(t, BF16), I32)

    def rhs(self, j, c, ks):
        return pltpu.bitcast(self.ref[self.at(j, ks[0] * T, c, len(ks) * T)], BF16)

    def lhs(self, j, ks, zeros):
        cols = [self.ref[self.at(j, 0, c, self.rows)] for c in ks]
        for z in zeros:
            cols[-1] = jnp.concatenate([cols[-1][:-8], cols[-1][-8:] | z], 0)
        return jnp.concatenate([pltpu.bitcast(c, BF16) for c in cols], 1)


_EARLY = dict(wq=(1, D // 2, 4), wk=(1, D // 2, 4), wv=(1, D // 2, 4), wo=(1, D // 2, 4),
              xa=(1, T, 4), xb=(1, T, 4), oa=(1, T, 4))
_LATE = dict(wd2=(2, 3 * T, 2), wd1=(1, T, 4), sa2=(2, Q, 4), sa1=(1, T, 8))
_MLP = dict(win=(2, D // 4, 7), ha=(2, Q, 2), ya2=(2, Q, 3), ya1=(1, T, 1))
_Z2 = dict(z22=(2, S // 4, 3), z21=(1, S // 2, 1))


def _rows(*tables):
    return max(sum(_Operand.size(*s) for s in t.values()) for t in tables) + 8


def _kernel(x_hbm, wqkv_hbm, wo_hbm, win_hbm, wsp_hbm, b_hbm, wout_hbm, out_hbm,
            x_v, raw_a, raw_b, ops_v, mlp_v, z2_v, p_v, qk0, v0, qk1, v1, h_v, gz_v, z1_v, stat_v,
            bias_v, b_v, sems, osem, bar, *small):
    stage_v, tmp_v, perm_v = small[:6], small[6:8], small[8:]
    op = {}
    for ref, table in ((ops_v, _EARLY), (ops_v, _LATE), (mlp_v, _MLP), (z2_v, _Z2)):
        top = 0
        for name, shape in table.items():
            op[name] = _Operand(ref, top, *shape)
            top += _Operand.size(*shape)
    xa, xb, ha = op['xa'], op['xb'], op['ha']
    hb = _Operand(mlp_v, op['ya2'].base, *_MLP['ha'])
    xc = _Operand(z2_v, 0, *_EARLY['xa'])

    zero = lax.fori_loop(0, 2, lambda _, c: c ^ 1, 0)
    last, phase, paced, pending = [None], [0.0], {}, []
    ready, busy = {}, [False]

    def overlap(main, *sides):
        for phase[0], f in _merge(main, *sides):
            f()

    def pace(ref):
        if last[0] is None:
            return
        r = int(phase[0] * (last[0].shape[0] // 32)) * 32
        old = paced.get(id(ref), (None, 0))
        if old[0] is not last[0] or old[1] != r:
            paced[id(ref)] = last[0], r
            n = 8 if ref.dtype == F32 else 16
            ref[_ds(zero * n + (ref.shape[0] - n), n, n), 0:T] = last[0][r:r + n].astype(ref.dtype)

    for ref in (ops_v, mlp_v, z2_v):
        ref[_ds(ref.shape[0] - 8, 8), 0:T] = jnp.zeros((8, T), I32)

    def due(ref, *times):
        def run():
            pending.append(ref[_ds(zero * 8 + (ref.shape[0] - 8), 8), 0:T])
        return [(when, run) for when in times]

    def barrier():
        pl.semaphore_signal(bar, 1)
        pl.semaphore_wait(bar, 1)

    def products(lhs, rhs, u, emit, ks, level, first):
        if level == 0:
            def run():
                last[0] = jnp.dot(lhs.lhs(first, ks, pending), rhs.rhs(first, u, ks), preferred_element_type=F32)
                pending.clear()
                emit(0, 0, last[0])
            return [(len(ks) * lhs.rows / 4, run)]
        h = 2 ** (level - 1)
        state = {(i, j): [None, None] for i in range(h) for j in range(h)}

        def step(n):
            def take(i, j, m):
                s = state[i, j]
                if n == 0:
                    s[0] = m
                elif n == 1:
                    s[:] = s[0] + m, m
                elif n == 2:
                    emit(h + i, j, m + s[1])
                    s[1] = m
                elif n == 3:
                    s[:] = s[0] + m, m - s[1]
                elif n == 4:
                    emit(i, j, s[0] - m)
                    s[0] = m
                elif n == 5:
                    emit(i, h + j, m + s[0])
                    s[1] = s[1] + m
                else:
                    emit(h + i, h + j, s[1] + m)
            return take
        return [t for n, r in enumerate(_ORDER) for t in products(lhs, rhs, u, step(n), ks, level - 1, first * 7 + r)]

    def unit(lhs, rhs, u, emit, ks=None):
        return products(lhs, rhs, u, lambda a, b, v: emit(a * lhs.rows, b, v), ks or range(lhs.nt), lhs.levels, 0)

    def expand2(table, ref, get, dst, r, c):
        def task(r1):
            def run():
                pace(ref)
                quad = [_combine(table[r1], lambda a, b: get(2 * a + i, 2 * b + j)) for i in (0, 1) for j in (0, 1)]
                dst.put(r, c, _seven(table, quad), 7 * r1)
            return (3, run)
        return [task(r1) for r1 in _ORDER]

    def layer_norm(src, load, nt, stat, gain=1.0):
        def mean(r):
            def run():
                assert ready.get(id(src), True)
                pace(src)
                m = jnp.sum(_sum([load(r, c) for c in range(nt)]), axis=-1, keepdims=True) * (1.0 / (nt * T))
                stat_v[_ds(stat + r, 16), :] = jnp.broadcast_to(m, (16, T))
            return (nt / 2, run)

        def rstd(r):
            def run():
                pace(src)
                m = stat_v[_ds(stat + r, 16), :]
                v = [load(r, c) - m for c in range(nt)]
                var = jnp.sum(_sum([t * t for t in v]), axis=-1, keepdims=True) * (1.0 / (nt * T))
                inv = lax.rsqrt(var + EPS)
                stat_v[_ds(stat + TM + r, 16), :] = jnp.broadcast_to(inv if gain == 1.0 else gain * inv, (16, T))
            return (3 * nt / 4, run)

        def norm(r, c):
            m, inv = stat_v[_ds(stat + r, 16), :], stat_v[_ds(stat + TM + r, 16), :]
            return (load(r, c) - m) * inv
        return [f(r) for f in (mean, rstd) for r in range(0, TM, 16)], norm

    def raw_tile(ref, r, c):
        return ref[_ds(r, 16, 16), _tile(c)]

    def x_blk(i):
        return x_v.at[_ds(i * TM, TM, 16)]

    def h_blk(i):
        return h_v.at[_ds(i * TM, 7 * S + TM)]

    def ln_x(i, dst):
        x = x_blk(i)
        stats, norm = layer_norm(x_v, lambda r, c: raw_tile(x, r, c).astype(F32), 8, 0)

        def task(r, c):
            def run():
                pace(x_v)
                dst.put(r, c, _seven(_LHS, [norm(a + r, b + c) for a in (0, T) for b in (0, 4)]))
            return (5, run)
        return stats, [task(r, c) for r in range(0, T, 16) for c in range(4)]

    def ln_h(i, dst):
        h = h_blk(i)
        stats, norm = layer_norm(h_v, lambda r, c: h[_ds(c * S + r, 16), :], 8, 2 * TM, 0.5)
        return stats, [t for c in range(2) for r in range(0, Q, 16) for t in expand2(
            _LHS, h_v, lambda a, b, r=r, c=c: norm(a * Q + r, 2 * b + c), dst, r, c)]

    def ln_z(i, gz):
        stats, norm = layer_norm(gz, lambda r, c: gz[_ds(c * TM + r, 16), :], 14, 4 * TM)
        z21, z22 = op['z21'].shifted(i, T), op['z22'].shifted(i, Q)

        def task(r):
            def run():
                pace(gz)
                z21.put(r, 0, _seven(_RHS, [norm(a + r, c) for a in (0, T) for c in (12, 13)]))
            return (4, run)
        return stats, [task(r) for r in range(0, T, 16)] + [
            t for c in range(3) for r in range(0, Q, 16) for t in expand2(
                _RHS, gz, lambda a, b, r=r, c=c: norm(a * Q + r, 3 * b + c), z22, r, c)]

    def win_prep(i, n):
        src, dst = raw_b.at[_ds(i * n, 3 * D // 4 + n, 16)], op['win'].shifted(i, n)
        return [t for r in range(0, n, 16) for u in range(7) for t in expand2(
            _RHS, raw_b, lambda a, b, r=r, u=u: raw_tile(
                src, a * (D // 4) + r, 14 * (b % 2) + 7 * (b // 2) + u).astype(F32), dst, r, u)]

    def wd_tile(src, k, r, c):
        return raw_tile(src, k % 7 * T + r, k // 7 * 8 + c).astype(F32)

    def wd_prep1():
        def task(r, c):
            def run():
                pace(raw_b)
                op['wd1'].put(r, c, _seven(_RHS, [wd_tile(raw_b, k, r, b + c) for k in (12, 13) for b in (0, 4)]))
            return (3.5, run)
        return [task(r, c) for c in range(4) for r in range(0, T, 16)]

    def wd_prep2(i):
        src, dst = raw_b.at[_ds(i * 32, 6 * T + 32, 16)], op['wd2'].shifted(i, 32, 96)
        return [t for r in (0, 16) for k in range(3) for u in range(2) for t in expand2(
            _RHS, raw_b, lambda a, b, r=r, k=k, u=u: wd_tile(src, 3 * a + k, r, 4 * u + b), dst, k * T + r, u)]

    def sp_prep1(i):
        src = raw_a.at[_ds(i * TM, TM, 16)]

        def task(r, b):
            def run():
                pace(raw_a)
                op['sa1'].put(r, b, _seven(_LHS, [raw_tile(src, a + r, 2 * b + c).astype(F32)
                                                  for a in (0, T) for c in (0, 1)]))
            return (3.5, run)
        return [task(r, b) for b in range(NB) for r in range(0, T, 16)]

    def sp_prep2(i):
        src = raw_a.at[_ds(i * TM, TM, 16)]

        def gather(ref, r, c, a):
            def run():
                pace(raw_a)
                low, out = lax.broadcasted_iota(I32, (8, T), 1) < Q, []
                for half in (0, 1):
                    u, v = (pltpu.bitcast(raw_tile(src, a * Q + r, 4 * c + 2 * k + half), I32) for k in (0, 1))
                    out += [jnp.where(low, u, pltpu.roll(v, Q, 1)), jnp.where(low, pltpu.roll(u, Q, 1), v)]
                for b, t in enumerate([pltpu.bitcast(t, BF16).astype(F32) for t in out]):
                    ref[_ds((4 * a + b) * 16, 16), :] = t
            return (2, run)
        jobs = [(tmp_v[r // 16 % 2], r, c) for c in range(4) for r in range(0, Q, 16)]
        return _stagger([[[gather(*job, a) for a in range(4)] for job in jobs],
                         [expand2(_LHS, ref, lambda a, b, ref=ref: ref[_ds((4 * a + b) * 16, 16), :], op['sa2'], r, c)
                          for ref, r, c in jobs]])

    def qkv_prep(t, k):
        def where(stage, r):
            return perm_v[2 * stage + r // G % 2], (r // (D // 2) * G + r % G) * 4

        def drop(stage, r, vals):
            ref, o = where(stage, r)
            for c, v in enumerate(vals):
                ref[_ds(o + 8 * c, 8), :] = pltpu.bitcast(v, F32)

        def grab(stage, r, cs):
            ref, o = where(stage, r)
            pace(ref)
            return [pltpu.bitcast(ref[_ds(o + 8 * c, 8), :], I32) for c in cs]

        def skew(r):
            def run():
                pace(raw_a)
                drop(0, r, _skew([pltpu.bitcast(raw_tile(raw_a, t // 2 * D + r, t % 2 * 8 + c), I32)
                                  for c in range(8)], 1, 2))
            return (3, run)

        def unskew(r):
            return (4, lambda: drop(1, r, _unskew(grab(0, r, range(8)), 1, 2)))

        def store(r, c):
            def run():
                op['w' + 'qkv'[t]].put(r, c, _seven(_RHS, [
                    pltpu.bitcast(p, BF16).astype(F32) for a in (0, D // 2) for p in grab(1, a + r, (c, 4 + c))]))
            return (3, run)
        gs = range(k * T, (k + 1) * T, G)
        return [[[f(a + r) for r in range(g, g + G, 16) for a in (0, D // 2)] for g in gs]
                for f in (skew, unskew)] + [[[store(r, c) for r in range(g, g + G, 16) for c in range(4)] for g in gs]]

    def wo_prep(*cs):
        def swap(g, c, ref, b):
            def run():
                pace(raw_a)
                parts = [pltpu.bitcast(raw_tile(raw_a, D + i * T + g, 8 + b + 2 * c), I32) for i in range(8)]
                for j, p in enumerate(_unskew(_skew(parts, 0, 1), 0, 1)):
                    ref[_ds((b * 8 + j) * 8, 8), :] = pltpu.bitcast(p, F32)
            return (5, run)

        def store(g, c, ref, j):
            def run():
                pace(ref)
                op['wo'].put(j * T + g, c, _seven(_RHS, [
                    pltpu.bitcast(pltpu.bitcast(ref[_ds((b * 8 + a + j) * 8, 8), :], I32), BF16).astype(F32)
                    for a in (0, 4) for b in (0, 1)]))
            return (3, run)
        jobs = [(g, c, tmp_v[g // 16 % 2]) for c in cs for g in range(0, T, 16)]
        return _stagger([[[swap(*job, b) for b in (0, 1)] for job in jobs],
                         [[store(*job, j) for j in range(4)] for job in jobs]])

    def bias_prep():
        def task(k):
            def run():
                bias_v[_ds(k * T, T), :] = jnp.broadcast_to(b_v[...].astype(F32)[k:k + 1, :], (T, T)).T
            return (4, run)
        return [task(k) for k in range(S // T)]

    def row(c, r):
        return c * (TM + PAD) + PAD + r

    def qkv(lhs, bufs, which, ks=range(4), first=False):
        tasks = []
        for t in which:
            for u in range(4):
                def emit(a, b, v, t=t, u=u):
                    ref, c = bufs[t // 2], t % 2 * 8 + 4 * b + u
                    if ks[0]:
                        v = v + ref[_ds(row(c, a), T), :]
                    ref[_ds(row(c, a), T), :] = v
                    ready[id(ref)] = t > 0 and ks[-1] == 3 and (u, a, b) == (3, T, 1)
                    if first and t and a == 0:
                        ref[_ds(row(c, -PAD), PAD), :] = jnp.broadcast_to(v[0:1], (PAD, T))
                tasks += unit(lhs, op['w' + 'qkv'[t]], u, emit, ks)
        return tasks

    def history(src, dst, *which):
        def run():
            for t in which:
                for c in range(t % 2 * 8, t % 2 * 8 + 8):
                    dst[t // 2][_ds(row(c, -PAD), PAD), :] = src[t // 2][_ds(row(c, TM - PAD), PAD), :]
        return [(0, run)]

    scale = DH ** -0.5

    def slot(stage, w, r):
        return stage_v[2 * stage + r // Q % 2], (w * 2 + r // T) * Q + r % Q

    def grab(where, r, ws=range(W)):
        pace(where(0, r)[0])
        return [ref[_ds(o, 8), :] for ref, o in (where(w, r) for w in ws)]

    def drop(where, r, vals, first=0):
        for w, t in enumerate(vals, first):
            ref, o = where(w, r)
            ref[_ds(o, 8), :] = t

    def by_group(f, n=8):
        return [[f(a + r, range(k, k + n)) for a in (0, T) for r in range(g, g + Q, 8) for k in range(0, 8, n)]
                for g in (0, Q)]

    raw, prob, mixed = (functools.partial(slot, s) for s in range(3))

    def logits(bufs, dst, first=False):
        qk = bufs[0]

        def scores(r, ws):
            def run():
                assert ready[id(qk)]
                pace(qk)
                q = [qk[_ds(row(c, r), 8), :] for c in range(8)]
                drop(raw, r, (_sum([lax.mul(q[c], qk[_ds(row(8 + c, r - DIL * w), 8), :]) for c in range(8)])
                              for w in ws), ws[0])
            return (3.75, run)

        def fold(r, ws):
            def run():
                ps = grab(raw, r, ws)
                for bit in (16, 1):
                    low = (lax.broadcasted_iota(I32, (8, T), 1) & bit) == 0
                    ps = [p + jnp.where(low, pltpu.roll(p, T - bit, 1), pltpu.roll(p, bit, 1)) for p in ps]
                if first and r < DIL * W:
                    pos = lax.broadcasted_iota(I32, (8, T), 0) + r
                    ps = [jnp.where(pos >= DIL * w, p, -1e9 / scale) for w, p in zip(ws, ps)]
                drop(lambda w, r: (dst, w * TM + r), r, ps, ws[0])
            return (11.849 / 2, run)
        return _stagger([by_group(scores, 2), by_group(fold, 4)])

    def attend(bufs, src):
        v = bufs[1]

        def softmax(r, _):
            def run():
                lg = grab(lambda w, r: (src, w * TM + r), r)
                m = functools.reduce(jnp.maximum, lg)
                e = [jnp.exp2((p - m) * (scale * math.log2(math.e))) for p in lg]
                inv = 1.0 / _sum(e)
                drop(prob, r, [t * inv for t in e])
            return (7, run)

        def mix(r, cs):
            def run():
                assert ready[id(v)]
                pace(v)
                p = grab(prob, r)
                drop(mixed, r, (_sum([lax.mul(p[w], v[_ds(row(c, r - DIL * w), 8), :]) for w in range(W)])
                                for c in cs), cs[0])
            return (3.75, run)

        def combo(r, c):
            def run():
                pace(mixed(0, r)[0])
                assert not busy[0]
                op['oa'].put(r, c, _seven(_LHS, [ref[_ds(o, 16), :] for ref, o in (
                    mixed(b + c, a + r) for a in (0, T) for b in (0, 4))]))
            return (2, run)
        return _stagger([by_group(softmax), by_group(mix, 2),
                         [[combo(g + r, c) for r in range(0, Q, 16) for c in range(4)] for g in (0, Q)]])

    def proj(i):
        tasks, x, h = [], x_blk(i), h_blk(i)
        for u in range(4):
            def emit(a, b, v, u=u):
                c = b + 2 * u
                busy[0] = (u, a, b) != (3, T, 1)
                h[_ds(c * S + a, T), :] = x[_ds(a, T), _tile(c)].astype(F32) + v
            tasks += unit(op['oa'], op['wo'], u, emit)
        return tasks

    def z1_blk(i):
        return z1_v.at[_ds(i * T, 3 * S + T)]

    def z1_at(c, r, n):
        return _ds((c // 2 * S + r) // 2, n // 2), _tile(c % 2)

    def up(i, lhs, gz):
        tasks, z1 = [], z1_blk(i)
        for u in range(7):
            def emit(a, b, v, u=u):
                c = 7 * (b // 2) + u
                ready[id(gz)] = (u, a, b) == (6, 3 * Q, 3)
                if b % 2 == 0:
                    z1[z1_at(c, a, Q)] = pltpu.bitcast(v.astype(BF16), I32)
                else:
                    gz[_ds(c * TM + a, Q), :] = _gelu2(v)
            tasks += unit(lhs, op['win'], u, emit)
        return tasks

    def gate_head():
        def park(c):
            def emit(a, b, v):
                qk1[_ds(c(b) * TM + a, v.shape[0]), :] = v
            return emit
        tasks = unit(op['sa1'], op['z21'], 0, park(lambda b: 12 + b), range(2 * HEAD))
        for u in range(3):
            tasks += unit(op['sa2'], op['z22'], u, park(lambda b, u=u: 3 * b + u), range(HEAD))
        return tasks

    def gate_step(i, _, rest=False):
        last[0] = None
        z1, h, out, bias = z1_blk(i), h_blk(i), x_blk(i), bias_v.at[_ds(i * TM, TM)]
        extra = [(wd_prep2(3), 0.0, 0.244)] if rest else []

        def gated(c, r, v):
            n = v.shape[0]
            if rest:
                v = v + qk1[_ds(c * TM + r, n), :]
            return _gelu2(pltpu.bitcast(z1[z1_at(c, r, n)], BF16).astype(F32)) * (v + bias[_ds(r, n), :])

        y = {}

        def gate1(a, b, v):
            y[a, b] = gated(12 + b, a, v)
            if len(y) == 4:
                op['ya1'].put(0, 0, _seven(_LHS, [y[0, 0], y[0, 1], y[T, 0], y[T, 1]]))
        main, marks, sides = unit(op['sa1'], op['z21'], 0, gate1, range(2 * HEAD * rest, 8)), [], []
        for u in range(3):
            ref = (v0, v1)[u % 2]

            def gate2(a, b, v, u=u, ref=ref):
                ref[_ds(4 * a + b * Q, Q), :] = gated(3 * b + u, a, v)
            marks.append(_cost(main))
            main += unit(op['sa2'], op['z22'], u, gate2, range(HEAD * rest, 4))
            side = [expand2(_LHS, ref, lambda a, b, r=r, ref=ref: ref[_ds((4 * a + b) * Q + r, 16), :],
                            op['ya2'], r, u) for r in range(0, Q, 16)]
            sides.append([t for ts in zip(*side) for t in ts])
        marks.append(_cost(main))
        for u in range(4):
            def down1(a, b, v, u=u):
                at = _ds((4 * b + u) * S + a, T)
                h[at, :] = h[at, :] + v
            main += unit(op['ya1'], op['wd1'], u, down1)
        marks.append(_cost(main))
        for u in range(2):
            def down2(a, b, v, u=u):
                c = 4 * u + b
                out[_ds(a, Q), _tile(c)] = (h[_ds(c * S + a, Q), :] + v).astype(BF16)
                if a % T == Q and b % 2 == 1:
                    at = _ds(i * TM + a - Q, T, 16), slice((c - 1) * T, (c + 1) * T)
                    pltpu.make_async_copy(x_v.at[at], out_hbm.at[at], osem).start()
            main += unit(op['ya2'], op['wd2'], u, down2)
        t = [(m + 1) / _cost(main) for m in marks]
        span = (0.988, 0.99, 1.9) if rest else (0.99, 0.377, 1.905)
        nxt = i + 1 if rest else jnp.minimum(i + 1, NB - 1)
        overlap(main, *[(s, t[u + 1], t[u + 1] + span[u] * (t[u + 2] - t[u + 1])) for u, s in enumerate(sides)],
                 (sp_prep1(nxt), t[0], 0.823 if rest else 0.66),
                (sp_prep2(nxt), t[4] + (-0.079 if rest else -0.046), 0.985, due(ops_v, 0.99)), *extra)
        last[0] = None

    cur, alt = (qk0, v0), (qk1, v1)

    def attn_step(i, _):
        last[0] = None
        if isinstance(i, int):
            stats, sums = ln_h(0, ha)
            extra = [(stats, 0.29, 0.51), (sums, 0.51, 0.879, due(mlp_v, 0.99)),
                     (win_prep(3, 64), 0.0, 0.962, due(mlp_v, 0.25, 0.45, 0.65, 0.85))]
        else:
            stats, sums = ln_x(i + 1, xa)
            extra = [(stats, 0.299, 0.718), (sums, 0.751, 0.98, due(ops_v, 0.99)),
                     (win_prep(i - 3, 48), 0.001, 0.885, due(mlp_v, 0.25, 0.45, 0.619, 0.85))]
        overlap(history(cur, cur, 1) + qkv(xa, cur, (0, 1)) + history(cur, cur, 2) + qkv(xa, cur, (2,)) + proj(i - 1),
                 (attend(cur, p_v), 0.0, 0.492), (logits(cur, p_v), 0.501, 0.848), *extra)
        last[0] = None

    def up_step(j, _):
        last[0] = None
        i, sides = 2 * j + 1, []
        for t, z, h in ((0.0, ln_z(i - 1, gz_v), ln_h(i + 1, ha)), (0.501, ln_z(i, qk1), ln_h(i + 2, hb))):
            sides += [(z[0], t, t + 0.13), (z[1], t + 0.13, t + 0.331, due(z2_v, t + 0.331 + 0.022)),
                      (h[0], t + 0.25, t + 0.347), (h[1], t + 0.347, t + 0.47)]
        wd = wd_prep2(j)
        overlap(up(i, hb, qk1) + up(i + 1, ha, gz_v), *sides, ([], 0, 0, due(mlp_v, 0.99)),
                 *[(wd[k * len(wd) // 2:(k + 1) * len(wd) // 2], t + 0.011, t + 0.135, due(ops_v, t + 0.135 + 0.01))
                   for k, t in enumerate((0.0, 0.5))])
        last[0] = None

    copies = {}

    def start(key, src, dst):
        copies[key] = pltpu.make_async_copy(src, dst, sems.at[len(copies)])
        copies[key].start()

    def wait(*keys):
        for k in keys:
            copies[k].wait()

    def start_rows(t, k):
        for r in (k * T, D // 2 + k * T):
            start((t, r), wqkv_hbm.at[r:r + T, t * D:(t + 1) * D],
                  raw_a.at[t // 2 * D + r:t // 2 * D + r + T, t % 2 * D:(t % 2 + 1) * D])

    def start_x(lo, hi):
        start(('x', lo), x_hbm.at[lo * TM:hi * TM], x_v.at[lo * TM:hi * TM])

    def start_wo(k):
        start(('wo', k), wo_hbm.at[:, k * D // 2:(k + 1) * D // 2],
              raw_a.at[D:2 * D, D + k * D // 2:D + (k + 1) * D // 2])

    queue = [lambda: start_rows(0, 0), lambda: start_x(0, 1), lambda: start_x(1, 2),
             *[functools.partial(start_rows, t, k) for t in range(3) for k in range(4)][1:],
             lambda: start_wo(0), lambda: start_x(2, 3), lambda: start_wo(1), lambda: start_x(3, 4),
             lambda: start('win', win_hbm, raw_b.at[0:D]), lambda: start_x(4, NB), lambda: start('b', b_hbm, b_v)]

    def more(n):
        for _ in range(min(n, len(queue))):
            queue.pop(0)()

    def arrive(*chunks, ahead=0):
        wait(*[(t, a + k * T) for t, k in chunks for a in (0, D // 2)])
        more(len(chunks) + ahead)
        return _stagger([sum(st, []) for st in zip(*[qkv_prep(t, k) for t, k in chunks])])

    more(5)
    _run(arrive((0, 0)))
    wait(('x', 0))
    more(1)
    _run(sum(ln_x(0, xa), []))
    wait(('x', 1))
    more(1)
    overlap(qkv(xa, cur, (0,), [0]), (sum(ln_x(1, xb), []), 0.0, 0.86))
    overlap(qkv(xb, alt, (0,), [0]), (arrive((0, 1)), 0.0, 0.8))
    for t, ks, chunks, ahead, hi in (
            (0, [1], [(0, 2)], 0, 0.85), (0, [2], [(0, 3)], 0, 0.85), (0, [3], [(1, 0), (1, 1)], 0, 0.97),
            (1, [0, 1], [(1, 2), (1, 3)], 2, 0.745), (1, [2, 3], [(2, 0), (2, 1), (2, 2)], 0, 0.963)):
        overlap(qkv(xa, cur, (t,), ks, True) + qkv(xb, alt, (t,), ks),
                 (arrive(*chunks, ahead=ahead), 0.0, hi, due(ops_v, 0.98)))
    side = arrive((2, 3), ahead=len(queue))
    wait(('wo', 0), ('x', 2))
    overlap(qkv(xa, cur, (2,), [0, 1, 2], True) + qkv(xa, cur, (2,), [3], True) + history(cur, alt, 1, 2)
             + qkv(xb, alt, (2,)),
             (side, 0.0, 0.303), (logits(cur, p_v, True), 0.0, 0.88),
             (sum(ln_x(2, xc), []), 0.55, 0.96, due(z2_v, 0.96 + 0.02)),
            (wo_prep(0, 1), 0.257, 0.784, due(ops_v, 0.784 + 0.05)))
    wait(('x', 3), ('wo', 1))
    stats, sums = ln_x(3, xa)
    overlap(history(alt, cur, 1) + qkv(xc, cur, (0, 1)) + proj(0) + history(alt, cur, 2) + qkv(xc, cur, (2,)) + proj(1),
             (attend(cur, p_v), 0.0, 0.395), (wo_prep(2, 3), 0.0, 0.353),
             (logits(alt, gz_v), 0.105, 0.479), (attend(alt, gz_v), 0.479, 0.77), (logits(cur, p_v), 0.521, 0.97),
             (stats, 0.36, 0.85), (sums, 0.85, 0.96, due(ops_v, 0.96 + 0.02)))
    wait('win', ('x', 4), 'b')
    start('wsp', wsp_hbm, raw_a.at[0:S])
    lax.fori_loop(3, NB - 1, attn_step, None)
    attn_step(NB - 1, None)
    for k in range(2):
        start(('wd', k), wout_hbm.at[k * FH // 2:(k + 1) * FH // 2], raw_b.at[0:FH // 2, k * D:(k + 1) * D])
    barrier()
    overlap(up(0, ha, gz_v) + proj(NB - 1), (attend(cur, p_v), 0.0, 0.591),
             (sum(ln_h(1, hb), []) + bias_prep(), 0.429, 0.967, due(mlp_v, 0.97)))
    wait('wsp', ('wd', 0), ('wd', 1))
    lax.fori_loop(0, NB // 2 - 1, up_step, None)
    z6, z7 = ln_z(NB - 2, gz_v), ln_z(NB - 1, qk0)
    main = up(NB - 1, hb, qk0), gate_head()
    mid = (_cost(main[0]) + 1) / _cost(main[0] + main[1])
    overlap(main[0] + main[1], (z6[0], 0.0, 0.15), (z6[1], 0.15, 0.445, due(z2_v, 0.5)),
             (wd_prep1() + sp_prep1(0), 0.0, 0.2, due(ops_v, 0.2 + 0.04)), (sp_prep2(0), 0.448, 0.696),
             (z7[0], mid, 0.783), (z7[1], 0.783, 0.97, due(z2_v, 0.99)))
    barrier()
    gate_step(0, None, True)
    lax.fori_loop(1, NB, gate_step, None)
    pltpu.make_async_copy(x_v.at[0:S], out_hbm, osem).wait()


@jax.jit
def pallas_sequential_preLN__sliding_local_dilated__mixer_gmlp__prompt_kernel(
        A_x, A_wqkv, A_wo, B_x, B_w_in, B_w_sp, B_b_sp, B_w_out):
    del B_x
    hbm, vm = pl.BlockSpec(memory_space=pl.ANY), pltpu.VMEM
    out = pl.pallas_call(
        _kernel,
        out_shape=jax.ShapeDtypeStruct((S, D), BF16),
        in_specs=[hbm] * 7,
        out_specs=hbm,
        scratch_shapes=[
            vm((S + PAD, D), BF16),
            vm((S + PAD, S), BF16),
            vm((D + PAD, 2 * FH), BF16),
            vm((_rows(_EARLY, _LATE), 2 * T), I32), vm((_rows(_MLP), 2 * T), I32), vm((_rows(_Z2), 2 * T), I32),
            vm((W * TM + PAD, T), F32),
            *[vm((n * (TM + PAD) + PAD, T), F32) for n in (16, 8, 16, 8)],
            vm((8 * S + PAD, T), F32), vm((14 * TM + PAD, T), F32), vm((7 * S // 2, 2 * T), I32),
            vm((6 * TM, T), F32), vm((S, T), F32), vm((S // T, T), BF16),
            pltpu.SemaphoreType.DMA((36,)), pltpu.SemaphoreType.DMA(()), pltpu.SemaphoreType.REGULAR(()),
            *[vm((16 * Q + 8, T), F32)] * 6, *[vm((16 * 16 + 8, T), F32)] * 2, *[vm((8 * G + 8, T), F32)] * 4,
        ],
        compiler_params=pltpu.CompilerParams(vmem_limit_bytes=126 * 1024 * 1024),
    )(A_x.reshape(S, D), A_wqkv, A_wo, B_w_in, B_w_sp, B_b_sp.reshape(S // T, T), B_w_out)
    return out.reshape(1, S, D)
```

```python
import functools
import math

import numpy as np
import jax
import jax.numpy as jnp
from jax import lax
import jax.experimental.pallas as pl
import jax.experimental.pallas.tpu as pltpu

S, D, FH = 2048, 1024, 1792
DH, W, DIL = 32, 8, 2
EPS = 1e-5
F32, BF16, I32 = jnp.float32, jnp.bfloat16, jnp.int32
T = 128
Q = 64
TM = 2 * T
NB = S // TM
PAD = 16
G = 32
HEAD = 2


def _gelu2(h):
    c = math.sqrt(2.0 / math.pi)
    return h + h * jnp.tanh(h * (2 * c + (8 * c * 0.044715) * (h * h)))


def _skew(parts, axis, unit):
    return [c if i == 0 else pltpu.roll(c, unit * i, axis) for i, c in enumerate(parts)]


def _unskew(parts, axis, unit):
    n = parts[0].shape[axis]
    idx = lax.broadcasted_iota(I32, parts[0].shape, axis)
    x = [parts[-j % 8] for j in range(8)]
    for b in (1, 2, 4):
        on = (idx & (b * unit)) != 0
        x = [jnp.where(on, x[(j - b) % 8], x[j]) for j in range(8)]
    return [t if j == 0 else pltpu.roll(t, n - unit * j, axis) for j, t in enumerate(x)]


_LHS = (((1, 0, 0), (1, 1, 1)), ((1, 1, 0), (1, 1, 1)), ((1, 0, 0),), ((1, 1, 1),),
        ((1, 0, 0), (1, 0, 1)), ((1, 1, 0), (-1, 0, 0)), ((1, 0, 1), (-1, 1, 1)))
_RHS = (((1, 0, 0), (1, 1, 1)), ((1, 0, 0),), ((1, 0, 1), (-1, 1, 1)), ((1, 1, 0), (-1, 0, 0)),
        ((1, 1, 1),), ((1, 0, 0), (1, 0, 1)), ((1, 1, 0), (1, 1, 1)))
_ORDER = (6, 3, 1, 0, 4, 2, 5)


def _combine(terms, get):
    v = get(*terms[0][1:])
    for sign, a, b in terms[1:]:
        v = (lax.add if sign > 0 else lax.sub)(v, get(a, b))
    return v


def _seven(table, quad):
    return [_combine(terms, lambda a, b: quad[2 * a + b]) for terms in table]


def _sum(xs):
    return functools.reduce(lax.add, xs)


def _cost(tasks):
    return sum(c for c, _ in tasks)


def _merge(main, *sides):
    span, t, ev = _cost(main), 0.0, []
    for c, f in main:
        ev.append((t / span, 1, c / span, f))
        t += c
    for side, lo, hi, *timed in sides:
        ev += [(when, 0, 0.0, f) for events in timed for when, f in events]
        total, t = _cost(side), 0.0
        for c, f in side:
            ev.append((lo + (hi - lo) * t / total, 0, 0.0, f))
            t += c
    t0, span = 0.0, 1.0
    for when, _, c, f in sorted(ev, key=lambda e: e[:2]):
        if c:
            t0, span = when, c
        yield min(0.999, (when - t0) / span), f


def _stagger(stages):
    n, out = len(stages[0]), []
    for k in range(n + len(stages) - 1):
        now = [st[k - s] for s, st in enumerate(stages) if 0 <= k - s < n]
        now = [((j + 0.5) / len(g), s, t) for s, g in enumerate(now) for j, t in enumerate(g)]
        out += [t for _, _, t in sorted(now, key=lambda e: e[:2])]
    return out


def _run(tasks):
    for _, f in tasks:
        f()


def _tile(c):
    return slice(c * T, (c + 1) * T)


def _ds(start, n, align=8):
    if isinstance(start, int):
        return pl.ds(lax.add(np.int32(start), np.int32(0)), n)
    return pl.ds(pl.multiple_of(start, align), n)


class _Operand:
    def __init__(self, ref, base, levels, rows, nt):
        self.ref, self.base, self.levels, self.rows, self.nt = ref, base, levels, rows, nt

    @staticmethod
    def size(levels, rows, nt):
        return (7 ** levels * nt + 1) // 2 * rows // 2

    def shifted(self, i, step, most=None):
        size = self.size(self.levels, self.rows, self.nt) - (most or self.rows - step) // 2
        return _Operand(self.ref.at[_ds(self.base + i * (step // 2), size)], 0, self.levels, self.rows, self.nt)

    def at(self, j, r, c, n):
        g = j * self.nt + c
        return _ds(self.base + g // 2 * self.rows // 2 + r // 2, n // 2), _tile(g % 2)

    def put(self, r, c, mats, first=0):
        for j, t in enumerate(mats):
            self.ref[self.at(first + j, r, c, t.shape[0])] = pltpu.bitcast(lax.convert_element_type(t, BF16), I32)

    def rhs(self, j, c, ks):
        return pltpu.bitcast(self.ref[self.at(j, ks[0] * T, c, len(ks) * T)], BF16)

    def lhs(self, j, ks, zeros):
        cols = [self.ref[self.at(j, 0, c, self.rows)] for c in ks]
        for z in zeros:
            cols[-1] = jnp.concatenate([cols[-1][:-8], cols[-1][-8:] | z], 0)
        return jnp.concatenate([pltpu.bitcast(c, BF16) for c in cols], 1)


_EARLY = dict(wq=(1, D // 2, 4), wk=(1, D // 2, 4), wv=(1, D // 2, 4), wo=(1, D // 2, 4),
              xa=(1, T, 4), xb=(1, T, 4), oa=(1, T, 4))
_LATE = dict(wd2=(2, 3 * T, 2), wd1=(1, T, 4), sa2=(2, Q, 4), sa1=(1, T, 8))
_MLP = dict(win=(2, D // 4, 7), ha=(2, Q, 2), ya2=(2, Q, 3), ya1=(1, T, 1))
_Z2 = dict(z22=(2, S // 4, 3), z21=(1, S // 2, 1))


def _rows(*tables):
    return max(sum(_Operand.size(*s) for s in t.values()) for t in tables) + 8


def _kernel(x_hbm, wqkv_hbm, wo_hbm, win_hbm, wsp_hbm, b_hbm, wout_hbm, out_hbm,
            x_v, raw_a, raw_b, ops_v, mlp_v, z2_v, p_v, qk0, v0, qk1, v1, h_v, gz_v, z1_v, stat_v,
            bias_v, b_v, sems, osem, bar, *small):
    stage_v, tmp_v, perm_v = small[:6], small[6:8], small[8:]
    op = {}
    for ref, table in ((ops_v, _EARLY), (ops_v, _LATE), (mlp_v, _MLP), (z2_v, _Z2)):
        top = 0
        for name, shape in table.items():
            op[name] = _Operand(ref, top, *shape)
            top += _Operand.size(*shape)
    xa, xb, ha = op['xa'], op['xb'], op['ha']
    hb = _Operand(mlp_v, op['ya2'].base, *_MLP['ha'])
    xc = _Operand(z2_v, 0, *_EARLY['xa'])

    zero = lax.fori_loop(0, 2, lambda _, c: c ^ 1, 0)
    last, phase, paced, pending = [None], [0.0], {}, []
    ready, busy = {}, [False]

    def overlap(main, *sides):
        for phase[0], f in _merge(main, *sides):
            f()

    def pace(ref):
        if last[0] is None:
            return
        r = int(phase[0] * (last[0].shape[0] // 32)) * 32
        old = paced.get(id(ref), (None, 0))
        if old[0] is not last[0] or old[1] != r:
            paced[id(ref)] = last[0], r
            n = 8 if ref.dtype == F32 else 16
            ref[_ds(zero * n + (ref.shape[0] - n), n, n), 0:T] = last[0][r:r + n].astype(ref.dtype)

    for ref in (ops_v, mlp_v, z2_v):
        ref[_ds(ref.shape[0] - 8, 8), 0:T] = jnp.zeros((8, T), I32)

    def due(ref, *times):
        def run():
            pending.append(ref[_ds(zero * 8 + (ref.shape[0] - 8), 8), 0:T])
        return [(when, run) for when in times]

    def barrier():
        pl.semaphore_signal(bar, 1)
        pl.semaphore_wait(bar, 1)

    def products(lhs, rhs, u, emit, ks, level, first):
        if level == 0:
            def run():
                last[0] = jnp.dot(lhs.lhs(first, ks, pending), rhs.rhs(first, u, ks), preferred_element_type=F32)
                pending.clear()
                emit(0, 0, last[0])
            return [(len(ks) * lhs.rows / 4, run)]
        h = 2 ** (level - 1)
        state = {(i, j): [None, None] for i in range(h) for j in range(h)}

        def step(n):
            def take(i, j, m):
                s = state[i, j]
                if n == 0:
                    s[0] = m
                elif n == 1:
                    s[:] = s[0] + m, m
                elif n == 2:
                    emit(h + i, j, m + s[1])
                    s[1] = m
                elif n == 3:
                    s[:] = s[0] + m, m - s[1]
                elif n == 4:
                    emit(i, j, s[0] - m)
                    s[0] = m
                elif n == 5:
                    emit(i, h + j, m + s[0])
                    s[1] = s[1] + m
                else:
                    emit(h + i, h + j, s[1] + m)
            return take
        return [t for n, r in enumerate(_ORDER) for t in products(lhs, rhs, u, step(n), ks, level - 1, first * 7 + r)]

    def unit(lhs, rhs, u, emit, ks=None):
        return products(lhs, rhs, u, lambda a, b, v: emit(a * lhs.rows, b, v), ks or range(lhs.nt), lhs.levels, 0)

    def expand2(table, ref, get, dst, r, c):
        def task(r1):
            def run():
                pace(ref)
                quad = [_combine(table[r1], lambda a, b: get(2 * a + i, 2 * b + j)) for i in (0, 1) for j in (0, 1)]
                dst.put(r, c, _seven(table, quad), 7 * r1)
            return (3, run)
        return [task(r1) for r1 in _ORDER]

    def layer_norm(src, load, nt, stat, gain=1.0):
        def mean(r):
            def run():
                assert ready.get(id(src), True)
                pace(src)
                m = jnp.sum(_sum([load(r, c) for c in range(nt)]), axis=-1, keepdims=True) * (1.0 / (nt * T))
                stat_v[_ds(stat + r, 16), :] = jnp.broadcast_to(m, (16, T))
            return (nt / 2, run)

        def rstd(r):
            def run():
                pace(src)
                m = stat_v[_ds(stat + r, 16), :]
                v = [load(r, c) - m for c in range(nt)]
                var = jnp.sum(_sum([t * t for t in v]), axis=-1, keepdims=True) * (1.0 / (nt * T))
                inv = lax.rsqrt(var + EPS)
                stat_v[_ds(stat + TM + r, 16), :] = jnp.broadcast_to(inv if gain == 1.0 else gain * inv, (16, T))
            return (3 * nt / 4, run)

        def norm(r, c):
            m, inv = stat_v[_ds(stat + r, 16), :], stat_v[_ds(stat + TM + r, 16), :]
            return (load(r, c) - m) * inv
        return [f(r) for f in (mean, rstd) for r in range(0, TM, 16)], norm

    def raw_tile(ref, r, c):
        return ref[_ds(r, 16, 16), _tile(c)]

    def x_blk(i):
        return x_v.at[_ds(i * TM, TM, 16)]

    def h_blk(i):
        return h_v.at[_ds(i * TM, 7 * S + TM)]

    def ln_x(i, dst):
        x = x_blk(i)
        stats, norm = layer_norm(x_v, lambda r, c: raw_tile(x, r, c).astype(F32), 8, 0)

        def task(r, c):
            def run():
                pace(x_v)
                dst.put(r, c, _seven(_LHS, [norm(a + r, b + c) for a in (0, T) for b in (0, 4)]))
            return (5, run)
        return stats, [task(r, c) for r in range(0, T, 16) for c in range(4)]

    def ln_h(i, dst):
        h = h_blk(i)
        stats, norm = layer_norm(h_v, lambda r, c: h[_ds(c * S + r, 16), :], 8, 2 * TM, 0.5)
        return stats, [t for c in range(2) for r in range(0, Q, 16) for t in expand2(
            _LHS, h_v, lambda a, b, r=r, c=c: norm(a * Q + r, 2 * b + c), dst, r, c)]

    def ln_z(i, gz):
        stats, norm = layer_norm(gz, lambda r, c: gz[_ds(c * TM + r, 16), :], 14, 4 * TM)
        z21, z22 = op['z21'].shifted(i, T), op['z22'].shifted(i, Q)

        def task(r):
            def run():
                pace(gz)
                z21.put(r, 0, _seven(_RHS, [norm(a + r, c) for a in (0, T) for c in (12, 13)]))
            return (4, run)
        return stats, [task(r) for r in range(0, T, 16)] + [
            t for c in range(3) for r in range(0, Q, 16) for t in expand2(
                _RHS, gz, lambda a, b, r=r, c=c: norm(a * Q + r, 3 * b + c), z22, r, c)]

    def win_prep(i, n):
        src, dst = raw_b.at[_ds(i * n, 3 * D // 4 + n, 16)], op['win'].shifted(i, n)
        return [t for r in range(0, n, 16) for u in range(7) for t in expand2(
            _RHS, raw_b, lambda a, b, r=r, u=u: raw_tile(
                src, a * (D // 4) + r, 14 * (b % 2) + 7 * (b // 2) + u).astype(F32), dst, r, u)]

    def wd_tile(src, k, r, c):
        return raw_tile(src, k % 7 * T + r, k // 7 * 8 + c).astype(F32)

    def wd_prep1():
        def task(r, c):
            def run():
                pace(raw_b)
                op['wd1'].put(r, c, _seven(_RHS, [wd_tile(raw_b, k, r, b + c) for k in (12, 13) for b in (0, 4)]))
            return (3.5, run)
        return [task(r, c) for c in range(4) for r in range(0, T, 16)]

    def wd_prep2(i):
        src, dst = raw_b.at[_ds(i * 32, 6 * T + 32, 16)], op['wd2'].shifted(i, 32, 96)
        return [t for r in (0, 16) for k in range(3) for u in range(2) for t in expand2(
            _RHS, raw_b, lambda a, b, r=r, k=k, u=u: wd_tile(src, 3 * a + k, r, 4 * u + b), dst, k * T + r, u)]

    def sp_prep1(i):
        src = raw_a.at[_ds(i * TM, TM, 16)]

        def task(r, b):
            def run():
                pace(raw_a)
                op['sa1'].put(r, b, _seven(_LHS, [raw_tile(src, a + r, 2 * b + c).astype(F32)
                                                  for a in (0, T) for c in (0, 1)]))
            return (3.5, run)
        return [task(r, b) for b in range(NB) for r in range(0, T, 16)]

    def sp_prep2(i, where):
        src = raw_a.at[_ds(i * TM, TM, 16)]

        def gather(ref, o, r, c, a):
            def run():
                pace(raw_a)
                low, out = lax.broadcasted_iota(I32, (8, T), 1) < Q, []
                for half in (0, 1):
                    u, v = (pltpu.bitcast(raw_tile(src, a * Q + r, 4 * c + 2 * k + half), I32) for k in (0, 1))
                    out += [jnp.where(low, u, pltpu.roll(v, Q, 1)), jnp.where(low, pltpu.roll(u, Q, 1), v)]
                for b, t in enumerate([pltpu.bitcast(t, BF16).astype(F32) for t in out]):
                    ref[_ds(o + (4 * a + b) * 16, 16), :] = t
            return (2, run)
        jobs = [(*where(4 * c + r // 16), r, c) for c in range(4) for r in range(0, Q, 16)]
        return ([[gather(*job, a) for a in range(4)] for job in jobs],
                [expand2(_LHS, ref, lambda a, b, ref=ref, o=o: ref[_ds(o + (4 * a + b) * 16, 16), :], op['sa2'], r, c)
                 for ref, o, r, c in jobs])

    def qkv_prep(t, k):
        def where(stage, r):
            return perm_v[2 * stage + r // G % 2], (r // (D // 2) * G + r % G) * 4

        def drop(stage, r, vals):
            ref, o = where(stage, r)
            for c, v in enumerate(vals):
                ref[_ds(o + 8 * c, 8), :] = pltpu.bitcast(v, F32)

        def grab(stage, r, cs):
            ref, o = where(stage, r)
            pace(ref)
            return [pltpu.bitcast(ref[_ds(o + 8 * c, 8), :], I32) for c in cs]

        def skew(r):
            def run():
                pace(raw_a)
                drop(0, r, _skew([pltpu.bitcast(raw_tile(raw_a, t // 2 * D + r, t % 2 * 8 + c), I32)
                                  for c in range(8)], 1, 2))
            return (3, run)

        def unskew(r):
            return (4, lambda: drop(1, r, _unskew(grab(0, r, range(8)), 1, 2)))

        def store(r, c):
            def run():
                op['w' + 'qkv'[t]].put(r, c, _seven(_RHS, [
                    pltpu.bitcast(p, BF16).astype(F32) for a in (0, D // 2) for p in grab(1, a + r, (c, 4 + c))]))
            return (3, run)
        gs = range(k * T, (k + 1) * T, G)
        return [[[f(a + r) for r in range(g, g + G, 16) for a in (0, D // 2)] for g in gs]
                for f in (skew, unskew)] + [[[store(r, c) for r in range(g, g + G, 16) for c in range(4)] for g in gs]]

    def wo_prep(*cs):
        def swap(g, c, ref, b):
            def run():
                pace(raw_a)
                parts = [pltpu.bitcast(raw_tile(raw_a, D + i * T + g, 8 + b + 2 * c), I32) for i in range(8)]
                for j, p in enumerate(_unskew(_skew(parts, 0, 1), 0, 1)):
                    ref[_ds((b * 8 + j) * 8, 8), :] = pltpu.bitcast(p, F32)
            return (5, run)

        def store(g, c, ref, j):
            def run():
                pace(ref)
                op['wo'].put(j * T + g, c, _seven(_RHS, [
                    pltpu.bitcast(pltpu.bitcast(ref[_ds((b * 8 + a + j) * 8, 8), :], I32), BF16).astype(F32)
                    for a in (0, 4) for b in (0, 1)]))
            return (3, run)
        jobs = [(g, c, tmp_v[g // 16 % 2]) for c in cs for g in range(0, T, 16)]
        return _stagger([[[swap(*job, b) for b in (0, 1)] for job in jobs],
                         [[store(*job, j) for j in range(4)] for job in jobs]])

    def bias_prep():
        def task(k):
            def run():
                bias_v[_ds(k * T, T), :] = jnp.broadcast_to(b_v[...].astype(F32)[k:k + 1, :], (T, T)).T
            return (4, run)
        return [task(k) for k in range(S // T)]

    def row(c, r):
        return c * (TM + PAD) + PAD + r

    def qkv(lhs, bufs, which, ks=range(4), first=False):
        tasks = []
        for t in which:
            for u in range(4):
                def emit(a, b, v, t=t, u=u):
                    ref, c = bufs[t // 2], t % 2 * 8 + 4 * b + u
                    if ks[0]:
                        v = v + ref[_ds(row(c, a), T), :]
                    ref[_ds(row(c, a), T), :] = v
                    ready[id(ref)] = t > 0 and ks[-1] == 3 and (u, a, b) == (3, T, 1)
                    if first and t and a == 0:
                        ref[_ds(row(c, -PAD), PAD), :] = jnp.broadcast_to(v[0:1], (PAD, T))
                tasks += unit(lhs, op['w' + 'qkv'[t]], u, emit, ks)
        return tasks

    def history(src, dst, *which):
        def run():
            for t in which:
                for c in range(t % 2 * 8, t % 2 * 8 + 8):
                    dst[t // 2][_ds(row(c, -PAD), PAD), :] = src[t // 2][_ds(row(c, TM - PAD), PAD), :]
        return [(0, run)]

    scale = DH ** -0.5

    def slot(stage, w, r):
        return stage_v[2 * stage + r // Q % 2], (w * 2 + r // T) * Q + r % Q

    def grab(where, r, ws=range(W)):
        pace(where(0, r)[0])
        return [ref[_ds(o, 8), :] for ref, o in (where(w, r) for w in ws)]

    def drop(where, r, vals, first=0):
        for w, t in enumerate(vals, first):
            ref, o = where(w, r)
            ref[_ds(o, 8), :] = t

    def by_group(f, n=8):
        return [[f(a + r, range(k, k + n)) for a in (0, T) for r in range(g, g + Q, 8) for k in range(0, 8, n)]
                for g in (0, Q)]

    raw, prob, mixed = (functools.partial(slot, s) for s in range(3))

    def logits(bufs, dst, first=False):
        qk = bufs[0]

        def scores(r, ws):
            def run():
                assert ready[id(qk)]
                pace(qk)
                q = [qk[_ds(row(c, r), 8), :] for c in range(8)]
                drop(raw, r, (_sum([lax.mul(q[c], qk[_ds(row(8 + c, r - DIL * w), 8), :]) for c in range(8)])
                              for w in ws), ws[0])
            return (3.75, run)

        def fold(r, ws):
            def run():
                ps = grab(raw, r, ws)
                for bit in (16, 1):
                    low = (lax.broadcasted_iota(I32, (8, T), 1) & bit) == 0
                    ps = [p + jnp.where(low, pltpu.roll(p, T - bit, 1), pltpu.roll(p, bit, 1)) for p in ps]
                if first and r < DIL * W:
                    pos = lax.broadcasted_iota(I32, (8, T), 0) + r
                    ps = [jnp.where(pos >= DIL * w, p, -1e9 / scale) for w, p in zip(ws, ps)]
                drop(lambda w, r: (dst, w * TM + r), r, ps, ws[0])
            return (11.849 / 2, run)
        return _stagger([by_group(scores, 2), by_group(fold, 4)])

    def attend(bufs, src):
        v = bufs[1]

        def softmax(r, _):
            def run():
                lg = grab(lambda w, r: (src, w * TM + r), r)
                m = functools.reduce(jnp.maximum, lg)
                e = [jnp.exp2((p - m) * (scale * math.log2(math.e))) for p in lg]
                inv = 1.0 / _sum(e)
                drop(prob, r, [t * inv for t in e])
            return (7, run)

        def mix(r, cs):
            def run():
                assert ready[id(v)]
                pace(v)
                p = grab(prob, r)
                drop(mixed, r, (_sum([lax.mul(p[w], v[_ds(row(c, r - DIL * w), 8), :]) for w in range(W)])
                                for c in cs), cs[0])
            return (3.75, run)

        def combo(r, c):
            def run():
                pace(mixed(0, r)[0])
                assert not busy[0]
                op['oa'].put(r, c, _seven(_LHS, [ref[_ds(o, 16), :] for ref, o in (
                    mixed(b + c, a + r) for a in (0, T) for b in (0, 4))]))
            return (2, run)
        return _stagger([by_group(softmax), by_group(mix, 2),
                         [[combo(g + r, c) for r in range(0, Q, 16) for c in range(4)] for g in (0, Q)]])

    def proj(i):
        tasks, x, h = [], x_blk(i), h_blk(i)
        for u in range(4):
            def emit(a, b, v, u=u):
                c = b + 2 * u
                busy[0] = (u, a, b) != (3, T, 1)
                h[_ds(c * S + a, T), :] = x[_ds(a, T), _tile(c)].astype(F32) + v
            tasks += unit(op['oa'], op['wo'], u, emit)
        return tasks

    def z1_blk(i):
        return z1_v.at[_ds(i * T, 3 * S + T)]

    def z1_at(c, r, n):
        return _ds((c // 2 * S + r) // 2, n // 2), _tile(c % 2)

    def up(i, lhs, gz):
        tasks, z1 = [], z1_blk(i)
        for u in range(7):
            def emit(a, b, v, u=u):
                c = 7 * (b // 2) + u
                ready[id(gz)] = (u, a, b) == (6, 3 * Q, 3)
                if b % 2 == 0:
                    z1[z1_at(c, a, Q)] = pltpu.bitcast(v.astype(BF16), I32)
                else:
                    gz[_ds(c * TM + a, Q), :] = _gelu2(v)
            tasks += unit(lhs, op['win'], u, emit)
        return tasks

    def gate_head():
        def park(c):
            def emit(a, b, v):
                qk1[_ds(c(b) * TM + a, v.shape[0]), :] = v
            return emit
        tasks = unit(op['sa1'], op['z21'], 0, park(lambda b: 12 + b), range(2 * HEAD))
        for u in range(3):
            tasks += unit(op['sa2'], op['z22'], u, park(lambda b, u=u: 3 * b + u), range(HEAD))
        return tasks

    def gate_step(i, _, rest=False):
        last[0] = None
        z1, h, out, bias = z1_blk(i), h_blk(i), x_blk(i), bias_v.at[_ds(i * TM, TM)]
        extra = [(wd_prep2(3), 0.0, 0.244)] if rest else []

        def gated(c, r, v):
            n = v.shape[0]
            if rest:
                v = v + qk1[_ds(c * TM + r, n), :]
            return _gelu2(pltpu.bitcast(z1[z1_at(c, r, n)], BF16).astype(F32)) * (v + bias[_ds(r, n), :])

        y = {}

        def gate1(a, b, v):
            y[a, b] = gated(12 + b, a, v)
            if len(y) == 4:
                op['ya1'].put(0, 0, _seven(_LHS, [y[0, 0], y[0, 1], y[T, 0], y[T, 1]]))
        main, marks, sides = unit(op['sa1'], op['z21'], 0, gate1, range(2 * HEAD * rest, 8)), [], []
        for u in range(3):
            ref = (v0, v1)[u % 2]

            def gate2(a, b, v, u=u, ref=ref):
                ref[_ds(4 * a + b * Q, Q), :] = gated(3 * b + u, a, v)
            marks.append(_cost(main))
            main += unit(op['sa2'], op['z22'], u, gate2, range(HEAD * rest, 4))
            side = [expand2(_LHS, ref, lambda a, b, r=r, ref=ref: ref[_ds((4 * a + b) * Q + r, 16), :],
                            op['ya2'], r, u) for r in range(0, Q, 16)]
            sides.append([t for ts in zip(*side) for t in ts])
        marks.append(_cost(main))
        for u in range(4):
            def down1(a, b, v, u=u):
                at = _ds((4 * b + u) * S + a, T)
                h[at, :] = h[at, :] + v
            main += unit(op['ya1'], op['wd1'], u, down1)
        marks.append(_cost(main))
        for u in range(2):
            def down2(a, b, v, u=u):
                c = 4 * u + b
                out[_ds(a, Q), _tile(c)] = (h[_ds(c * S + a, Q), :] + v).astype(BF16)
                if a % T == Q and b % 2 == 1:
                    at = _ds(i * TM + a - Q, T, 16), slice((c - 1) * T, (c + 1) * T)
                    pltpu.make_async_copy(x_v.at[at], out_hbm.at[at], osem).start()
            main += unit(op['ya2'], op['wd2'], u, down2)
        t = [(m + 1) / _cost(main) for m in marks]
        span = (0.988, 0.99, 2.352) if rest else (0.811, 0.377, 1.947)
        nxt = i + 1 if rest else jnp.minimum(i + 1, NB - 1)
        fetch, sums = (sum(part, []) for part in sp_prep2(nxt, lambda n: (qk0, n * TM)))
        overlap(main, (fetch, 0.047 if rest else 0.0, 0.47 if rest else 0.377),
                *[(s, t[u + 1], t[u + 1] + span[u] * (t[u + 2] - t[u + 1])) for u, s in enumerate(sides)],
                 (sp_prep1(nxt), t[0] + (0.134 if rest else 0.0), 0.823 if rest else 0.635),
                (sums, t[4] + (-0.079 if rest else 0.022), 0.906 if rest else 0.95, due(ops_v, 0.99)), *extra)
        last[0] = None

    cur, alt = (qk0, v0), (qk1, v1)

    def attn_step(i, _):
        last[0] = None
        if isinstance(i, int):
            stats, sums = ln_h(0, ha)
            extra = [(stats, 0.29, 0.51), (sums, 0.51, 0.879, due(mlp_v, 0.99)),
                     (win_prep(3, 64), 0.0, 0.962, due(mlp_v, 0.25, 0.45, 0.65, 0.85))]
        else:
            stats, sums = ln_x(i + 1, xa)
            extra = [(stats, 0.299, 0.718), (sums, 0.751, 0.98, due(ops_v, 0.99)),
                     (win_prep(i - 3, 48), 0.001, 0.885, due(mlp_v, 0.25, 0.45, 0.619, 0.85))]
        overlap(history(cur, cur, 1) + qkv(xa, cur, (0, 1)) + history(cur, cur, 2) + qkv(xa, cur, (2,)) + proj(i - 1),
                 (attend(cur, p_v), 0.0, 0.492), (logits(cur, p_v), 0.501, 0.848), *extra)
        last[0] = None

    def up_step(j, _):
        last[0] = None
        i, sides = 2 * j + 1, []
        for t, z, h in ((0.0, ln_z(i - 1, gz_v), ln_h(i + 1, ha)), (0.501, ln_z(i, qk1), ln_h(i + 2, hb))):
            sides += [(z[0], t, t + 0.13), (z[1], t + 0.13, t + 0.331, due(z2_v, t + 0.331 + 0.022)),
                      (h[0], t + 0.25, t + 0.347), (h[1], t + 0.347, t + 0.47)]
        wd = wd_prep2(j)
        overlap(up(i, hb, qk1) + up(i + 1, ha, gz_v), *sides, ([], 0, 0, due(mlp_v, 0.99)),
                 *[(wd[k * len(wd) // 2:(k + 1) * len(wd) // 2], t + 0.011, t + 0.135, due(ops_v, t + 0.135 + 0.01))
                   for k, t in enumerate((0.0, 0.5))])
        last[0] = None

    copies = {}

    def start(key, src, dst):
        copies[key] = pltpu.make_async_copy(src, dst, sems.at[len(copies)])
        copies[key].start()

    def wait(*keys):
        for k in keys:
            copies[k].wait()

    def start_rows(t, k):
        for r in (k * T, D // 2 + k * T):
            start((t, r), wqkv_hbm.at[r:r + T, t * D:(t + 1) * D],
                  raw_a.at[t // 2 * D + r:t // 2 * D + r + T, t % 2 * D:(t % 2 + 1) * D])

    def start_x(lo, hi):
        start(('x', lo), x_hbm.at[lo * TM:hi * TM], x_v.at[lo * TM:hi * TM])

    def start_wo(k):
        start(('wo', k), wo_hbm.at[:, k * D // 2:(k + 1) * D // 2],
              raw_a.at[D:2 * D, D + k * D // 2:D + (k + 1) * D // 2])

    queue = [lambda: start_rows(0, 0), lambda: start_x(0, 1), lambda: start_x(1, 2),
             *[functools.partial(start_rows, t, k) for t in range(3) for k in range(4)][1:],
             lambda: start_wo(0), lambda: start_x(2, 3), lambda: start_wo(1), lambda: start_x(3, 4),
             lambda: start('win', win_hbm, raw_b.at[0:D]), lambda: start_x(4, NB), lambda: start('b', b_hbm, b_v)]

    def more(n):
        for _ in range(min(n, len(queue))):
            queue.pop(0)()

    def arrive(*chunks, ahead=0):
        wait(*[(t, a + k * T) for t, k in chunks for a in (0, D // 2)])
        more(len(chunks) + ahead)
        return _stagger([sum(st, []) for st in zip(*[qkv_prep(t, k) for t, k in chunks])])

    more(5)
    _run(arrive((0, 0)))
    wait(('x', 0))
    more(1)
    _run(sum(ln_x(0, xa), []))
    wait(('x', 1))
    more(1)
    overlap(qkv(xa, cur, (0,), [0]), (sum(ln_x(1, xb), []), 0.0, 0.86))
    overlap(qkv(xb, alt, (0,), [0]), (arrive((0, 1)), 0.0, 0.8))
    for t, ks, chunks, ahead, hi in (
            (0, [1], [(0, 2)], 0, 0.85), (0, [2], [(0, 3)], 0, 0.85), (0, [3], [(1, 0), (1, 1)], 0, 0.97),
            (1, [0, 1], [(1, 2), (1, 3)], 2, 0.745), (1, [2, 3], [(2, 0), (2, 1), (2, 2)], 0, 0.963)):
        overlap(qkv(xa, cur, (t,), ks, True) + qkv(xb, alt, (t,), ks),
                 (arrive(*chunks, ahead=ahead), 0.0, hi, due(ops_v, 0.98)))
    side = arrive((2, 3), ahead=len(queue))
    wait(('wo', 0), ('x', 2))
    overlap(qkv(xa, cur, (2,), [0, 1, 2], True) + qkv(xa, cur, (2,), [3], True) + history(cur, alt, 1, 2)
             + qkv(xb, alt, (2,)),
             (side, 0.0, 0.303), (logits(cur, p_v, True), 0.0, 0.88),
             (sum(ln_x(2, xc), []), 0.55, 0.96, due(z2_v, 0.96 + 0.02)),
            (wo_prep(0, 1), 0.257, 0.784, due(ops_v, 0.784 + 0.05)))
    wait(('x', 3), ('wo', 1))
    stats, sums = ln_x(3, xa)
    overlap(history(alt, cur, 1) + qkv(xc, cur, (0, 1)) + proj(0) + history(alt, cur, 2) + qkv(xc, cur, (2,)) + proj(1),
             (attend(cur, p_v), 0.0, 0.395), (wo_prep(2, 3), 0.0, 0.353),
             (logits(alt, gz_v), 0.105, 0.479), (attend(alt, gz_v), 0.479, 0.77), (logits(cur, p_v), 0.521, 0.97),
             (stats, 0.36, 0.85), (sums, 0.85, 0.96, due(ops_v, 0.96 + 0.02)))
    wait('win', ('x', 4), 'b')
    start('wsp', wsp_hbm, raw_a.at[0:S])
    lax.fori_loop(3, NB - 1, attn_step, None)
    attn_step(NB - 1, None)
    for k in range(2):
        start(('wd', k), wout_hbm.at[k * FH // 2:(k + 1) * FH // 2], raw_b.at[0:FH // 2, k * D:(k + 1) * D])
    barrier()
    overlap(up(0, ha, gz_v) + proj(NB - 1), (attend(cur, p_v), 0.0, 0.591),
             (sum(ln_h(1, hb), []) + bias_prep(), 0.429, 0.967, due(mlp_v, 0.97)))
    wait('wsp', ('wd', 0), ('wd', 1))
    lax.fori_loop(0, NB // 2 - 1, up_step, None)
    z6, z7 = ln_z(NB - 2, gz_v), ln_z(NB - 1, qk0)
    main = up(NB - 1, hb, qk0), gate_head()
    mid = (_cost(main[0]) + 1) / _cost(main[0] + main[1])
    overlap(main[0] + main[1], (z6[0], 0.0, 0.15), (z6[1], 0.15, 0.445, due(z2_v, 0.5)),
             (wd_prep1() + sp_prep1(0), 0.0, 0.2, due(ops_v, 0.2 + 0.04)),
            (_stagger(sp_prep2(0, lambda n: (tmp_v[n % 2], 0))), 0.448, 0.696),
             (z7[0], mid, 0.783), (z7[1], 0.783, 0.97, due(z2_v, 0.99)))
    barrier()
    gate_step(0, None, True)
    lax.fori_loop(1, NB, gate_step, None)
    pltpu.make_async_copy(x_v.at[0:S], out_hbm, osem).wait()


@jax.jit
def pallas_sequential_preLN__sliding_local_dilated__mixer_gmlp__prompt_kernel(
        A_x, A_wqkv, A_wo, B_x, B_w_in, B_w_sp, B_b_sp, B_w_out):
    del B_x
    hbm, vm = pl.BlockSpec(memory_space=pl.ANY), pltpu.VMEM
    out = pl.pallas_call(
        _kernel,
        out_shape=jax.ShapeDtypeStruct((S, D), BF16),
        in_specs=[hbm] * 7,
        out_specs=hbm,
        scratch_shapes=[
            vm((S + PAD, D), BF16),
            vm((S + PAD, S), BF16),
            vm((D + PAD, 2 * FH), BF16),
            vm((_rows(_EARLY, _LATE), 2 * T), I32), vm((_rows(_MLP), 2 * T), I32), vm((_rows(_Z2), 2 * T), I32),
            vm((W * TM + PAD, T), F32),
            *[vm((n * (TM + PAD) + PAD, T), F32) for n in (16, 8, 16, 8)],
            vm((8 * S + PAD, T), F32), vm((14 * TM + PAD, T), F32), vm((7 * S // 2, 2 * T), I32),
            vm((6 * TM, T), F32), vm((S, T), F32), vm((S // T, T), BF16),
            pltpu.SemaphoreType.DMA((36,)), pltpu.SemaphoreType.DMA(()), pltpu.SemaphoreType.REGULAR(()),
            *[vm((16 * Q + 8, T), F32)] * 6, *[vm((16 * 16 + 8, T), F32)] * 2, *[vm((8 * G + 8, T), F32)] * 4,
        ],
        compiler_params=pltpu.CompilerParams(vmem_limit_bytes=126 * 1024 * 1024),
    )(A_x.reshape(S, D), A_wqkv, A_wo, B_w_in, B_w_sp, B_b_sp.reshape(S // T, T), B_w_out)
    return out.reshape(1, S, D)
```
